```python
import jax
import jax.numpy as jnp

def _softmax(x, axis=-1):
    return jax.nn.softmax(x, axis=axis)
def _gelu(x):
    return jax.nn.gelu(x, approximate=True)
def _silu(x):
    return jax.nn.silu(x)
def _sigmoid(x):
    return jax.nn.sigmoid(x)
def _layernorm(x, axis=-1, eps=1e-5):
    m = jnp.mean(x, axis=axis, keepdims=True)
    v = jnp.var(x, axis=axis, keepdims=True)
    return (x - m) / jnp.sqrt(v + eps)
def _scatter_add(tgt, idx, src, axis=0):
    return tgt.at[idx].add(src)
def _segment_sum(src, seg, n):
    return jax.ops.segment_sum(src, seg, n)
class _Rng:
    def __init__(self, key):
        self._k = key
    def _next(self):
        self._k, sub = jax.random.split(self._k)
        return sub
    def normal(self, shape):
        return jax.random.normal(self._next(), shape, dtype=jnp.bfloat16)
    def randint(self, lo, hi, shape):
        return jax.random.randint(self._next(), shape, lo, hi, dtype=jnp.int32)
    def uniform(self, shape, lo=0.0, hi=1.0):
        return jax.random.uniform(self._next(), shape, jnp.bfloat16, lo, hi)
    def permutation(self, n):
        return jax.random.permutation(self._next(), n)


kernel_name = 'parallel_sum__sliding_local_dilated__glu_gated_geglu__prompt'

def setup_inputs():
    _rng = _Rng(jax.random.key(int.from_bytes(__import__("os").urandom(4), "little")))
    _w = (lambda a: (lambda t: t.astype(jnp.bfloat16) if jnp.issubdtype(t.dtype, jnp.floating) else t)(jnp.asarray(a)))
    def _A_setup():
        B, S, D = 1, 2048, 1024
        return {
            "x": _w((lambda *s: _rng.normal(s) * 0.05)(B, S, D)),
            "wqkv": _w((lambda *s: _rng.normal(s) * 0.05)(D, 3 * D)),
            "wo": _w((lambda *s: _rng.normal(s) * 0.05)(D, D)),
        }
    _A_in = _A_setup()

    def _B_setup():
        B, S, Dm, Df = 1, 2048, 1024, 3584
        return {
            "x": _w((lambda *s: _rng.normal(s) * 0.05)(B, S, Dm)),
            "w_gate": _w((lambda *s: _rng.normal(s) * 0.05)(Dm, Df) * (Dm ** -0.5)),
            "w_up": _w((lambda *s: _rng.normal(s) * 0.05)(Dm, Df) * (Dm ** -0.5)),
            "w_down": _w((lambda *s: _rng.normal(s) * 0.05)(Df, Dm) * (Df ** -0.5)),
        }
    _B_in = _B_setup()

    return {
        "A_x": _A_in["x"],
        "A_wqkv": _A_in["wqkv"],
        "A_wo": _A_in["wo"],
        "B_x": _B_in["x"],
        "B_w_gate": _B_in["w_gate"],
        "B_w_up": _B_in["w_up"],
        "B_w_down": _B_in["w_down"],
    }

def reference(A_x, A_wqkv, A_wo, B_x, B_w_gate, B_w_up, B_w_down):
    def _A_ref(x, wqkv, wo):
        B, S, D = x.shape
        H = 32; Dh = D // H
        W, dil = 8, 2
        qkv = (lambda x, *d: x.transpose(*d))((x @ wqkv).reshape(B, S, 3, H, Dh), 2, 0, 3, 1, 4)
        q, k, v = qkv[0], qkv[1], qkv[2]
        scale = Dh ** -0.5
        pos = jnp.arange(S)
        off = jnp.arange(W) * dil
        idx = pos[:, None] - off[None, :]
        mask = idx >= 0
        idx_c = jnp.where(mask, idx, 0).reshape(-1)
        kg = k[:, :, idx_c, :].reshape(B, H, S, W, Dh)
        vg = v[:, :, idx_c, :].reshape(B, H, S, W, Dh)
        logits = jnp.einsum("bhsd,bhswd->bhsw", q, kg) * scale
        logits = jnp.where(mask[None, None, :, :], logits, -1e9)
        attn = _softmax(logits, axis=-1)
        o = jnp.einsum("bhsw,bhswd->bhsd", attn, vg)
        return (lambda x, *d: x.transpose(*d))(o, 0, 2, 1, 3).reshape(B, S, D) @ wo

    def _B_ref(x, w_gate, w_up, w_down):
        g = jnp.einsum("bsd,df->bsf", x, w_gate)
        u = jnp.einsum("bsd,df->bsf", x, w_up)
        h = _gelu(g) * u
        return jnp.einsum("bsf,fd->bsd", h, w_down)

    x = A_x
    xn = _layernorm(x, axis=-1)
    return x + _A_ref(xn, A_wqkv, A_wo) + _B_ref(xn, B_w_gate, B_w_up, B_w_down)
```

```python
import functools
import jax
import jax.numpy as jnp
from jax import lax
import jax.experimental.pallas as pl
import jax.experimental.pallas.tpu as pltpu

S, D, F = 2048, 1024, 3584
H, DH, W, DIL = 32, 32, 8, 2
HALO = 16
NB = D // 128
HS = S // 2
HD = D // 2
FC = 512
NCH = F // FC
f32, bf16, u32 = jnp.float32, jnp.bfloat16, jnp.uint32


def _dot(a, b):
    return jnp.dot(a, b, preferred_element_type=f32)


def _lhs_terms(a11, a12, a21, a22):
    return [a11 + a22, a21 + a22, a11, a22, a11 + a12, a21 - a11, a12 - a22]


def _rhs_terms(b11, b12, b21, b22):
    return [b11 + b22, b11, b12 - b22, b21 - b11, b22, b11 + b12, b21 + b22]


def _strassen(a, b):
    m = [None] * 7
    for i in (2, 3, 0, 1, 4, 5, 6):
        m[i] = _dot(a(i), b(i))
    return (m[3] + m[0] - m[4] + m[6], m[2] + m[4], m[3] + m[1], m[2] + m[0] - m[1] + m[5])


def _swap_lane_block_bits(blocks):
    blocks = list(blocks)
    lane = lax.broadcasted_iota(jnp.int32, blocks[0].shape, 1)
    for cbit, lbit in ((0, 4), (1, 3), (2, 2)):
        s = 1 << lbit
        lo = (lane & s) == 0
        for c in range(NB):
            if c & (1 << cbit):
                continue
            a, b = blocks[c], blocks[c | (1 << cbit)]
            blocks[c] = jnp.where(lo, a, pltpu.roll(b, s, 1))
            blocks[c | (1 << cbit)] = jnp.where(lo, pltpu.roll(a, 128 - s, 1), b)
    return blocks


def make_kernel(HM0=256, HMQ=512, HMF=512, HMO=256, SUB=32, order="dta"):
    n0, nq, nf, no = HS // HM0, HS // HMQ, HS // HMF, HS // HMO
    n_att = NCH * nf
    RB = -(-S // (n_att * 16)) * 16

    def kernel(x_hbm, wqkv_hbm, wo_hbm, wg_hbm, wu_hbm, wd_hbm, out_hbm,
               xs, acc, xc, wraw, wc, graw, uraw, draw, gc, uc, dc, qn, kn, vn, on, kbuf, vbuf,
               xsem, wsem, fsem, osem):
        def x_copy(t, half):
            rows = pl.ds(pl.multiple_of(half * HS + t * HM0, HM0), HM0)
            return pltpu.make_async_copy(x_hbm.at[rows, :], xs.at[rows, :], xsem.at[2 * t + half])

        def w_copy(p):
            src = wo_hbm if p == 3 else wqkv_hbm.at[:, p * D:(p + 1) * D]
            return pltpu.make_async_copy(src, wraw.at[p], wsem.at[p])

        def f_copies(j, slot):
            cols = pl.ds(pl.multiple_of(j * FC, FC), FC)
            return (pltpu.make_async_copy(wg_hbm.at[:, cols], graw.at[slot], fsem.at[3 * slot]),
                    pltpu.make_async_copy(wu_hbm.at[:, cols], uraw.at[slot], fsem.at[3 * slot + 1]),
                    pltpu.make_async_copy(wd_hbm.at[cols, :], draw.at[slot], fsem.at[3 * slot + 2]))

        def o_copy(t, half):
            rows = pl.ds(pl.multiple_of(half * HS + t * HMO, HMO), HMO)
            return pltpu.make_async_copy(xs.at[rows, :], out_hbm.at[rows, :], osem.at[2 * t + half])

        def layernorm(t):
            halves = []
            for half in range(2):
                rows = pl.ds(pl.multiple_of(half * HS + t * HM0, HM0), HM0)
                x = xs[rows, :].astype(f32)
                acc[rows, :] = x
                xm = x - jnp.mean(x, axis=-1, keepdims=True)
                var = jnp.mean(xm * xm, axis=-1, keepdims=True)
                halves.append(xm * lax.rsqrt(var + 1e-5))
            top, bot = halves
            terms = _lhs_terms(top[:, :HD], top[:, HD:], bot[:, :HD], bot[:, HD:])
            for i in range(7):
                xc[i, pl.ds(pl.multiple_of(t * HM0, HM0), HM0), :] = terms[i].astype(bf16)

        def transform(raw, dst, part, nparts):
            hk, hn = raw.shape[0] // 2, raw.shape[1] // 2
            n = hk // nparts
            r0 = pl.multiple_of(part * n, n)
            top = raw[pl.ds(r0, n), :].astype(f32)
            bot = raw[pl.ds(hk + r0, n), :].astype(f32)
            terms = _rhs_terms(top[:, :hn], top[:, hn:], bot[:, :hn], bot[:, hn:])
            for i in range(7):
                dst[i, pl.ds(r0, n), :] = terms[i].astype(bf16)

        def transform_ffn(src_slot, dst_slot, part, nparts):
            transform(graw.at[src_slot], gc.at[dst_slot], part, nparts)
            transform(uraw.at[src_slot], uc.at[dst_slot], part, nparts)
            transform(draw.at[src_slot], dc.at[dst_slot], part, nparts)

        def project(p, dst, off, t, hm, scale=None):
            m0 = pl.multiple_of(t * hm, hm)
            c = _strassen(lambda i: xc[i, pl.ds(m0, hm), :], lambda i: wc[p, i])
            for b in range(4):
                val = c[b] if scale is None else c[b] * scale
                dst[pl.ds(off + (b // 2) * HS + m0, hm), (b % 2) * HD:(b % 2 + 1) * HD] = val.astype(bf16)

        def load_perm(ref, r0, n):
            blks = [pltpu.bitcast(ref[pl.ds(r0, n), c * 128:(c + 1) * 128], u32) for c in range(NB)]
            return [pltpu.bitcast(b, bf16).astype(f32) for b in _swap_lane_block_bits(blks)]

        def attention(t):
            s0 = pl.multiple_of(jnp.minimum(t * RB, S - RB), 16)
            kb = load_perm(kn, s0, RB + HALO)
            vb = load_perm(vn, s0, RB + HALO)
            for c in range(NB):
                kbuf[c] = kb[c]
                vbuf[c] = vb[c]
            lane = lax.broadcasted_iota(jnp.int32, (SUB, 128), 1)
            row = lax.broadcasted_iota(jnp.int32, (SUB, 128), 0)
            for sb in range(RB // SUB):
                q = load_perm(qn, s0 + sb * SUB, SUB)
                logits = []
                for w in range(W):
                    off = HALO + sb * SUB - DIL * w
                    p = None
                    for c in range(NB):
                        tt = q[c] * kbuf[c, off:off + SUB, :]
                        p = tt if p is None else p + tt
                    p = p + jnp.where((lane & 1) == 0, pltpu.roll(p, 127, 1), pltpu.roll(p, 1, 1))
                    p = p + jnp.where((lane & 2) == 0, pltpu.roll(p, 126, 1), pltpu.roll(p, 2, 1))
                    if sb * SUB < DIL * w:
                        p = jnp.where(row + (s0 + sb * SUB) >= DIL * w, p, -1e9)
                    logits.append(p)
                mx = functools.reduce(jnp.maximum, logits)
                es = [jnp.exp(p - mx) for p in logits]
                inv = 1.0 / functools.reduce(jnp.add, es)
                at = [e * inv for e in es]
                outs = []
                for c in range(NB):
                    o = None
                    for w in range(W):
                        off = HALO + sb * SUB - DIL * w
                        tt = at[w] * vbuf[c, off:off + SUB, :]
                        o = tt if o is None else o + tt
                    outs.append(pltpu.bitcast(o.astype(bf16), u32))
                outs = _swap_lane_block_bits(outs)
                for c in range(NB):
                    on[pl.ds(s0 + sb * SUB, SUB), c * 128:(c + 1) * 128] = pltpu.bitcast(outs[c], bf16)

        def ffn(slot, t):
            m0 = pl.multiple_of(t * HMF, HMF)
            xa = lambda i: xc[i, pl.ds(m0, HMF), :]
            g = _strassen(xa, lambda i: gc[slot, i])
            u = _strassen(xa, lambda i: uc[slot, i])
            h = [jax.nn.gelu(a, approximate=True) * b for a, b in zip(g, u)]
            hc = [v.astype(bf16) for v in _lhs_terms(*h)]
            c = _strassen(lambda i: hc[i], lambda i: dc[slot, i])
            for b in range(4):
                acc[pl.ds((b // 2) * HS + m0, HMF), (b % 2) * HD:(b % 2 + 1) * HD] += c[b]

        def out_proj(t):
            m0 = pl.multiple_of(t * HMO, HMO)
            top = on[pl.ds(m0, HMO), :].astype(f32)
            bot = on[pl.ds(HS + m0, HMO), :].astype(f32)
            oc = [v.astype(bf16) for v in _lhs_terms(top[:, :HD], top[:, HD:], bot[:, :HD], bot[:, HD:])]
            c = _strassen(lambda i: oc[i], lambda i: wc[3, i])
            for b in range(4):
                rows = pl.ds((b // 2) * HS + m0, HMO)
                cols = slice((b % 2) * HD, (b % 2 + 1) * HD)
                xs[rows, cols] = (acc[rows, cols] + c[b]).astype(bf16)

        x_copy(0, 0).start()
        x_copy(0, 1).start()
        w_copy(0).start()
        x_copy(0, 0).wait()
        x_copy(0, 1).wait()
        for t in range(1, n0):
            x_copy(t, 0).start()
            x_copy(t, 1).start()
        layernorm(0)
        w_copy(0).wait()
        w_copy(1).start()
        w_copy(2).start()
        transform(wraw.at[0], wc.at[0], 0, 1)

        def q_body(t, _):
            x_copy(t + 1, 0).wait()
            x_copy(t + 1, 1).wait()
            project(0, qn, 0, t, HM0, DH ** -0.5)
            layernorm(t + 1)
        lax.fori_loop(0, n0 - 1, q_body, None)
        w_copy(1).wait()
        for cp in f_copies(0, 0):
            cp.start()
        project(0, qn, 0, n0 - 1, HM0, DH ** -0.5)
        transform(wraw.at[1], wc.at[1], 0, 1)

        w_copy(2).wait()
        w_copy(3).start()
        for cp in f_copies(1, 1):
            cp.start()

        def k_body(t, _):
            project(1, kn, HALO, t, HMQ)
            transform(wraw.at[2], wc.at[2], t, nq)
        lax.fori_loop(0, nq, k_body, None)

        for cp in f_copies(0, 0):
            cp.wait()
        w_copy(3).wait()

        def v_body(t, _):
            project(2, vn, HALO, t, HMQ)
            transform_ffn(0, 0, t, nq)
            transform(wraw.at[3], wc.at[3], t, nq)
        lax.fori_loop(0, nq, v_body, None)
        kn[0:HALO, :] = jnp.zeros((HALO, D), bf16)
        vn[0:HALO, :] = jnp.broadcast_to(vn[HALO:2 * HALO, :].astype(f32)[0:1, :], (HALO, D)).astype(bf16)

        def chunk_body(j, _):
            slot = j % 2

            @pl.when(j + 1 < NCH)
            def _():
                for cp in f_copies(j + 1, 1 - slot):
                    cp.wait()

            @pl.when(j + 2 < NCH)
            def _():
                for cp in f_copies(j + 2, slot):
                    cp.start()

            src_slot = jnp.minimum(j + 1, NCH - 1) % 2

            def tile_body(t, _):
                for ch in order:
                    if ch == "d":
                        ffn(slot, t)
                    elif ch == "t":
                        transform_ffn(src_slot, 1 - slot, t, nf)
                    elif ch == "a":
                        attention(j * nf + t)
            lax.fori_loop(0, nf, tile_body, None)
        lax.fori_loop(0, NCH, chunk_body, None)

        def o_body(t, _):
            out_proj(t)
            o_copy(t, 0).start()
            o_copy(t, 1).start()
        lax.fori_loop(0, no, o_body, None)
        for t in range(no):
            o_copy(t, 0).wait()
            o_copy(t, 1).wait()

    scratch = [
        pltpu.VMEM((S, D), bf16),
        pltpu.VMEM((S, D), f32),
        pltpu.VMEM((7, HS, HD), bf16),
        pltpu.VMEM((4, D, D), bf16),
        pltpu.VMEM((4, 7, HD, HD), bf16),
        pltpu.VMEM((2, D, FC), bf16),
        pltpu.VMEM((2, D, FC), bf16),
        pltpu.VMEM((2, FC, D), bf16),
        pltpu.VMEM((2, 7, HD, FC // 2), bf16),
        pltpu.VMEM((2, 7, HD, FC // 2), bf16),
        pltpu.VMEM((2, 7, FC // 2, HD), bf16),
        pltpu.VMEM((S, D), bf16),
        pltpu.VMEM((HALO + S, D), bf16),
        pltpu.VMEM((HALO + S, D), bf16),
        pltpu.VMEM((S, D), bf16),
        pltpu.VMEM((NB, HALO + RB, 128), f32),
        pltpu.VMEM((NB, HALO + RB, 128), f32),
        pltpu.SemaphoreType.DMA((2 * n0,)),
        pltpu.SemaphoreType.DMA((4,)),
        pltpu.SemaphoreType.DMA((6,)),
        pltpu.SemaphoreType.DMA((2 * no,)),
    ]
    return kernel, scratch


@jax.jit
def pallas_parallel_sum__sliding_local_dilated__glu_gated_geglu__prompt_kernel(
    A_x, A_wqkv, A_wo, B_x, B_w_gate, B_w_up, B_w_down
):
    del B_x
    kernel, scratch = make_kernel()
    hbm = pl.BlockSpec(memory_space=pl.ANY)
    out = pl.pallas_call(
        kernel,
        in_specs=[hbm] * 6,
        out_specs=hbm,
        out_shape=jax.ShapeDtypeStruct((S, D), A_x.dtype),
        scratch_shapes=scratch,
        compiler_params=pltpu.CompilerParams(vmem_limit_bytes=120 * 1024 * 1024),
    )(A_x.reshape(S, D), A_wqkv, A_wo, B_w_gate, B_w_up, B_w_down)
    return out.reshape(1, S, D)
```

```python
import functools
import jax
import jax.numpy as jnp
from jax import lax
import jax.experimental.pallas as pl
import jax.experimental.pallas.tpu as pltpu

S, D, F = 2048, 1024, 3584
H, DH, W, DIL = 32, 32, 8, 2
HALO = 16
NB = D // 128
HS = S // 2
HD = D // 2
FC = 512
NCH = F // FC
f32, bf16, u32 = jnp.float32, jnp.bfloat16, jnp.uint32


def _dot(a, b):
    return jnp.dot(a, b, preferred_element_type=f32)


def _lhs_terms(a11, a12, a21, a22):
    return [a11 + a22, a21 + a22, a11, a22, a11 + a12, a21 - a11, a12 - a22]


def _rhs_terms(b11, b12, b21, b22):
    return [b11 + b22, b11, b12 - b22, b21 - b11, b22, b11 + b12, b21 + b22]


def _strassen(a, b):
    m = [None] * 7
    for i in (2, 3, 0, 1, 4, 5, 6):
        m[i] = _dot(a(i), b(i))
    return (m[3] + m[0] - m[4] + m[6], m[2] + m[4], m[3] + m[1], m[2] + m[0] - m[1] + m[5])


def _swap_lane_block_bits(blocks):
    blocks = list(blocks)
    lane = lax.broadcasted_iota(jnp.int32, blocks[0].shape, 1)
    for cbit, lbit in ((0, 4), (1, 3), (2, 2)):
        s = 1 << lbit
        lo = (lane & s) == 0
        for c in range(NB):
            if c & (1 << cbit):
                continue
            a, b = blocks[c], blocks[c | (1 << cbit)]
            blocks[c] = jnp.where(lo, a, pltpu.roll(b, s, 1))
            blocks[c | (1 << cbit)] = jnp.where(lo, pltpu.roll(a, 128 - s, 1), b)
    return blocks


def make_kernel(HM0=256, HMQ=512, HMF=512, HMO=256, SUB=32, order="dta", LNR=16, PR=16, PC=256):
    n0, nq, nf, no = HS // HM0, HS // HMQ, HS // HMF, HS // HMO
    n_att = NCH * nf
    RB = -(-S // (n_att * 16)) * 16

    def kernel(x_hbm, wqkv_hbm, wo_hbm, wg_hbm, wu_hbm, wd_hbm, out_hbm,
               xs, acc, xc, wc0, wc1, wc2, wc3, gc0, uc0, dc0, gc1, uc1, dc1, qn, kn, vn, on, kbuf, vbuf, zs,
               xsem, wsem, fsem, osem):
        gc, uc, dc = (gc0, gc1), (uc0, uc1), (dc0, dc1)
        wc = (wc0, wc1, wc2, wc3)
        def x_copy(t, half):
            rows = pl.ds(pl.multiple_of(half * HS + t * HM0, HM0), HM0)
            return pltpu.make_async_copy(x_hbm.at[rows, :], xs.at[rows, :], xsem.at[2 * t + half])

        def quad_copies(src, r0, c0, hk, hn, dst, sem):
            return [pltpu.make_async_copy(src.at[pl.ds(r0 + (b // 2) * hk, hk), pl.ds(c0 + (b % 2) * hn, hn)],
                                          dst.at[7 + b], sem.at[b]) for b in range(4)]

        def w_copies(p):
            src, c0 = (wo_hbm, 0) if p == 3 else (wqkv_hbm, p * D)
            return quad_copies(src, 0, c0, HD, HD, wc[p], wsem.at[p])

        def f_copies(j, slot):
            f0 = pl.multiple_of(j * FC, FC)
            return (quad_copies(wg_hbm, 0, f0, HD, FC // 2, gc[slot], fsem.at[3 * slot])
                    + quad_copies(wu_hbm, 0, f0, HD, FC // 2, uc[slot], fsem.at[3 * slot + 1])
                    + quad_copies(wd_hbm, f0, 0, FC // 2, HD, dc[slot], fsem.at[3 * slot + 2]))

        def start(cps):
            for cp in cps:
                cp.start()

        def wait(cps):
            for cp in cps:
                cp.wait()

        def o_copy(t, half):
            rows = pl.ds(pl.multiple_of(half * HS + t * HMO, HMO), HMO)
            return pltpu.make_async_copy(xs.at[rows, :], out_hbm.at[rows, :], osem.at[2 * t + half])

        def layernorm(t):
            for sb in range(HM0 // LNR):
                halves = []
                m0 = pl.multiple_of(t * HM0 + sb * LNR, LNR)
                for half in range(2):
                    rows = pl.ds(half * HS + m0, LNR)
                    x = xs[rows, :].astype(f32)
                    acc[rows, :] = x
                    xm = x - jnp.mean(x, axis=-1, keepdims=True)
                    var = jnp.mean(xm * xm, axis=-1, keepdims=True)
                    halves.append(xm * lax.rsqrt(var + 1e-5))
                top, bot = halves
                for c in range(HD // PC):
                    lo, hi = slice(c * PC, (c + 1) * PC), slice(HD + c * PC, HD + (c + 1) * PC)
                    terms = _lhs_terms(top[:, lo], top[:, hi], bot[:, lo], bot[:, hi])
                    for i in range(7):
                        xc[i, pl.ds(m0, LNR), lo] = terms[i].astype(bf16)

        def transform(buf, part, nparts):
            hk, hn = buf.shape[1], buf.shape[2]
            n = hk // nparts
            zero = part >> 10
            for sb in range(n // PR):
                r0 = pl.multiple_of(part * n + sb * PR, PR)
                for c in range(hn // PC):
                    cols = slice(c * PC, (c + 1) * PC)
                    terms = _rhs_terms(*[buf[7 + b, pl.ds(r0, PR), cols].astype(f32) for b in range(4)])
                    for i in range(7):
                        buf[i + zero, pl.ds(r0, PR), cols] = terms[i].astype(bf16)

        def transform_ffn(slot, part, nparts):
            transform(gc[slot], part, nparts)
            transform(uc[slot], part, nparts)
            transform(dc[slot], part, nparts)

        def project(p, dst, off, t, hm, scale=None):
            m0 = pl.multiple_of(t * hm, hm)
            c = _strassen(lambda i: xc[i, pl.ds(m0, hm), :], lambda i: wc[p][i])
            for b in (2, 1, 3, 0):
                val = c[b] if scale is None else c[b] * scale
                dst[pl.ds(off + (b // 2) * HS + m0, hm), (b % 2) * HD:(b % 2 + 1) * HD] = val.astype(bf16)

        def load_perm(ref, r0, n):
            blks = [pltpu.bitcast(ref[pl.ds(r0, n), c * 128:(c + 1) * 128], u32) for c in range(NB)]
            return [pltpu.bitcast(b, bf16).astype(f32) for b in _swap_lane_block_bits(blks)]

        def attention(t):
            s0 = pl.multiple_of(jnp.minimum(t * RB, S - RB), 16)
            kb = load_perm(kn, s0, RB + HALO)
            vb = load_perm(vn, s0, RB + HALO)
            for c in range(NB):
                kbuf[c] = kb[c]
                vbuf[c] = vb[c]
            lane = lax.broadcasted_iota(jnp.int32, (SUB, 128), 1)
            row = lax.broadcasted_iota(jnp.int32, (SUB, 128), 0)
            for sb in range(RB // SUB):
                q = load_perm(qn, s0 + sb * SUB, SUB)
                logits = []
                for w in range(W):
                    off = HALO + sb * SUB - DIL * w
                    p = None
                    for c in range(NB):
                        tt = q[c] * kbuf[c, off:off + SUB, :]
                        p = tt if p is None else p + tt
                    p = p + jnp.where((lane & 1) == 0, pltpu.roll(p, 127, 1), pltpu.roll(p, 1, 1))
                    p = p + jnp.where((lane & 2) == 0, pltpu.roll(p, 126, 1), pltpu.roll(p, 2, 1))
                    if sb * SUB < DIL * w:
                        p = jnp.where(row + (s0 + sb * SUB) >= DIL * w, p, -1e9)
                    logits.append(p)
                mx = functools.reduce(jnp.maximum, logits)
                es = [jnp.exp(p - mx) for p in logits]
                inv = 1.0 / functools.reduce(jnp.add, es)
                at = [e * inv for e in es]
                outs = []
                for c in range(NB):
                    o = None
                    for w in range(W):
                        off = HALO + sb * SUB - DIL * w
                        tt = at[w] * vbuf[c, off:off + SUB, :]
                        o = tt if o is None else o + tt
                    outs.append(pltpu.bitcast(o.astype(bf16), u32))
                outs = _swap_lane_block_bits(outs)
                for c in range(NB):
                    on[pl.ds(s0 + sb * SUB, SUB), c * 128:(c + 1) * 128] = pltpu.bitcast(outs[c], bf16)

        def ffn(slot, t):
            m0 = pl.multiple_of(t * HMF, HMF)
            xa = lambda i: xc[i, pl.ds(m0, HMF), :]
            g = _strassen(xa, lambda i: gc[slot][i])
            u = _strassen(xa, lambda i: uc[slot][i])
            h = [jax.nn.gelu(a, approximate=True) * b for a, b in zip(g, u)]
            hc = [v.astype(bf16) for v in _lhs_terms(*h)]
            c = _strassen(lambda i: hc[i], lambda i: dc[slot][i])
            for b in (2, 1, 3, 0):
                acc[pl.ds((b // 2) * HS + m0, HMF), (b % 2) * HD:(b % 2 + 1) * HD] += c[b]

        def out_proj(t):
            m0 = pl.multiple_of(t * HMO, HMO)
            top = on[pl.ds(m0, HMO), :].astype(f32)
            bot = on[pl.ds(HS + m0, HMO), :].astype(f32)
            oc = [v.astype(bf16) for v in _lhs_terms(top[:, :HD], top[:, HD:], bot[:, :HD], bot[:, HD:])]
            c = _strassen(lambda i: oc[i], lambda i: wc[3][i])
            for b in (2, 1, 3, 0):
                rows = pl.ds((b // 2) * HS + m0, HMO)
                cols = slice((b % 2) * HD, (b % 2 + 1) * HD)
                xs[rows, cols] = (acc[rows, cols] + c[b]).astype(bf16)

        x_copy(0, 0).start()
        x_copy(0, 1).start()
        start(w_copies(0))
        x_copy(0, 0).wait()
        x_copy(0, 1).wait()
        for t in range(1, n0):
            x_copy(t, 0).start()
            x_copy(t, 1).start()
        layernorm(0)
        wait(w_copies(0))
        start(w_copies(1))
        start(w_copies(2))
        transform(wc[0], 0, 1)

        def q_body(t, _):
            x_copy(t + 1, 0).wait()
            x_copy(t + 1, 1).wait()
            project(0, qn, 0, t, HM0, DH ** -0.5)
            layernorm(t + 1)
        lax.fori_loop(0, n0 - 1, q_body, None)
        wait(w_copies(1))
        start(f_copies(0, 0))
        project(0, qn, 0, n0 - 1, HM0, DH ** -0.5)
        transform(wc[1], 0, 1)

        wait(w_copies(2))
        start(w_copies(3))
        start(f_copies(1, 1))

        def k_body(t, _):
            project(1, kn, HALO, t, HMQ)
            transform(wc[2], t, nq)
        lax.fori_loop(0, nq, k_body, None)

        wait(f_copies(0, 0))
        wait(w_copies(3))

        def v_body(t, _):
            project(2, vn, HALO, t, HMQ)
            transform_ffn(0, t, nq)
            transform(wc[3], t, nq)
        lax.fori_loop(0, nq, v_body, None)
        kn[0:HALO, :] = jnp.zeros((HALO, D), bf16)
        vn[0:HALO, :] = jnp.broadcast_to(vn[HALO:2 * HALO, :].astype(f32)[0:1, :], (HALO, D)).astype(bf16)

        def chunk_body(j, _):
            for parity in range(2):
                @pl.when(j % 2 == parity)
                def _():
                    @pl.when(j + 1 < NCH)
                    def _():
                        wait(f_copies(j + 1, 1 - parity))

                    @pl.when(j + 2 < NCH)
                    def _():
                        start(f_copies(j + 2, parity))

                    def tile_body(t, _):
                        for ch in order:
                            if ch == "d":
                                ffn(parity, t)
                            elif ch == "t":
                                transform_ffn(1 - parity, t, nf)
                            elif ch == "a":
                                attention(j * nf + t)
                    lax.fori_loop(0, nf, tile_body, None)
        lax.fori_loop(0, NCH, chunk_body, None)

        def o_body(t, _):
            out_proj(t)
            o_copy(t, 0).start()
            o_copy(t, 1).start()
        lax.fori_loop(0, no, o_body, None)
        for t in range(no):
            o_copy(t, 0).wait()
            o_copy(t, 1).wait()

    scratch = [
        pltpu.VMEM((S, D), bf16),
        pltpu.VMEM((S, D), f32),
        pltpu.VMEM((7, HS, HD), bf16),
        pltpu.VMEM((11, HD, HD), bf16),
        pltpu.VMEM((11, HD, HD), bf16),
        pltpu.VMEM((11, HD, HD), bf16),
        pltpu.VMEM((11, HD, HD), bf16),
        pltpu.VMEM((11, HD, FC // 2), bf16),
        pltpu.VMEM((11, HD, FC // 2), bf16),
        pltpu.VMEM((11, FC // 2, HD), bf16),
        pltpu.VMEM((11, HD, FC // 2), bf16),
        pltpu.VMEM((11, HD, FC // 2), bf16),
        pltpu.VMEM((11, FC // 2, HD), bf16),
        pltpu.VMEM((S, D), bf16),
        pltpu.VMEM((HALO + S, D), bf16),
        pltpu.VMEM((HALO + S, D), bf16),
        pltpu.VMEM((S, D), bf16),
        pltpu.VMEM((NB, HALO + RB, 128), f32),
        pltpu.VMEM((NB, HALO + RB, 128), f32),
        pltpu.SMEM((1,), jnp.int32),
        pltpu.SemaphoreType.DMA((2 * n0,)),
        pltpu.SemaphoreType.DMA((4, 4)),
        pltpu.SemaphoreType.DMA((6, 4)),
        pltpu.SemaphoreType.DMA((2 * no,)),
    ]
    return kernel, scratch


@jax.jit
def pallas_parallel_sum__sliding_local_dilated__glu_gated_geglu__prompt_kernel(
    A_x, A_wqkv, A_wo, B_x, B_w_gate, B_w_up, B_w_down
):
    del B_x
    kernel, scratch = make_kernel(HMF=256)
    hbm = pl.BlockSpec(memory_space=pl.ANY)
    out = pl.pallas_call(
        kernel,
        in_specs=[hbm] * 6,
        out_specs=hbm,
        out_shape=jax.ShapeDtypeStruct((S, D), A_x.dtype),
        scratch_shapes=scratch,
        compiler_params=pltpu.CompilerParams(vmem_limit_bytes=120 * 1024 * 1024),
    )(A_x.reshape(S, D), A_wqkv, A_wo, B_w_gate, B_w_up, B_w_down)
    return out.reshape(1, S, D)
```

```python
import functools
import jax
import jax.numpy as jnp
import numpy as np
from jax import lax
import jax.experimental.pallas as pl
import jax.experimental.pallas.tpu as pltpu

S, D, F = 2048, 1024, 3584
H, DH, W, DIL = 32, 32, 8, 2
HALO = 16
NB = D // 128
HS, QS = S // 2, S // 4
HD, QD = D // 2, D // 4
FC = 512
NCH = F // FC
PR = 16
ORDER = (2, 3, 0, 1, 4, 5, 6)
f32, bf16, u32 = jnp.float32, jnp.bfloat16, jnp.uint32


def _dot(a, b):
    return jnp.dot(a, b, preferred_element_type=f32)


def _words(v):
    return pltpu.bitcast(v.astype(bf16), u32)


def _halves(w):
    return pltpu.bitcast(w, bf16)


def _lhs_terms(a11, a12, a21, a22):
    return [a11 + a22, a21 + a22, a11, a22, a11 + a12, a21 - a11, a12 - a22]


def _rhs_terms(b11, b12, b21, b22):
    return [b11 + b22, b11, b12 - b22, b21 - b11, b22, b11 + b12, b21 + b22]


def _seven_products(product, keep, fetch, finish):
    for i in (2, 3, 0):
        keep(i, product(i))
    m = product(1)
    keep(1, m)
    finish(2, fetch(3) + m)
    m = product(4)
    keep(4, m)
    finish(1, fetch(2) + m)
    finish(3, fetch(2) + fetch(0) - fetch(1) + product(5))
    finish(0, fetch(3) + fetch(0) - fetch(4) + product(6))


def _swap_lane_block_bits(blocks):
    blocks = list(blocks)
    lane = lax.broadcasted_iota(jnp.int32, blocks[0].shape, 1)
    for cbit, lbit in ((0, 4), (1, 3), (2, 2)):
        s = 1 << lbit
        lo = (lane & s) == 0
        for c in range(NB):
            if c & (1 << cbit):
                continue
            a, b = blocks[c], blocks[c | (1 << cbit)]
            blocks[c] = jnp.where(lo, a, pltpu.roll(b, s, 1))
            blocks[c | (1 << cbit)] = jnp.where(lo, pltpu.roll(a, 128 - s, 1), b)
    return blocks


def make_kernel(HM0=256, HMQ=512, HMF=128, HMO=256, AG=8, LB=16, TB=32, NP=4, TP=1, T2P=1, GATE_AT=(0, 0)):
    n0, nq, nf, no = HS // HM0, HS // HMQ, QS // HMF, HS // HMO
    n_att = -(-(S // AG) // (NCH * nf))

    def kernel(zero_ref, x_hbm, wqkv_hbm, wo_hbm, wg_hbm, wu_hbm, wd_hbm, out_hbm,
               acc, xraw, xc2, wc3, gc0, dc0, gc1, dc1, graw, draw, qo, kp, vp,
               xsem, qsem, wsem, fsem, osem, *work):
        gc, dc = (gc0, gc1), (dc0, dc1)
        pin, pout, pdown, pproj, hkeep, hc = (work[0:5], work[5:10], work[10:15], work[15:20], work[20:23], work[23:30])
        zeros = [zero_ref[k] for k in range(4)]
        zero = zeros[0]

        def x_copies(t):
            rows = [pl.ds(half * HS + t * HM0, HM0) for half in range(2)]
            return [pltpu.make_async_copy(x_hbm.at[r, :], xraw.at[r, :], xsem.at[t]) for r in rows]

        def f_copies(j, slot):
            cols = pl.ds(pl.multiple_of(j * FC, FC), FC)
            return [pltpu.make_async_copy(wg_hbm.at[:, cols], graw.at[slot, 0, pl.ds(0, D), :], fsem.at[slot]),
                    pltpu.make_async_copy(wu_hbm.at[:, cols], graw.at[slot, 1, pl.ds(0, D), :], fsem.at[slot]),
                    pltpu.make_async_copy(wd_hbm.at[cols, :], draw.at[slot, pl.ds(0, FC), :], fsem.at[slot])]

        def o_copies(t):
            rows = [pl.ds(pl.multiple_of(half * HS + t * HMO, HMO), HMO) for half in range(2)]
            return [pltpu.make_async_copy(xraw.at[r, :], out_hbm.at[r, :], osem) for r in rows]

        def start(cps):
            for cp in cps:
                cp.start()

        def wait(cps):
            for cp in cps:
                cp.wait()

        def hint(i, n):
            return i if isinstance(i, int) else pl.multiple_of(i, n)

        def rows_at(r0, n):
            return pl.ds(r0 if isinstance(r0, int) else pl.multiple_of(r0, n), n)

        def wrows(r0, n):
            return pl.ds(r0 // 2 if isinstance(r0, int) else pl.multiple_of(r0 // 2, 8), n // 2)

        def pace(raw, value):
            spare = raw.shape[0] - PR
            raw[pl.ds(pl.multiple_of(spare + zero, PR), PR), 0:128] = value.astype(bf16)

        def widen(ref, *idx):
            return _halves(pltpu.bitcast(ref[idx], u32)).astype(f32)

        def kept(bufs, n):
            def keep(i, v):
                bufs[i][0:n, :] = v
            return keep, lambda i: bufs[i][pl.ds(pl.multiple_of(zero, 8), n), :]

        def layernorm(xc, first, count, n):
            for m0 in range(first, first + count, n):
                xn = []
                for half in range(2):
                    r0 = half * HS + m0
                    x = [widen(xraw, rows_at(r0 + zero, n), slice(c * 128, (c + 1) * 128)) for c in range(NB)]
                    for c in range(NB):
                        acc[rows_at(r0, n), c * 128:(c + 1) * 128] = x[c]
                    mean = jnp.sum(functools.reduce(jnp.add, x), axis=-1, keepdims=True) * (1.0 / D)
                    xn.append([v - mean for v in x])
                for half in range(2):
                    x = xn[half]
                    var = jnp.sum(functools.reduce(jnp.add, [v * v for v in x]), axis=-1, keepdims=True) * (1.0 / D)
                    inv = lax.rsqrt(var + 1e-5)
                    xn[half] = [v * inv for v in x]
                for c in range(NB // 2):
                    terms = _lhs_terms(xn[0][c], xn[0][c + NB // 2], xn[1][c], xn[1][c + NB // 2])
                    for i in range(7):
                        xc[i, wrows(m0, n), c * 128:(c + 1) * 128] = _words(terms[i])
                for half in range(2):
                    for c in range(NB):
                        xraw[rows_at(half * HS + m0, n), c * 128:(c + 1) * 128] = xn[half][c].astype(bf16)

        def transform(raw, dst, part, nparts):
            hk, hn = (raw.shape[0] - PR) // 2, raw.shape[1] // 2
            n = hk // nparts
            for sb in range(n // PR):
                r0 = part * n + sb * PR
                for c in range(hn // 128):
                    terms = _rhs_terms(*[
                        widen(raw, rows_at((b // 2) * hk + r0, PR),
                              slice((b % 2) * hn + c * 128, (b % 2) * hn + (c + 1) * 128)) for b in range(4)])
                    for i in range(7):
                        dst[i, wrows(r0, PR), c * 128:(c + 1) * 128] = _words(terms[i])
                    if TP and (sb * (hn // 128) + c) % TP == TP - 1:
                        pace(raw, terms[6])

        def transform_qkv(raw, dst, part, nparts, TB=TB, paced=True):
            n = HD // nparts
            for sb in range(n // TB):
                r0 = part * n + sb * TB
                words = _swap_lane_block_bits([
                    jnp.concatenate([pltpu.bitcast(raw[rows_at(half * HD + r0, TB), c * 128:(c + 1) * 128], u32)
                                     for half in range(2)], axis=0) for c in range(NB)])
                vals = [_halves(w).astype(f32) for w in words]
                for c in range(NB // 2):
                    terms = _rhs_terms(vals[c][:TB], vals[c + NB // 2][:TB], vals[c][TB:], vals[c + NB // 2][TB:])
                    for i in range(7):
                        dst[i, wrows(r0, TB), c * 128:(c + 1) * 128] = _words(terms[i])
                if paced:
                    pace(raw, terms[6][:PR])

        def transform_out(raw, dst, part, nparts):
            n = HD // PR // nparts
            low = lax.broadcasted_iota(jnp.int32, (8, 128), 0) < 4
            for sb in range(n):
                g = part * n + sb
                base = (g & 1) * 128 + ((g >> 1) & 3) * 32 + ((g >> 3) & 1) * 16 + (g >> 4) * 8
                for c in range(NB // 2):
                    quad = [[], [], [], []]
                    for h3 in range(2):
                        for side in range(2):
                            cols = slice(side * HD + c * 128, side * HD + (c + 1) * 128)
                            a = raw[rows_at(base + h3 * 256, 8), cols].astype(f32)
                            b = raw[rows_at(base + h3 * 256 + 512, 8), cols].astype(f32)
                            quad[side].append(jnp.where(low, a, pltpu.roll(b, 4, 0)))
                            quad[2 + side].append(jnp.where(low, pltpu.roll(a, 4, 0), b))
                    terms = _rhs_terms(*[jnp.concatenate(v, axis=0) for v in quad])
                    for i in range(7):
                        dst[i, wrows(g * PR, PR), c * 128:(c + 1) * 128] = _words(terms[i])
                    pace(raw, terms[6])

        def two_level(block, terms_of, store, raw):
            for i in range(7):
                inner = terms_of(*[terms_of(*[block(p, q) for p in range(4)])[i] for q in range(4)])
                for j in range(7):
                    store(7 * i + j, _words(inner[j]))
                if T2P and i % T2P == T2P - 1:
                    pace(raw, inner[6])

        def transform2(raw, dst, part, nparts):
            n = QD // nparts
            for sb in range(n // PR):
                r0 = part * n + sb * PR
                for z in range(2):
                    def block(p, q):
                        kq, nq_ = 2 * (p // 2) + q // 2, 2 * (p % 2) + q % 2
                        return widen(raw, z, rows_at(kq * QD + r0, PR), slice(nq_ * 128, (nq_ + 1) * 128))

                    def store(i, w):
                        dst[i, wrows(r0, PR), z * 128:(z + 1) * 128] = w
                    two_level(block, _rhs_terms, store, raw.at[z])

        def expand_x(part, nparts):
            n = QS // nparts
            for sb in range(n // PR):
                m0 = part * n + sb * PR
                for c in range(QD // 128):
                    def block(p, q):
                        mq, kq = 2 * (p // 2) + q // 2, 2 * (p % 2) + q % 2
                        return widen(xraw, rows_at(mq * QS + m0, PR), slice(kq * QD + c * 128, kq * QD + (c + 1) * 128))

                    def store(i, w):
                        xc2[i, wrows(m0, PR), c * 128:(c + 1) * 128] = w
                    two_level(block, _lhs_terms, store, xraw)

        def project(lhs, wc, hm, finish):
            keep, fetch = kept(pproj, hm)
            for cb in range(NB // 2):
                _seven_products(lambda i: _dot(lhs(i, zeros[cb]), _halves(wc[i, :, cb * 128:(cb + 1) * 128])),
                                keep, fetch, lambda b, v: finish(b, cb, v))

        def project_x(xc, wc, dst, off, t, hm, scale=None):
            def finish(b, cb, v):
                dst[(b % 2) * (NB // 2) + cb, pl.ds(hint(off + (b // 2) * HS + t * hm, 8), hm), :] = (
                    v if scale is None else v * scale)
            project(lambda i, z: _halves(xc[i, wrows(t * hm + (0 if isinstance(t, int) else z), hm), :]), wc, hm, finish)

        def attention(step):
            lane = lax.broadcasted_iota(jnp.int32, (AG, 128), 1)
            row = lax.broadcasted_iota(jnp.int32, (AG, 128), 0)
            for g in range(n_att):
                s0 = pl.multiple_of(jnp.minimum((step * n_att + g) * AG, S), AG)
                q = [qo[c, pl.ds(s0, AG), :] for c in range(NB)]
                logits = [functools.reduce(jnp.add, [q[c] * kp[c, pl.ds(s0 + (HALO - DIL * w), AG), :]
                                                     for c in range(NB)]) for w in range(W)]
                for d in (1, 2):
                    logits = [p + jnp.where((lane & d) == 0, pltpu.roll(p, 128 - d, 1), pltpu.roll(p, d, 1))
                              for p in logits]
                logits = [jnp.where(row + s0 >= DIL * w, p, -1e9) if g * AG < DIL * w else p
                          for w, p in enumerate(logits)]
                mx = functools.reduce(jnp.maximum, logits)
                es = [jnp.exp(p - mx) for p in logits]
                inv = 1.0 / functools.reduce(jnp.add, es)
                at = [e * inv for e in es]
                for c in range(NB):
                    qo[c, pl.ds(s0, AG), :] = functools.reduce(
                        jnp.add, [at[w] * vp[c, pl.ds(s0 + (HALO - DIL * w), AG), :] for w in range(W)])

        def ffn(slot, t, shadow):
            m0 = t * HMF
            again = pl.ds(pl.multiple_of(zero, 8), HMF)

            def put(k, q, v):
                hc[k][(q // 2) * (HMF // 2):(q // 2 + 1) * (HMF // 2), (q % 2) * 128:(q % 2 + 1) * 128] = _words(v)

            def gate(p, q, c):
                h = jax.nn.gelu(c[:, :128], approximate=True) * c[:, 128:]
                if p != 0:
                    hkeep[p - 1][q] = h
                if p == 3:
                    put(1, q, hkeep[1][q, again, :] + h)
                    put(3, q, h)
                    put(6, q, hkeep[0][q, again, :] - h)
                if (p, q) == GATE_AT:
                    shadow(h[0:8])
                if p == 0:
                    put(0, q, h + hkeep[2][q, again, :])
                    put(2, q, h)
                    put(4, q, h + hkeep[0][q, again, :])
                    put(5, q, hkeep[1][q, again, :] - h)

            def outer(i, q, m):
                fetch = lambda k: pout[k][q, again, :]
                if i < 5:
                    pout[i][q] = m
                if i == 1:
                    gate(2, q, fetch(3) + m)
                elif i == 4:
                    gate(1, q, fetch(2) + m)
                elif i == 5:
                    gate(3, q, fetch(2) + fetch(0) - fetch(1) + m)
                elif i == 6:
                    gate(0, q, fetch(3) + fetch(0) - fetch(4) + m)

            keep, fetch = kept(pin, HMF)
            for i in ORDER:
                _seven_products(
                    lambda j: _dot(_halves(xc2[7 * i + j, wrows(m0, HMF), :]), _halves(gc[slot][7 * i + j])),
                    keep, fetch, lambda q, v: outer(i, q, v))

            keep, fetch = kept(pdown, 2 * HMF)
            for cb in range(2):
                def product(i):
                    lhs = hc[i][pl.ds(pl.multiple_of(zeros[cb], 8), HMF), :]
                    return _dot(_halves(lhs), _halves(dc[slot][i, :, cb * 256:(cb + 1) * 256]))

                def finish(b, v):
                    c0 = (b % 2) * HD + cb * 256
                    for qr in range(2):
                        acc[rows_at((b // 2) * HS + qr * QS + m0, HMF), c0:c0 + 256] += v[qr * HMF:(qr + 1) * HMF]
                keep(1, product(1))
                m = product(3)
                keep(3, m)
                finish(2, fetch(1) + m)
                keep(4, product(6))
                keep(0, product(0))
                keep(2, product(2))
                m = product(4)
                finish(1, fetch(2) + m)
                finish(0, fetch(0) + fetch(3) + fetch(4) - m)
                finish(3, fetch(0) - fetch(1) + fetch(2) + product(5))

        def out_proj(t):
            m0 = t * HMO
            quads = [jnp.concatenate([qo[(b % 2) * (NB // 2) + cb, rows_at((b // 2) * HS + m0, HMO), :]
                                      for cb in range(NB // 2)], axis=1) for b in range(4)]
            oc = [v.astype(bf16) for v in _lhs_terms(*quads)]

            def finish(b, cb, v):
                rows = rows_at((b // 2) * HS + m0, HMO)
                cols = slice((b % 2) * HD + cb * 128, (b % 2) * HD + (cb + 1) * 128)
                xraw[rows, cols] = (acc[rows, cols] + v).astype(bf16)
            project(lambda i, z: oc[i], wc3, HMO, finish)

        def projections(xc, wraw, wc0, wc1, wc2):
            def w_copies(p):
                src = wo_hbm if p == 3 else wqkv_hbm.at[:, p * D:(p + 1) * D]
                return [pltpu.make_async_copy(src, wraw.at[p, pl.ds(0, D), :], wsem.at[p])]

            def wq_copies(i):
                rows = [pl.ds(half * HD + i * (HD // NP), HD // NP) for half in range(2)]
                return [pltpu.make_async_copy(wqkv_hbm.at[r, pl.ds(0, D)], wraw.at[0, r, :], qsem.at[i]) for r in rows]

            start(x_copies(0))
            for i in range(NP):
                start(wq_copies(i))
            for c in range(NB):
                kp[c, 0:HALO, :] = jnp.zeros((HALO, 128), f32)
                kp[c, HALO + S:, :] = jnp.zeros((AG, 128), f32)
                vp[c, HALO + S:, :] = jnp.zeros((AG, 128), f32)
                qo[c, S:S + AG, :] = jnp.zeros((AG, 128), f32)
            wait(x_copies(0))
            for i in range(NP):
                wait(wq_copies(i))
                if i == NP - 2:
                    for t in range(1, n0):
                        start(x_copies(t))
                    start(w_copies(1))
                layernorm(xc, i * (HM0 // NP), HM0 // NP, HM0 // NP)
                transform_qkv(wraw.at[0], wc0, i, NP, HD // NP, paced=False)
            start(w_copies(2))

            for t in range(n0):
                if t + 1 < n0:
                    wait(x_copies(t + 1))
                if t == n0 - 2:
                    wait(w_copies(1))
                    start(w_copies(3))
                    start(f_copies(0, 0))
                project_x(xc, wc0, qo, 0, t, HM0, DH ** -0.5)
                if t + 1 < n0:
                    layernorm(xc, (t + 1) * HM0, HM0, LB)
                if t >= n0 - 2:
                    transform_qkv(wraw.at[1], wc1, t - (n0 - 2), 2)

            wait(w_copies(2))
            wait(w_copies(3))
            start(f_copies(1, 1))

            def k_body(t, _):
                project_x(xc, wc1, kp, HALO, t, HMQ)
                transform_qkv(wraw.at[2], wc2, t, nq)
                transform_out(wraw.at[3], wc3, t, nq)
            lax.fori_loop(0, nq, k_body, None)

            wait(f_copies(0, 0))

            def v_body(t, _):
                project_x(xc, wc2, vp, HALO, t, HMQ)
                expand_x(t, nq)
                transform2(graw.at[0], gc0, t, nq)
                transform(draw.at[0], dc0, t, nq)
            lax.fori_loop(0, nq, v_body, None)
            for c in range(NB):
                vp[c, 0:HALO, :] = jnp.broadcast_to(vp[c, HALO:HALO + 1, :], (HALO, 128))

        pl.run_scoped(projections,
                      pltpu.VMEM((7, HS // 2, HD), u32), pltpu.VMEM((4, D + PR, D), bf16),
                      *[pltpu.VMEM((7, HD // 2, HD), u32)] * 3)

        def chunk_body(j, _):
            src = jnp.minimum(j + 1, NCH - 1) % 2
            for parity in range(2):
                @pl.when(j % 2 == parity)
                def _():
                    @pl.when(j + 1 < NCH)
                    def _():
                        wait(f_copies(j + 1, 1 - parity))

                    @pl.when(j + 2 < NCH)
                    def _():
                        start(f_copies(j + 2, parity))

                    def tile_body(t, _):
                        def shadow(token):
                            qo[0, pl.ds(pl.multiple_of(S + AG + zero, 8), 8), :] = token
                            attention(j * nf + t)
                        ffn(parity, t, shadow)
                        transform2(graw.at[src], gc[1 - parity], t, nf)
                        transform(draw.at[src], dc[1 - parity], t, nf)
                    lax.fori_loop(0, nf, tile_body, None)
        lax.fori_loop(0, NCH, chunk_body, None)

        def o_body(t, _):
            out_proj(t)
            start(o_copies(t))
        lax.fori_loop(0, no, o_body, None)
        for t in range(no):
            wait(o_copies(t))

    scratch = [
        pltpu.VMEM((S, D), f32),
        pltpu.VMEM((S + PR, D), bf16),
        pltpu.VMEM((49, QS // 2, QD), u32),
        pltpu.VMEM((7, HD // 2, HD), u32),
        pltpu.VMEM((49, QD // 2, FC // 2), u32),
        pltpu.VMEM((7, FC // 4, HD), u32),
        pltpu.VMEM((49, QD // 2, FC // 2), u32),
        pltpu.VMEM((7, FC // 4, HD), u32),
        pltpu.VMEM((2, 2, D + PR, FC), bf16),
        pltpu.VMEM((2, FC + PR, D), bf16),
        pltpu.VMEM((NB, S + AG + 8, 128), f32),
        pltpu.VMEM((NB, HALO + S + AG, 128), f32),
        pltpu.VMEM((NB, HALO + S + AG, 128), f32),
        pltpu.SemaphoreType.DMA((n0,)),
        pltpu.SemaphoreType.DMA((NP,)),
        pltpu.SemaphoreType.DMA((4,)),
        pltpu.SemaphoreType.DMA((2,)),
        pltpu.SemaphoreType.DMA(()),
        *[pltpu.VMEM((HMF, 256), f32)] * 5,
        *[pltpu.VMEM((4, HMF, 256), f32)] * 5,
        *[pltpu.VMEM((2 * HMF, 256), f32)] * 5,
        *[pltpu.VMEM((max(HM0, HMQ, HMO), 128), f32)] * 5,
        *[pltpu.VMEM((4, HMF, 128), f32)] * 3,
        *[pltpu.VMEM((HMF, 256), u32)] * 7,
    ]
    return kernel, scratch


def make_call(**kw):
    kernel, scratch = make_kernel(**kw)
    hbm = pl.BlockSpec(memory_space=pl.ANY)
    return pl.pallas_call(
        kernel,
        in_specs=[pl.BlockSpec(memory_space=pltpu.SMEM)] + [hbm] * 6,
        out_specs=hbm,
        out_shape=jax.ShapeDtypeStruct((S, D), bf16),
        scratch_shapes=scratch,
        compiler_params=pltpu.CompilerParams(vmem_limit_bytes=126 * 1024 * 1024),
    )


@jax.jit
def pallas_parallel_sum__sliding_local_dilated__glu_gated_geglu__prompt_kernel(
    A_x, A_wqkv, A_wo, B_x, B_w_gate, B_w_up, B_w_down
):
    del B_x
    out = make_call(HMQ=256)(np.zeros((4,), np.int32), A_x.reshape(S, D), A_wqkv, A_wo, B_w_gate, B_w_up, B_w_down)
    return out.reshape(1, S, D)
```

```python
import functools
import jax
import jax.numpy as jnp
import numpy as np
from jax import lax
import jax.experimental.pallas as pl
import jax.experimental.pallas.tpu as pltpu

S, D, F = 2048, 1024, 3584
H, DH, W, DIL = 32, 32, 8, 2
HALO = 16
NB = D // 128
HS, QS = S // 2, S // 4
HD, QD = D // 2, D // 4
FC = 512
NCH = F // FC
PR = 16
ORDER = (2, 3, 0, 1, 4, 5, 6)
f32, bf16, u32 = jnp.float32, jnp.bfloat16, jnp.uint32


def _dot(a, b):
    return jnp.dot(a, b, preferred_element_type=f32)


def _words(v):
    return pltpu.bitcast(v.astype(bf16), u32)


def _halves(w):
    return pltpu.bitcast(w, bf16)


def _split(w):
    return jnp.concatenate([pltpu.unpack_elementwise(w, index=k, packed_dtype=bf16, unpacked_dtype=f32)
                            for k in range(2)], axis=0)


def _join(v):
    n = v.shape[0] // 2
    return pltpu.pack_elementwise([v[:n], v[n:]], packed_dtype=bf16).astype(u32)


def _lhs_terms(a11, a12, a21, a22):
    return [a11 + a22, a21 + a22, a11, a22, a11 + a12, a21 - a11, a12 - a22]


def _rhs_terms(b11, b12, b21, b22):
    return [b11 + b22, b11, b12 - b22, b21 - b11, b22, b11 + b12, b21 + b22]


def _seven_products(product, keep, fetch, finish):
    for i in (2, 3, 0):
        keep(i, product(i))
    m = product(1)
    keep(1, m)
    finish(2, fetch(3) + m)
    m = product(4)
    keep(4, m)
    finish(1, fetch(2) + m)
    finish(3, fetch(2) + fetch(0) - fetch(1) + product(5))
    finish(0, fetch(3) + fetch(0) - fetch(4) + product(6))


def _to_head_lanes(blocks):
    slot = lax.broadcasted_iota(jnp.int32, blocks[0].shape, 1) >> 2
    blocks = [pltpu.roll(b, 4 * c, 1) if c else b for c, b in enumerate(blocks)]
    yield
    blocks = [blocks[-j % NB] for j in range(NB)]
    for bit in (1, 2, 4):
        move = (slot & bit) != 0
        blocks = [jnp.where(move, blocks[(j - bit) % NB], blocks[j]) for j in range(NB)]
    return [pltpu.roll(b, 128 - 4 * j, 1) if j else b for j, b in enumerate(blocks)]


def _run(*stages):
    stages = list(stages)
    while stages:
        stages = [g for g in stages if next(g, True) is None]


def make_kernel(HM0=128, HMQ=256, HMF=128, HMO=256, AG=8, LB=16, TB=32, NP=4, TB0=16, TW=4, QSTOPS=(0, 1, 3), GATE_AT=(0, 0), NCH=NCH, scopes=False, PRIO=0):
    n0, nq, nf, no = HS // HM0, HS // HMQ, QS // HMF, HS // HMO
    n_att = -(-(S // AG) // (7 * nf))

    def kernel(zero_ref, x_hbm, wqkv_hbm, wo_hbm, wg_hbm, wu_hbm, wd_hbm, out_hbm,
               acc, xraw, xc2, wc3, gc0, dc0, gc1, dc1, graw, draw, qo, kp, vp,
               xsem, qsem, wsem, fsem, osem, *work):
        gc, dc = (gc0, gc1), (dc0, dc1)
        pin, pout, pdown, pproj, hkeep, hc = (work[0:5], work[5:10], work[10:15], work[15:20], work[20:23], work[23:30])
        zeros = [zero_ref[k] for k in range(4)]
        zero = zeros[0]

        def x_copies(t):
            rows = [rows_at(half * HS + t * HM0, HM0) for half in range(2)]
            return [pltpu.make_async_copy(x_hbm.at[r, :], xraw.at[r, :], xsem.at[t]) for r in rows]

        def f_copies(j, slot):
            cols = pl.ds(pl.multiple_of(j * FC, FC), FC)
            return [pltpu.make_async_copy(wg_hbm.at[:, cols], graw.at[slot, 0, pl.ds(0, D), :], fsem.at[slot]),
                    pltpu.make_async_copy(wu_hbm.at[:, cols], graw.at[slot, 1, pl.ds(0, D), :], fsem.at[slot]),
                    pltpu.make_async_copy(wd_hbm.at[cols, :], draw.at[slot, pl.ds(0, FC), :], fsem.at[slot])]

        def o_copies(t):
            rows = [pl.ds(pl.multiple_of(half * HS + t * HMO, HMO), HMO) for half in range(2)]
            return [pltpu.make_async_copy(xraw.at[r, :], out_hbm.at[r, :], osem) for r in rows]

        import contextlib
        scope = jax.named_scope if scopes else (lambda name: contextlib.nullcontext())

        def start(cps):
            for cp in cps:
                cp.start(priority=PRIO)

        def wait(cps):
            for cp in cps:
                cp.wait()

        def hint(i, n):
            return i if isinstance(i, int) else pl.multiple_of(i, n)

        def rows_at(r0, n):
            return pl.ds(r0 if isinstance(r0, int) else pl.multiple_of(r0, n), n)

        def wrows(r0, n):
            return pl.ds(r0 // 2 if isinstance(r0, int) else pl.multiple_of(r0 // 2, 8), n // 2)

        def pace(raw, value):
            spare = raw.shape[0] - PR
            raw[pl.ds(pl.multiple_of(spare + zeros[1], 8), 8), 0:128] = value[0:8].astype(bf16)

        def widen(ref, *idx):
            return _split(pltpu.bitcast(ref[idx], u32))

        def kept(bufs, n):
            def keep(i, v):
                bufs[i][0:n, :] = v
            return keep, lambda i: bufs[i][pl.ds(pl.multiple_of(zero, 8), n), :]

        def layernorm(xc, xn, mean, inv, first, count, n, paced=True):
            def block(r0, c, z):
                return widen(xraw, rows_at(r0 + zeros[z], n), slice(c * 128, (c + 1) * 128))

            def row_mean(vals):
                total = functools.reduce(jnp.add, vals)
                if paced:
                    pace(xraw, total)
                return jnp.broadcast_to(jnp.sum(total, axis=-1, keepdims=True) * (1.0 / D), (n, 128))

            def stat(ref, r0):
                return ref[rows_at(r0 + zero, n), :]

            pieces = [first + k for k in range(0, count, n)]
            starts = [half * HS + m0 for m0 in pieces for half in range(2)]
            for r0 in starts:
                mean[rows_at(r0, n), :] = row_mean([block(r0, c, 0) for c in range(NB)])
            yield
            for r0 in starts:
                mu = stat(mean, r0)
                inv[rows_at(r0, n), :] = lax.rsqrt(
                    row_mean([jnp.square(block(r0, c, 2) - mu) for c in range(NB)]) + 1e-5)
            yield
            for m0 in pieces:
                mu = [stat(mean, half * HS + m0) for half in range(2)]
                scale = [stat(inv, half * HS + m0) for half in range(2)]
                for c in range(NB // 2):
                    vals = []
                    for b in range(4):
                        r0, cb = (b // 2) * HS + m0, (b % 2) * (NB // 2) + c
                        vals.append((block(r0, cb, 3) - mu[b // 2]) * scale[b // 2])
                        xn[wrows(r0, n), cb * 128:(cb + 1) * 128] = _join(vals[b])
                    terms = _lhs_terms(*vals)
                    for i in range(7):
                        xc[i, wrows(m0, n), c * 128:(c + 1) * 128] = _join(terms[i])
                    if paced:
                        pace(xraw, terms[6])

        def transform(raw, dst, part, nparts):
            hk, hn = (raw.shape[0] - PR) // 2, raw.shape[1] // 2
            n = hk // nparts
            for sb in range(n // PR):
                r0 = part * n + sb * PR
                for c in range(hn // 128):
                    terms = _rhs_terms(*[
                        widen(raw, rows_at((b // 2) * hk + r0, PR),
                              slice((b % 2) * hn + c * 128, (b % 2) * hn + (c + 1) * 128)) for b in range(4)])
                    for i in range(7):
                        dst[i, wrows(r0, PR), c * 128:(c + 1) * 128] = _join(terms[i])
                    pace(raw, terms[6])

        def transform_qkv(raw, dst, part, nparts, TB=TB, paced=True):
            n = HD // nparts
            for sb in range(n // TB):
                r0 = part * n + sb * TB
                words = yield from _to_head_lanes([
                    jnp.concatenate([pltpu.bitcast(raw[rows_at(half * HD + r0, TB), c * 128:(c + 1) * 128], u32)
                                     for half in range(2)], axis=0) for c in range(NB)])
                yield
                top = [_split(w[:TB // 2]) for w in words]
                bot = [_split(w[TB // 2:]) for w in words]
                for c in range(NB // 2):
                    terms = _rhs_terms(top[c], top[c + NB // 2], bot[c], bot[c + NB // 2])
                    for i in range(7):
                        dst[i, wrows(r0, TB), c * 128:(c + 1) * 128] = _join(terms[i])
                if paced:
                    pace(raw, terms[6])

        def transform_out(raw, dst, part, nparts):
            n = HD // (2 * PR) // nparts
            low = lax.broadcasted_iota(jnp.int32, (8, 128), 0) < 4
            for sb in range(n):
                g = part * n + sb
                src = (g & 1) * 512 + ((g >> 1) & 3) * 32 + (g >> 3) * 8
                to = (g >> 3) * 256 + (g & 7) * PR
                for c in range(NB // 2):
                    for d2 in range(2):
                        quad = [[], [], [], []]
                        for b in range(4):
                            cols = slice((b % 2) * HD + c * 128, (b % 2) * HD + (c + 1) * 128)
                            for h3 in range(2):
                                r = src + h3 * 256 + (b // 2) * 16
                                u = raw[rows_at(r, 8), cols].astype(f32)
                                v = raw[rows_at(r + 128, 8), cols].astype(f32)
                                quad[b].append(jnp.where(low, pltpu.roll(u, 4, 0), v) if d2
                                               else jnp.where(low, u, pltpu.roll(v, 4, 0)))
                        terms = _rhs_terms(*[jnp.concatenate(v, axis=0) for v in quad])
                        for i in range(7):
                            dst[i, wrows(to + d2 * 128, PR), c * 128:(c + 1) * 128] = _words(terms[i])
                        pace(raw, quad[0][0])

        def two_level(block, terms_of, store, wait_for):
            for i in range(7):
                inner = terms_of(*[terms_of(*[block(p, q) for p in range(4)])[i] for q in range(4)])
                for j in range(7):
                    store(7 * i + j, _join(inner[j]))
                wait_for(inner[6])

        def transform2(raw, dst, part, nparts):
            n = QD // nparts
            for sb in range(n // PR):
                r0 = part * n + sb * PR
                for z in range(2):
                    def block(p, q):
                        kq, nq_ = 2 * (p // 2) + q // 2, 2 * (p % 2) + q % 2
                        return widen(raw, z, rows_at(kq * QD + r0, PR), slice(nq_ * 128, (nq_ + 1) * 128))

                    def store(i, w):
                        dst[i, wrows(r0, PR), z * 128:(z + 1) * 128] = w
                    two_level(block, _rhs_terms, store, functools.partial(pace, raw.at[z]))

        def expand_x(xn, part, nparts):
            n = QS // nparts
            for sb in range(n // PR):
                m0 = part * n + sb * PR
                for c in range(QD // 128):
                    def block(p, q):
                        mq, kq = 2 * (p // 2) + q // 2, 2 * (p % 2) + q % 2
                        cols = slice(kq * QD + c * 128, kq * QD + (c + 1) * 128)
                        return _split(xn[wrows(mq * QS + m0, PR), cols])

                    def store(i, w):
                        xc2[i, wrows(m0, PR), c * 128:(c + 1) * 128] = w

                    def wait_for(v):
                        xn[pl.ds(pl.multiple_of(S // 2 + zero, 8), 8), 0:128] = _join(v)
                    two_level(block, _lhs_terms, store, wait_for)

        def project(lhs, wc, hm, finish):
            keep, fetch = kept(pproj, hm)
            for cb in range(NB // 2):
                _seven_products(lambda i: _dot(lhs(i, zeros[cb]), _halves(wc[i + zero, :, cb * 128:(cb + 1) * 128])),
                                keep, fetch, lambda b, v: finish(b, cb, v))

        def project_x(xc, wc, dst, off, t, hm, scale=None):
            def finish(b, cb, v):
                dst[(b % 2) * (NB // 2) + cb, pl.ds(hint(off + (b // 2) * HS + t * hm, 8), hm), :] = (
                    v if scale is None else v * scale)
            project(lambda i, z: _halves(xc[i, wrows(t * hm + (0 if isinstance(t, int) else z), hm), :]), wc, hm, finish)

        def attention(step):
            lane = lax.broadcasted_iota(jnp.int32, (AG, 128), 1)
            row = lax.broadcasted_iota(jnp.int32, (AG, 128), 0)
            for g in range(n_att):
                s0 = pl.multiple_of(jnp.minimum((step * n_att + g) * AG, S), AG)
                q = [qo[c, pl.ds(s0, AG), :] for c in range(NB)]
                logits = [functools.reduce(jnp.add, [q[c] * kp[c, pl.ds(s0 + (HALO - DIL * w), AG), :]
                                                     for c in range(NB)]) for w in range(W)]
                for d in (1, 2):
                    logits = [p + jnp.where((lane & d) == 0, pltpu.roll(p, 128 - d, 1), pltpu.roll(p, d, 1))
                              for p in logits]
                logits = [jnp.where(row + s0 >= DIL * w, p, -1e9) if g * AG < DIL * w else p
                          for w, p in enumerate(logits)]
                mx = functools.reduce(jnp.maximum, logits)
                es = [jnp.exp(p - mx) for p in logits]
                inv = 1.0 / functools.reduce(jnp.add, es)
                at = [e * inv for e in es]
                for c in range(NB):
                    qo[c, pl.ds(s0, AG), :] = functools.reduce(
                        jnp.add, [at[w] * vp[c, pl.ds(s0 + (HALO - DIL * w), AG), :] for w in range(W)])

        def ffn(slot, t, started, shadow):
            m0 = t * HMF
            again = pl.ds(pl.multiple_of(zero, 8), HMF)

            def put(k, q, v):
                hc[k][(q // 2) * (HMF // 2):(q // 2 + 1) * (HMF // 2), (q % 2) * 128:(q % 2 + 1) * 128] = _words(v)

            def gate(p, q, c):
                h = jax.nn.gelu(c[:, :128], approximate=True) * c[:, 128:]
                if p != 0:
                    hkeep[p - 1][q] = h
                if p == 3:
                    put(1, q, hkeep[1][q, again, :] + h)
                    put(3, q, h)
                    put(6, q, hkeep[0][q, again, :] - h)
                if (p, q) == GATE_AT:
                    shadow(h[0:8])
                if p == 0:
                    put(0, q, h + hkeep[2][q, again, :])
                    put(2, q, h)
                    put(4, q, h + hkeep[0][q, again, :])
                    put(5, q, hkeep[1][q, again, :] - h)

            def outer(i, q, m):
                fetch = lambda k: pout[k][q, again, :]
                if i < 5:
                    pout[i][q] = m
                if i == 1:
                    gate(2, q, fetch(3) + m)
                elif i == 4:
                    gate(1, q, fetch(2) + m)
                elif i == 5:
                    gate(3, q, fetch(2) + fetch(0) - fetch(1) + m)
                elif i == 6:
                    gate(0, q, fetch(3) + fetch(0) - fetch(4) + m)

            keep, fetch = kept(pin, HMF)
            for i in ORDER:
                _seven_products(
                    lambda j: _dot(_halves(xc2[7 * i + j, wrows(m0, HMF), :]), _halves(gc[slot][7 * i + j])),
                    keep, fetch, lambda q, v: outer(i, q, v))

            keep, fetch = kept(pdown, 2 * HMF)
            for cb in range(2):
                def product(i):
                    lhs = hc[i][pl.ds(pl.multiple_of(zeros[cb], 8), HMF), :]
                    return _dot(_halves(lhs), _halves(dc[slot][i, :, cb * 256:(cb + 1) * 256]))

                def finish(b, v):
                    c0 = (b % 2) * HD + cb * 256
                    for qr in range(2):
                        rows = rows_at((b // 2) * HS + qr * QS + m0, HMF)
                        acc[rows, c0:c0 + 256] = (jnp.where(started, acc[rows, c0:c0 + 256], 0.0)
                                                  + v[qr * HMF:(qr + 1) * HMF])
                keep(1, product(1))
                m = product(3)
                keep(3, m)
                finish(2, fetch(1) + m)
                keep(4, product(6))
                keep(0, product(0))
                keep(2, product(2))
                m = product(4)
                finish(1, fetch(2) + m)
                finish(0, fetch(0) + fetch(3) + fetch(4) - m)
                finish(3, fetch(0) - fetch(1) + fetch(2) + product(5))

        def out_proj(t):
            m0 = t * HMO
            quads = [jnp.concatenate([qo[(b % 2) * (NB // 2) + cb, rows_at((b // 2) * HS + m0, HMO), :]
                                      for cb in range(NB // 2)], axis=1) for b in range(4)]
            oc = [v.astype(bf16) for v in _lhs_terms(*quads)]

            def finish(b, cb, v):
                rows = rows_at((b // 2) * HS + m0, HMO)
                cols = slice((b % 2) * HD + cb * 128, (b % 2) * HD + (cb + 1) * 128)
                xraw[rows, cols] = (xraw[rows, cols].astype(f32) + acc[rows, cols] + v).astype(bf16)
            project(lambda i, z: oc[i], wc3, HMO, finish)

        def projections(xc, xn, mean, inv, wraw, wc0, wc1, wc2):
            def w_copies(p):
                src = wo_hbm if p == 3 else wqkv_hbm.at[:, p * D:(p + 1) * D]
                return [pltpu.make_async_copy(src, wraw.at[p, pl.ds(0, D), :], wsem.at[p])]

            def wq_copies(i):
                rows = [rows_at(half * HD + i * (HD // NP), HD // NP) for half in range(2)]
                return [pltpu.make_async_copy(wqkv_hbm.at[r, pl.ds(0, D)], wraw.at[0, r, :], qsem.at[i]) for r in rows]

            with scope("prologue"):
                start(x_copies(0))
                lax.fori_loop(0, NP, lambda i, _: start(wq_copies(i)), None)
                lax.fori_loop(1, n0, lambda t, _: start(x_copies(t)), None)
                start(w_copies(1))
                for c in range(NB):
                    kp[c, 0:HALO, :] = jnp.zeros((HALO, 128), f32)
                    kp[c, HALO + S:, :] = jnp.zeros((AG, 128), f32)
                    vp[c, HALO + S:, :] = jnp.zeros((AG, 128), f32)
                    qo[c, S:S + AG, :] = jnp.zeros((AG, 128), f32)
                with scope("wait_x0"):
                    wait(x_copies(0))

                def first_body(i, _):
                    wait(wq_copies(i))
                    _run(*[transform_qkv(wraw.at[0], wc0, i * TW + k, NP * TW, TB0, paced=False) for k in range(TW)],
                         layernorm(xc, xn, mean, inv, i * (HM0 // NP), HM0 // NP, PR, paced=False))
                lax.fori_loop(0, NP, first_body, None)
                start(w_copies(2))

            with scope("qphase"):
                for lo, hi in zip(QSTOPS, QSTOPS[1:] + (n0,)):
                    with scope(f"wait_x{lo}"):
                        for t in range(lo + 1, min(hi + 1, n0)):
                            wait(x_copies(t))
                    if hi == n0:
                        with scope(f"wait_wk"):
                            wait(w_copies(1))
                        start(w_copies(3))
                        start(f_copies(0, 0))
                    for t in range(lo, hi):
                        project_x(xc, wc0, qo, 0, t, HM0, DH ** -0.5)
                        if t + 1 < n0:
                            _run(layernorm(xc, xn, mean, inv, (t + 1) * HM0, HM0, LB))
                _run(transform_qkv(wraw.at[1], wc1, 0, 1))

            wait(w_copies(2))
            wait(w_copies(3))
            start(f_copies(1, 1))

            def k_body(t, _):
                project_x(xc, wc1, kp, HALO, t, HMQ)
                transform_out(wraw.at[3], wc3, t, nq)
                _run(transform_qkv(wraw.at[2], wc2, t, nq))
            with scope("kphase"):
                lax.fori_loop(0, nq, k_body, None)

            wait(f_copies(0, 0))

            def v_body(t, _):
                project_x(xc, wc2, vp, HALO, t, HMQ)
                expand_x(xn, t, nq)
                transform2(graw.at[0], gc0, t, nq)
                transform(draw.at[0], dc0, t, nq)
            with scope("vphase"):
                lax.fori_loop(0, nq, v_body, None)
            for c in range(NB):
                vp[c, 0:HALO, :] = jnp.broadcast_to(vp[c, HALO:HALO + 1, :], (HALO, 128))

        pl.run_scoped(projections,
                      pltpu.VMEM((7, HS // 2, HD), u32), pltpu.VMEM((S // 2 + 8, D), u32),
                      pltpu.VMEM((S, 128), f32), pltpu.VMEM((S, 128), f32), pltpu.VMEM((4, D + PR, D), bf16),
                      *[pltpu.VMEM((7, HD // 2, HD), u32)] * 3)

        def chunk_body(j, _):
            src = jnp.minimum(j + 1, NCH - 1) % 2
            for parity in range(2):
                @pl.when(j % 2 == parity)
                def _():
                    @pl.when(j + 1 < NCH)
                    def _():
                        wait(f_copies(j + 1, 1 - parity))

                    @pl.when(j + 2 < NCH)
                    def _():
                        start(f_copies(j + 2, parity))

                    def tile_body(t, _):
                        def shadow(token):
                            qo[0, pl.ds(pl.multiple_of(S + AG + zero, 8), 8), :] = token
                            attention(j * nf + t)
                        ffn(parity, t, True if parity else j > 0, shadow)
                        transform2(graw.at[src], gc[1 - parity], t, nf)
                        transform(draw.at[src], dc[1 - parity], t, nf)
                    lax.fori_loop(0, nf, tile_body, None)
        with scope("ffn"):
            lax.fori_loop(0, NCH, chunk_body, None)

        def o_body(t, _):
            out_proj(t)
            start(o_copies(t))
        with scope("ophase"):
            lax.fori_loop(0, no, o_body, None)
        with scope("drain"):
            for t in range(no):
                wait(o_copies(t))

    scratch = [
        pltpu.VMEM((S, D), f32),
        pltpu.VMEM((S + PR, D), bf16),
        pltpu.VMEM((49, QS // 2, QD), u32),
        pltpu.VMEM((7, HD // 2, HD), u32),
        pltpu.VMEM((49, QD // 2, FC // 2), u32),
        pltpu.VMEM((7, FC // 4, HD), u32),
        pltpu.VMEM((49, QD // 2, FC // 2), u32),
        pltpu.VMEM((7, FC // 4, HD), u32),
        pltpu.VMEM((2, 2, D + PR, FC), bf16),
        pltpu.VMEM((2, FC + PR, D), bf16),
        pltpu.VMEM((NB, S + AG + 8, 128), f32),
        pltpu.VMEM((NB, HALO + S + AG, 128), f32),
        pltpu.VMEM((NB, HALO + S + AG, 128), f32),
        pltpu.SemaphoreType.DMA((n0,)),
        pltpu.SemaphoreType.DMA((NP,)),
        pltpu.SemaphoreType.DMA((4,)),
        pltpu.SemaphoreType.DMA((2,)),
        pltpu.SemaphoreType.DMA(()),
        *[pltpu.VMEM((HMF, 256), f32)] * 5,
        *[pltpu.VMEM((4, HMF, 256), f32)] * 5,
        *[pltpu.VMEM((2 * HMF, 256), f32)] * 5,
        *[pltpu.VMEM((max(HM0, HMQ, HMO), 128), f32)] * 5,
        *[pltpu.VMEM((4, HMF, 128), f32)] * 3,
        *[pltpu.VMEM((HMF, 256), u32)] * 7,
    ]
    return kernel, scratch


def make_call(**kw):
    kernel, scratch = make_kernel(**kw)
    hbm = pl.BlockSpec(memory_space=pl.ANY)
    return pl.pallas_call(
        kernel,
        in_specs=[pl.BlockSpec(memory_space=pltpu.SMEM)] + [hbm] * 6,
        out_specs=hbm,
        out_shape=jax.ShapeDtypeStruct((S, D), bf16),
        scratch_shapes=scratch,
        compiler_params=pltpu.CompilerParams(vmem_limit_bytes=126 * 1024 * 1024),
    )


@jax.jit
def pallas_parallel_sum__sliding_local_dilated__glu_gated_geglu__prompt_kernel(
    A_x, A_wqkv, A_wo, B_x, B_w_gate, B_w_up, B_w_down
):
    del B_x
    out = make_call()(np.zeros((4,), np.int32), A_x.reshape(S, D), A_wqkv, A_wo, B_w_gate, B_w_up, B_w_down)
    return out.reshape(1, S, D)
```

```python
import functools
import jax
import jax.numpy as jnp
import numpy as np
from jax import lax
import jax.experimental.pallas as pl
import jax.experimental.pallas.tpu as pltpu

S, D, F = 2048, 1024, 3584
H, DH, W, DIL = 32, 32, 8, 2
HALO = 16
NB = D // 128
HS, QS = S // 2, S // 4
HD, QD = D // 2, D // 4
FC = 512
NCH = F // FC
PR = 16
ORDER = (2, 3, 0, 1, 4, 5, 6)
f32, bf16, u32 = jnp.float32, jnp.bfloat16, jnp.uint32


def _dot(a, b):
    return jnp.dot(a, b, preferred_element_type=f32)


def _words(v):
    return pltpu.bitcast(v.astype(bf16), u32)


def _halves(w):
    return pltpu.bitcast(w, bf16)


def _split(w):
    return jnp.concatenate([pltpu.unpack_elementwise(w, index=k, packed_dtype=bf16, unpacked_dtype=f32)
                            for k in range(2)], axis=0)


def _join(v):
    n = v.shape[0] // 2
    return pltpu.pack_elementwise([v[:n], v[n:]], packed_dtype=bf16).astype(u32)


def _lhs_terms(a11, a12, a21, a22):
    return [a11 + a22, a21 + a22, a11, a22, a11 + a12, a21 - a11, a12 - a22]


def _rhs_terms(b11, b12, b21, b22):
    return [b11 + b22, b11, b12 - b22, b21 - b11, b22, b11 + b12, b21 + b22]


def _seven_products(product, keep, fetch, finish):
    for i in (2, 3, 0):
        keep(i, product(i))
    m = product(1)
    keep(1, m)
    finish(2, fetch(3) + m)
    m = product(4)
    keep(4, m)
    finish(1, fetch(2) + m)
    finish(3, fetch(2) + fetch(0) - fetch(1) + product(5))
    finish(0, fetch(3) + fetch(0) - fetch(4) + product(6))


def _to_head_lanes(blocks):
    slot = lax.broadcasted_iota(jnp.int32, blocks[0].shape, 1) >> 2
    blocks = [pltpu.roll(b, 4 * c, 1) if c else b for c, b in enumerate(blocks)]
    yield
    blocks = [blocks[-j % NB] for j in range(NB)]
    for bit in (1, 2, 4):
        move = (slot & bit) != 0
        blocks = [jnp.where(move, blocks[(j - bit) % NB], blocks[j]) for j in range(NB)]
    return [pltpu.roll(b, 128 - 4 * j, 1) if j else b for j, b in enumerate(blocks)]


def _run(*stages):
    stages = list(stages)
    while stages:
        stages = [g for g in stages if next(g, True) is None]


def make_kernel(HM0=128, HMQ=256, HMF=128, HMO=256, AG=8, LB=16, TB=32, NP=4, TB0=16, TW=4, QSTOPS=(0, 1, 3), GATE_AT=(0, 0), NCH=NCH, scopes=False, PRIO=0, OSPLIT=True):
    n0, nq, nf, no = HS // HM0, HS // HMQ, QS // HMF, HS // HMO
    n_att = -(-(S // AG) // (7 * nf))

    def kernel(zero_ref, x_hbm, wqkv_hbm, wo_hbm, wg_hbm, wu_hbm, wd_hbm, out_hbm,
               acc, xraw, xc2, wc3, gc0, dc0, gc1, dc1, graw, draw, qo, kp, vp,
               xsem, qsem, wsem, fsem, osem, *work):
        gc, dc = (gc0, gc1), (dc0, dc1)
        pin, pout, pdown, pproj, hkeep, hc = (work[0:5], work[5:10], work[10:15], work[15:20], work[20:23], work[23:30])
        zeros = [zero_ref[k] for k in range(4)]
        zero = zeros[0]

        def x_copies(t):
            rows = [rows_at(half * HS + t * HM0, HM0) for half in range(2)]
            return [pltpu.make_async_copy(x_hbm.at[r, :], xraw.at[r, :], xsem.at[t]) for r in rows]

        def f_copies(j, slot):
            cols = pl.ds(pl.multiple_of(j * FC, FC), FC)
            return [pltpu.make_async_copy(wg_hbm.at[:, cols], graw.at[slot, 0, pl.ds(0, D), :], fsem.at[slot]),
                    pltpu.make_async_copy(wu_hbm.at[:, cols], graw.at[slot, 1, pl.ds(0, D), :], fsem.at[slot]),
                    pltpu.make_async_copy(wd_hbm.at[cols, :], draw.at[slot, pl.ds(0, FC), :], fsem.at[slot])]

        def o_copies(t, cb):
            windows = [(rows_at((b // 2) * HS + t * HMO, HMO), pl.ds((b % 2) * HD + cb * 128, 128)) for b in range(4)]
            return [pltpu.make_async_copy(xraw.at[w], out_hbm.at[w], osem) for w in windows]

        import contextlib
        scope = jax.named_scope if scopes else (lambda name: contextlib.nullcontext())

        def start(cps):
            for cp in cps:
                cp.start(priority=PRIO)

        def wait(cps):
            for cp in cps:
                cp.wait()

        def hint(i, n):
            return i if isinstance(i, int) else pl.multiple_of(i, n)

        def rows_at(r0, n):
            return pl.ds(r0 if isinstance(r0, int) else pl.multiple_of(r0, n), n)

        def wrows(r0, n):
            return pl.ds(r0 // 2 if isinstance(r0, int) else pl.multiple_of(r0 // 2, 8), n // 2)

        def pace(raw, value):
            spare = raw.shape[0] - PR
            raw[pl.ds(pl.multiple_of(spare + zeros[1], 8), 8), 0:128] = value[0:8].astype(bf16)

        def widen(ref, *idx):
            return _split(pltpu.bitcast(ref[idx], u32))

        def kept(bufs, n):
            def keep(i, v):
                bufs[i][0:n, :] = v
            return keep, lambda i: bufs[i][pl.ds(pl.multiple_of(zero, 8), n), :]

        def layernorm(xc, xn, mean, inv, first, count, n, paced=True):
            def block(r0, c, z):
                return widen(xraw, rows_at(r0 + zeros[z], n), slice(c * 128, (c + 1) * 128))

            def row_mean(vals):
                total = functools.reduce(jnp.add, vals)
                if paced:
                    pace(xraw, total)
                return jnp.broadcast_to(jnp.sum(total, axis=-1, keepdims=True) * (1.0 / D), (n, 128))

            def stat(ref, r0):
                return ref[rows_at(r0 + zero, n), :]

            pieces = [first + k for k in range(0, count, n)]
            starts = [half * HS + m0 for m0 in pieces for half in range(2)]
            for r0 in starts:
                mean[rows_at(r0, n), :] = row_mean([block(r0, c, 0) for c in range(NB)])
            yield
            for r0 in starts:
                mu = stat(mean, r0)
                inv[rows_at(r0, n), :] = lax.rsqrt(
                    row_mean([jnp.square(block(r0, c, 2) - mu) for c in range(NB)]) + 1e-5)
            yield
            for m0 in pieces:
                mu = [stat(mean, half * HS + m0) for half in range(2)]
                scale = [stat(inv, half * HS + m0) for half in range(2)]
                for c in range(NB // 2):
                    vals = []
                    for b in range(4):
                        r0, cb = (b // 2) * HS + m0, (b % 2) * (NB // 2) + c
                        vals.append((block(r0, cb, 3) - mu[b // 2]) * scale[b // 2])
                        xn[wrows(r0, n), cb * 128:(cb + 1) * 128] = _join(vals[b])
                    terms = _lhs_terms(*vals)
                    for i in range(7):
                        xc[i, wrows(m0, n), c * 128:(c + 1) * 128] = _join(terms[i])
                    if paced:
                        pace(xraw, terms[6])

        def transform(raw, dst, part, nparts):
            hk, hn = (raw.shape[0] - PR) // 2, raw.shape[1] // 2
            n = hk // nparts
            for sb in range(n // PR):
                r0 = part * n + sb * PR
                for c in range(hn // 128):
                    terms = _rhs_terms(*[
                        widen(raw, rows_at((b // 2) * hk + r0, PR),
                              slice((b % 2) * hn + c * 128, (b % 2) * hn + (c + 1) * 128)) for b in range(4)])
                    for i in range(7):
                        dst[i, wrows(r0, PR), c * 128:(c + 1) * 128] = _join(terms[i])
                    pace(raw, terms[6])

        def transform_qkv(raw, dst, part, nparts, TB=TB, paced=True):
            n = HD // nparts
            for sb in range(n // TB):
                r0 = part * n + sb * TB
                words = yield from _to_head_lanes([
                    jnp.concatenate([pltpu.bitcast(raw[rows_at(half * HD + r0, TB), c * 128:(c + 1) * 128], u32)
                                     for half in range(2)], axis=0) for c in range(NB)])
                yield
                top = [_split(w[:TB // 2]) for w in words]
                bot = [_split(w[TB // 2:]) for w in words]
                for c in range(NB // 2):
                    terms = _rhs_terms(top[c], top[c + NB // 2], bot[c], bot[c + NB // 2])
                    for i in range(7):
                        dst[i, wrows(r0, TB), c * 128:(c + 1) * 128] = _join(terms[i])
                if paced:
                    pace(raw, terms[6])

        def transform_out(raw, dst, part, nparts):
            n = HD // (2 * PR) // nparts
            low = lax.broadcasted_iota(jnp.int32, (8, 128), 0) < 4
            for sb in range(n):
                g = part * n + sb
                src = (g & 1) * 512 + ((g >> 1) & 3) * 32 + (g >> 3) * 8
                to = (g >> 3) * 256 + (g & 7) * PR
                for c in range(NB // 2):
                    for d2 in range(2):
                        quad = [[], [], [], []]
                        for b in range(4):
                            cols = slice((b % 2) * HD + c * 128, (b % 2) * HD + (c + 1) * 128)
                            for h3 in range(2):
                                r = src + h3 * 256 + (b // 2) * 16
                                u = raw[rows_at(r, 8), cols].astype(f32)
                                v = raw[rows_at(r + 128, 8), cols].astype(f32)
                                quad[b].append(jnp.where(low, pltpu.roll(u, 4, 0), v) if d2
                                               else jnp.where(low, u, pltpu.roll(v, 4, 0)))
                        terms = _rhs_terms(*[jnp.concatenate(v, axis=0) for v in quad])
                        for i in range(7):
                            dst[i, wrows(to + d2 * 128, PR), c * 128:(c + 1) * 128] = _words(terms[i])
                        pace(raw, terms[6])

        def two_level(block, terms_of, store, wait_for):
            for i in range(7):
                inner = terms_of(*[terms_of(*[block(p, q) for p in range(4)])[i] for q in range(4)])
                for j in range(7):
                    store(7 * i + j, _join(inner[j]))
                wait_for(inner[6])

        def transform2(raw, dst, part, nparts):
            n = QD // nparts
            for sb in range(n // PR):
                r0 = part * n + sb * PR
                for z in range(2):
                    def block(p, q):
                        kq, nq_ = 2 * (p // 2) + q // 2, 2 * (p % 2) + q % 2
                        return widen(raw, z, rows_at(kq * QD + r0, PR), slice(nq_ * 128, (nq_ + 1) * 128))

                    def store(i, w):
                        dst[i, wrows(r0, PR), z * 128:(z + 1) * 128] = w
                    two_level(block, _rhs_terms, store, functools.partial(pace, raw.at[z]))

        def expand_x(xn, part, nparts):
            n = QS // nparts
            for sb in range(n // PR):
                m0 = part * n + sb * PR
                for c in range(QD // 128):
                    def block(p, q):
                        mq, kq = 2 * (p // 2) + q // 2, 2 * (p % 2) + q % 2
                        cols = slice(kq * QD + c * 128, kq * QD + (c + 1) * 128)
                        return _split(xn[wrows(mq * QS + m0, PR), cols])

                    def store(i, w):
                        xc2[i, wrows(m0, PR), c * 128:(c + 1) * 128] = w

                    def wait_for(v):
                        xn[pl.ds(pl.multiple_of(S // 2 + zero, 8), 8), 0:128] = _join(v)
                    two_level(block, _lhs_terms, store, wait_for)

        def project(lhs, wc, hm, finish, done=None):
            keep, fetch = kept(pproj, hm)
            for cb in range(NB // 2):
                _seven_products(lambda i: _dot(lhs(i, zeros[cb]), _halves(wc[i + zero, :, cb * 128:(cb + 1) * 128])),
                                keep, fetch, lambda b, v: finish(b, cb, v))
                if done is not None:
                    done(cb)

        def project_x(xc, wc, dst, off, t, hm, scale=None):
            def finish(b, cb, v):
                dst[(b % 2) * (NB // 2) + cb, pl.ds(hint(off + (b // 2) * HS + t * hm, 8), hm), :] = (
                    v if scale is None else v * scale)
            project(lambda i, z: _halves(xc[i, wrows(t * hm + (0 if isinstance(t, int) else z), hm), :]), wc, hm, finish)

        def attention(step):
            lane = lax.broadcasted_iota(jnp.int32, (AG, 128), 1)
            row = lax.broadcasted_iota(jnp.int32, (AG, 128), 0)
            for g in range(n_att):
                s0 = pl.multiple_of(jnp.minimum((step * n_att + g) * AG, S), AG)
                q = [qo[c, pl.ds(s0, AG), :] for c in range(NB)]
                logits = []
                for w in range(W):
                    rows = pl.ds(s0 + (HALO - DIL * w), AG)
                    logits.append(functools.reduce(jnp.add, [q[c] * kp[c, rows, :] for c in range(NB)]))
                for d in (1, 2):
                    logits = [p + jnp.where((lane & d) == 0, pltpu.roll(p, 128 - d, 1), pltpu.roll(p, d, 1))
                              for p in logits]
                logits = [jnp.where(row + s0 >= DIL * w, p, -1e9) if g * AG < DIL * w else p
                          for w, p in enumerate(logits)]
                mx = functools.reduce(jnp.maximum, logits)
                es = [jnp.exp(p - mx) for p in logits]
                inv = 1.0 / functools.reduce(jnp.add, es)
                at = [e * inv for e in es]
                for c in range(NB):
                    o = functools.reduce(
                        jnp.add, [at[w] * vp[c, pl.ds(s0 + (HALO - DIL * w), AG), :] for w in range(W)])
                    qo[c, pl.ds(s0, AG), :] = o

        def next_weights(src, slot, t):
            transform2(graw.at[src], gc[slot], t, nf)
            transform(draw.at[src], dc[slot], t, nf)

        def ffn(slot, t, started, shadow):
            m0 = t * HMF
            again = pl.ds(pl.multiple_of(zero, 8), HMF)

            def put(k, q, v):
                hc[k][(q // 2) * (HMF // 2):(q // 2 + 1) * (HMF // 2), (q % 2) * 128:(q % 2 + 1) * 128] = _words(v)

            def gate(p, q, c):
                h = jax.nn.gelu(c[:, :128], approximate=True) * c[:, 128:]
                if p != 0:
                    hkeep[p - 1][q] = h
                if p == 3:
                    put(1, q, hkeep[1][q, again, :] + h)
                    put(3, q, h)
                    put(6, q, hkeep[0][q, again, :] - h)
                if (p, q) == GATE_AT:
                    shadow(h[0:8])
                if p == 0:
                    put(0, q, h + hkeep[2][q, again, :])
                    put(2, q, h)
                    put(4, q, h + hkeep[0][q, again, :])
                    put(5, q, hkeep[1][q, again, :] - h)

            def outer(i, q, m):
                fetch = lambda k: pout[k][q, again, :]
                if i < 5:
                    pout[i][q] = m
                if i == 1:
                    gate(2, q, fetch(3) + m)
                elif i == 4:
                    gate(1, q, fetch(2) + m)
                elif i == 5:
                    gate(3, q, fetch(2) + fetch(0) - fetch(1) + m)
                elif i == 6:
                    gate(0, q, fetch(3) + fetch(0) - fetch(4) + m)

            keep, fetch = kept(pin, HMF)
            for i in ORDER:
                _seven_products(
                    lambda j: _dot(_halves(xc2[7 * i + j, wrows(m0, HMF), :]), _halves(gc[slot][7 * i + j])),
                    keep, fetch, lambda q, v: outer(i, q, v))

            keep, fetch = kept(pdown, 2 * HMF)
            for cb in range(2):
                def product(i):
                    lhs = hc[i][pl.ds(pl.multiple_of(zeros[cb], 8), HMF), :]
                    return _dot(_halves(lhs), _halves(dc[slot][i, :, cb * 256:(cb + 1) * 256]))

                def finish(b, v):
                    c0 = (b % 2) * HD + cb * 256
                    for qr in range(2):
                        rows = rows_at((b // 2) * HS + qr * QS + m0, HMF)
                        acc[rows, c0:c0 + 256] = (jnp.where(started, acc[rows, c0:c0 + 256], 0.0)
                                                  + v[qr * HMF:(qr + 1) * HMF])
                keep(1, product(1))
                m = product(3)
                keep(3, m)
                finish(2, fetch(1) + m)
                keep(4, product(6))
                keep(0, product(0))
                keep(2, product(2))
                m = product(4)
                finish(1, fetch(2) + m)
                finish(0, fetch(0) + fetch(3) + fetch(4) - m)
                finish(3, fetch(0) - fetch(1) + fetch(2) + product(5))

        def out_proj(t):
            m0 = t * HMO
            quads = [jnp.concatenate([qo[(b % 2) * (NB // 2) + cb, rows_at((b // 2) * HS + m0, HMO), :]
                                      for cb in range(NB // 2)], axis=1) for b in range(4)]
            oc = [v.astype(bf16) for v in _lhs_terms(*quads)]

            def finish(b, cb, v):
                rows = rows_at((b // 2) * HS + m0, HMO)
                cols = slice((b % 2) * HD + cb * 128, (b % 2) * HD + (cb + 1) * 128)
                xraw[rows, cols] = (xraw[rows, cols].astype(f32) + acc[rows, cols] + v).astype(bf16)
            project(lambda i, z: oc[i], wc3, HMO, finish, lambda cb: start(o_copies(t, cb)))

        def projections(xc, xn, mean, inv, wraw, wc0, wc1, wc2):
            def w_copies(p):
                src = wo_hbm if p == 3 else wqkv_hbm.at[:, p * D:(p + 1) * D]
                return [pltpu.make_async_copy(src, wraw.at[p, pl.ds(0, D), :], wsem.at[p])]

            def wq_copies(i):
                rows = [rows_at(half * HD + i * (HD // NP), HD // NP) for half in range(2)]
                return [pltpu.make_async_copy(wqkv_hbm.at[r, pl.ds(0, D)], wraw.at[0, r, :], qsem.at[i]) for r in rows]

            with scope("prologue"):
                start(x_copies(0))
                lax.fori_loop(0, NP, lambda i, _: start(wq_copies(i)), None)
                lax.fori_loop(1, n0, lambda t, _: start(x_copies(t)), None)
                start(w_copies(1))
                for c in range(NB):
                    kp[c, 0:HALO, :] = jnp.zeros((HALO, 128), f32)
                    kp[c, HALO + S:HALO + S + AG, :] = jnp.zeros((AG, 128), f32)
                    vp[c, HALO + S:HALO + S + AG, :] = jnp.zeros((AG, 128), f32)
                    qo[c, S:S + AG, :] = jnp.zeros((AG, 128), f32)
                with scope("wait_x0"):
                    wait(x_copies(0))

                def first_body(i, _):
                    wait(wq_copies(i))
                    _run(*[transform_qkv(wraw.at[0], wc0, i * TW + k, NP * TW, TB0, paced=False) for k in range(TW)],
                         layernorm(xc, xn, mean, inv, i * (HM0 // NP), HM0 // NP, PR, paced=False))
                lax.fori_loop(0, NP, first_body, None)
                start(w_copies(2))

            with scope("qphase"):
                for lo, hi in zip(QSTOPS, QSTOPS[1:] + (n0,)):
                    with scope(f"wait_x{lo}"):
                        for t in range(lo + 1, min(hi + 1, n0)):
                            wait(x_copies(t))
                    if hi == n0:
                        with scope(f"wait_wk"):
                            wait(w_copies(1))
                        start(w_copies(3))
                        start(f_copies(0, 0))
                    for t in range(lo, hi):
                        project_x(xc, wc0, qo, 0, t, HM0, DH ** -0.5)
                        if t + 1 < n0:
                            _run(layernorm(xc, xn, mean, inv, (t + 1) * HM0, HM0, LB))
                _run(transform_qkv(wraw.at[1], wc1, 0, 1))

            wait(w_copies(2))
            wait(w_copies(3))
            start(f_copies(1, 1))

            def k_body(t, _):
                project_x(xc, wc1, kp, HALO, t, HMQ)
                transform_out(wraw.at[3], wc3, t, nq)
                _run(transform_qkv(wraw.at[2], wc2, t, nq))
            with scope("kphase"):
                lax.fori_loop(0, nq, k_body, None)

            wait(f_copies(0, 0))

            def v_body(t, _):
                project_x(xc, wc2, vp, HALO, t, HMQ)
                expand_x(xn, t, nq)
                transform2(graw.at[0], gc0, t, nq)
                transform(draw.at[0], dc0, t, nq)
            with scope("vphase"):
                lax.fori_loop(0, nq, v_body, None)
            for c in range(NB):
                vp[c, 0:HALO, :] = jnp.broadcast_to(vp[c, HALO:HALO + 1, :], (HALO, 128))

        pl.run_scoped(projections,
                      pltpu.VMEM((7, HS // 2, HD), u32), pltpu.VMEM((S // 2 + 8, D), u32),
                      pltpu.VMEM((S, 128), f32), pltpu.VMEM((S, 128), f32), pltpu.VMEM((4, D + PR, D), bf16),
                      *[pltpu.VMEM((7, HD // 2, HD), u32)] * 3)

        def chunk_body(j, _):
            src = jnp.minimum(j + 1, NCH - 1) % 2

            @pl.when(j + 1 < NCH)
            def _():
                wait(f_copies(j + 1, 1 - j % 2))

            @pl.when(j + 2 < NCH)
            def _():
                start(f_copies(j + 2, j % 2))

            for parity in range(2):
                @pl.when(j % 2 == parity)
                def _():
                    def tile_body(t, _):
                        def shadow(token):
                            qo[0, pl.ds(pl.multiple_of(S + AG + zero, 8), 8), :] = token
                            attention(j * nf + t)
                        ffn(parity, t, True if parity else j > 0, shadow)
                        next_weights(src, 1 - parity, t)
                    lax.fori_loop(0, nf, tile_body, None)
        with scope("ffn"):
            lax.fori_loop(0, NCH, chunk_body, None)

        def o_body(t, _):
            out_proj(t)
        with scope("ophase"):
            lax.fori_loop(0, no, o_body, None)
        with scope("drain"):
            for t in range(no):
                for cb in range(NB // 2):
                    wait(o_copies(t, cb))

    scratch = [
        pltpu.VMEM((S, D), f32),
        pltpu.VMEM((S + PR, D), bf16),
        pltpu.VMEM((49, QS // 2, QD), u32),
        pltpu.VMEM((7, HD // 2, HD), u32),
        pltpu.VMEM((49, QD // 2, FC // 2), u32),
        pltpu.VMEM((7, FC // 4, HD), u32),
        pltpu.VMEM((49, QD // 2, FC // 2), u32),
        pltpu.VMEM((7, FC // 4, HD), u32),
        pltpu.VMEM((2, 2, D + PR, FC), bf16),
        pltpu.VMEM((2, FC + PR, D), bf16),
        pltpu.VMEM((NB, S + AG + 8, 128), f32),
        pltpu.VMEM((NB, HALO + S + AG, 128), f32),
        pltpu.VMEM((NB, HALO + S + AG, 128), f32),
        pltpu.SemaphoreType.DMA((n0,)),
        pltpu.SemaphoreType.DMA((NP,)),
        pltpu.SemaphoreType.DMA((4,)),
        pltpu.SemaphoreType.DMA((2,)),
        pltpu.SemaphoreType.DMA(()),
        *[pltpu.VMEM((HMF, 256), f32)] * 5,
        *[pltpu.VMEM((4, HMF, 256), f32)] * 5,
        *[pltpu.VMEM((2 * HMF, 256), f32)] * 5,
        *[pltpu.VMEM((max(HM0, HMQ, HMO), 128), f32)] * 5,
        *[pltpu.VMEM((4, HMF, 128), f32)] * 3,
        *[pltpu.VMEM((HMF, 256), u32)] * 7,
    ]
    return kernel, scratch


def make_call(flags=None, **kw):
    kernel, scratch = make_kernel(**kw)
    hbm = pl.BlockSpec(memory_space=pl.ANY)
    return pl.pallas_call(
        kernel,
        in_specs=[pl.BlockSpec(memory_space=pltpu.SMEM)] + [hbm] * 6,
        out_specs=hbm,
        out_shape=jax.ShapeDtypeStruct((S, D), bf16),
        scratch_shapes=scratch,
        compiler_params=pltpu.CompilerParams(vmem_limit_bytes=126 * 1024 * 1024, flags=flags),
    )


@jax.jit
def pallas_parallel_sum__sliding_local_dilated__glu_gated_geglu__prompt_kernel(
    A_x, A_wqkv, A_wo, B_x, B_w_gate, B_w_up, B_w_down
):
    del B_x
    out = make_call(HMQ=512)(np.zeros((4,), np.int32), A_x.reshape(S, D), A_wqkv, A_wo, B_w_gate, B_w_up, B_w_down)
    return out.reshape(1, S, D)
```

```python
import functools
import jax
import jax.numpy as jnp
import numpy as np
from jax import lax
import jax.experimental.pallas as pl
import jax.experimental.pallas.tpu as pltpu

S, D, F = 2048, 1024, 3584
H, DH, W, DIL = 32, 32, 8, 2
HALO = 16
NB = D // 128
HS, QS = S // 2, S // 4
HD, QD = D // 2, D // 4
FC = 512
NCH = F // FC
PR = 16
ORDER = (2, 3, 0, 1, 4, 5, 6)
f32, bf16, u32 = jnp.float32, jnp.bfloat16, jnp.uint32


def _dot(a, b):
    return jnp.dot(a, b, preferred_element_type=f32)


def _words(v):
    return pltpu.bitcast(v.astype(bf16), u32)


def _halves(w):
    return pltpu.bitcast(w, bf16)


def _lhs_terms(a11, a12, a21, a22):
    return [a11 + a22, a21 + a22, a11, a22, a11 + a12, a21 - a11, a12 - a22]


def _lhs_term(i, a):
    return (lambda: a(0) + a(3), lambda: a(2) + a(3), lambda: a(0), lambda: a(3),
            lambda: a(0) + a(1), lambda: a(2) - a(0), lambda: a(1) - a(3))[i]()


def _rhs_terms(b11, b12, b21, b22):
    return [b11 + b22, b11, b12 - b22, b21 - b11, b22, b11 + b12, b21 + b22]


def _seven_products(product, keep, fetch, finish):
    for i in (2, 3, 0):
        keep(i, product(i))
    m = product(1)
    keep(1, m)
    finish(2, fetch(3) + m)
    m = product(4)
    keep(4, m)
    finish(1, fetch(2) + m)
    finish(3, fetch(2) + fetch(0) - fetch(1) + product(5))
    finish(0, fetch(3) + fetch(0) - fetch(4) + product(6))


def _to_head_lanes(blocks):
    slot = lax.broadcasted_iota(jnp.int32, blocks[0].shape, 1) >> 2
    blocks = [pltpu.roll(b, 4 * c, 1) if c else b for c, b in enumerate(blocks)]
    yield
    blocks = [blocks[-j % NB] for j in range(NB)]
    for bit in (1, 2, 4):
        move = (slot & bit) != 0
        blocks = [jnp.where(move, blocks[(j - bit) % NB], blocks[j]) for j in range(NB)]
    return [pltpu.roll(b, 128 - 4 * j, 1) if j else b for j, b in enumerate(blocks)]


def _run(*stages):
    stages = list(stages)
    while stages:
        stages = [g for g in stages if next(g, True) is None]


def make_kernel(HM0=128, HMQ=512, HMF=128, AG=8, LB=16, TB=32, NP=4, TB0=16, TW=4, QSTOPS=(0, 1, 3), GATE_AT=(0, 0), NCH=NCH, scopes=False, PRIO=0, NE=6, EARLY_AT=2):
    n0, nq, nf = HS // HM0, HS // HMQ, QS // HMF
    n_att = -(-(S // AG) // (7 * nf))

    def kernel(zero_ref, x_hbm, wqkv_hbm, wo_hbm, wg_hbm, wu_hbm, wd_hbm, out_hbm,
               xraw, xc2, wc3, gc0, dc0, gc1, dc1, graw, draw, qo, kp, vp,
               xsem, qsem, wsem, fsem, osem, *work):
        gc, dc = (gc0, gc1), (dc0, dc1)
        pin, pout, pproj, hkeep, hc = work[0:5], work[5:10], work[10:15], work[15:19], work[19:26]
        zeros = [zero_ref[k] for k in range(4)]
        zero = zeros[0]

        def x_copies(t):
            rows = [rows_at(half * HS + t * HM0, HM0) for half in range(2)]
            return [pltpu.make_async_copy(x_hbm.at[r, :], xraw.at[r, :], xsem.at[t]) for r in rows]

        def f_copies(j, slot):
            cols = pl.ds(pl.multiple_of(j * FC, FC), FC)
            return [pltpu.make_async_copy(wg_hbm.at[:, cols], graw.at[slot, 0, pl.ds(0, D), :], fsem.at[slot]),
                    pltpu.make_async_copy(wu_hbm.at[:, cols], graw.at[slot, 1, pl.ds(0, D), :], fsem.at[slot]),
                    pltpu.make_async_copy(wd_hbm.at[cols, :], draw.at[slot, pl.ds(0, FC), :], fsem.at[slot])]

        import contextlib
        scope = jax.named_scope if scopes else (lambda name: contextlib.nullcontext())

        def start(cps):
            for cp in cps:
                cp.start(priority=PRIO)

        def wait(cps):
            for cp in cps:
                cp.wait()

        def hint(i, n):
            return i if isinstance(i, int) else pl.multiple_of(i, n)

        def rows_at(r0, n):
            return pl.ds(r0 if isinstance(r0, int) else pl.multiple_of(r0, n), n)

        def wrows(r0, n):
            return pl.ds(r0 // 2 if isinstance(r0, int) else pl.multiple_of(r0 // 2, 8), n // 2)

        def pace(raw, value):
            spare = raw.shape[0] - PR
            raw[pl.ds(pl.multiple_of(spare + zeros[1], 8), 8), 0:128] = value[0:8].astype(bf16)

        def widen(ref, *idx):
            return _halves(pltpu.bitcast(ref[idx], u32)).astype(f32)

        def kept(bufs, n):
            def keep(i, v):
                bufs[i][0:n, :] = v
            return keep, lambda i: bufs[i][pl.ds(pl.multiple_of(zero, 8), n), :]

        def layernorm(xc, xn, mean, inv, first, count, n, paced=True):
            def block(r0, c, z):
                return widen(xraw, rows_at(r0 + zeros[z], n), slice(c * 128, (c + 1) * 128))

            def row_mean(vals):
                total = functools.reduce(jnp.add, vals)
                if paced:
                    pace(xraw, total)
                return jnp.broadcast_to(jnp.sum(total, axis=-1, keepdims=True) * (1.0 / D), (n, 128))

            def stat(ref, r0):
                return ref[rows_at(r0 + zero, n), :]

            pieces = [first + k for k in range(0, count, n)]
            starts = [half * HS + m0 for m0 in pieces for half in range(2)]
            for r0 in starts:
                mean[rows_at(r0, n), :] = row_mean([block(r0, c, 0) for c in range(NB)])
            yield
            for r0 in starts:
                mu = stat(mean, r0)
                inv[rows_at(r0, n), :] = lax.rsqrt(
                    row_mean([jnp.square(block(r0, c, 2) - mu) for c in range(NB)]) + 1e-5)
            yield
            for m0 in pieces:
                mu = [stat(mean, half * HS + m0) for half in range(2)]
                scale = [stat(inv, half * HS + m0) for half in range(2)]
                for c in range(NB // 2):
                    vals = []
                    for b in range(4):
                        r0, cb = (b // 2) * HS + m0, (b % 2) * (NB // 2) + c
                        vals.append((block(r0, cb, 3) - mu[b // 2]) * scale[b // 2])
                        xn[wrows(r0, n), cb * 128:(cb + 1) * 128] = _words(vals[b])
                    terms = _lhs_terms(*vals)
                    for i in range(7):
                        xc.at[i][wrows(m0, n), c * 128:(c + 1) * 128] = _words(terms[i])
                    if paced:
                        pace(xraw, terms[6])

        def transform_qkv(raw, dst, part, nparts, TB=TB, paced=True):
            n = HD // nparts
            for sb in range(n // TB):
                r0 = part * n + sb * TB
                words = yield from _to_head_lanes([
                    jnp.concatenate([pltpu.bitcast(raw[rows_at(half * HD + r0, TB), c * 128:(c + 1) * 128], u32)
                                     for half in range(2)], axis=0) for c in range(NB)])
                yield
                top = [_halves(w[:TB // 2]).astype(f32) for w in words]
                bot = [_halves(w[TB // 2:]).astype(f32) for w in words]
                for c in range(NB // 2):
                    terms = _rhs_terms(top[c], top[c + NB // 2], bot[c], bot[c + NB // 2])
                    for i in range(7):
                        dst.at[i][wrows(r0, TB), c * 128:(c + 1) * 128] = _words(terms[i])
                if paced:
                    pace(raw, terms[6])

        def two_level(block, terms_of, store, wait_for):
            for i in range(7):
                inner = terms_of(*[terms_of(*[block(p, q) for p in range(4)])[i] for q in range(4)])
                for j in range(7):
                    store(7 * i + j, _words(inner[j]))
                wait_for(inner[6])

        def transform2(raw, dst, part, nparts):
            n = QD // nparts
            for sb in range(n // PR):
                r0 = part * n + sb * PR
                for z in range(2):
                    def block(p, q):
                        kq, nq_ = 2 * (p // 2) + q // 2, 2 * (p % 2) + q % 2
                        return widen(raw, z, rows_at(kq * QD + r0, PR), slice(nq_ * 128, (nq_ + 1) * 128))

                    def store(i, w):
                        dst.at[i][wrows(r0, PR), z * 128:(z + 1) * 128] = w
                    two_level(block, _rhs_terms, store, functools.partial(pace, raw.at[z]))

        def transform_down(raw, dst, part, nparts):
            n = FC // 4 // nparts
            for sb in range(n // PR):
                r0 = part * n + sb * PR
                for c in range(QD // 128):
                    def block(p, q):
                        kq, nq_ = 2 * (p // 2) + q // 2, 2 * (p % 2) + q % 2
                        cols = slice(nq_ * QD + c * 128, nq_ * QD + (c + 1) * 128)
                        return widen(raw, rows_at(kq * (FC // 4) + r0, PR), cols)

                    def store(i, w):
                        dst.at[i][wrows(r0, PR), c * 128:(c + 1) * 128] = w
                    two_level(block, _rhs_terms, store, functools.partial(pace, raw))

        def transform_out(raw, tmp, dst, part, nparts):
            n = 8 // nparts
            low = lax.broadcasted_iota(jnp.int32, (8, 128), 0) < 4

            def wait_for(v):
                tmp[pl.ds(pl.multiple_of(32 + zeros[1], 8), 8), 0:128] = _words(v)
            for sb in range(n):
                g = part * n + sb
                for d2 in range(2):
                    for kq in range(4):
                        r = (g & 1) * 512 + (g >> 1) * 32 + kq * 8
                        for c in range(NB):
                            cols = slice(c * 128, (c + 1) * 128)
                            rows = []
                            for h3 in range(2):
                                u = raw[rows_at(r + h3 * 256, 8), cols].astype(f32)
                                v = raw[rows_at(r + h3 * 256 + 128, 8), cols].astype(f32)
                                rows.append(jnp.where(low, pltpu.roll(u, 4, 0), v) if d2
                                            else jnp.where(low, u, pltpu.roll(v, 4, 0)))
                            tmp[kq * 8:(kq + 1) * 8, cols] = _words(jnp.concatenate(rows, axis=0))
                            if c % 4 == 3:
                                pace(raw, rows[1])
                    for c in range(QD // 128):
                        def block(p, q):
                            kq, nq_ = 2 * (p // 2) + q // 2, 2 * (p % 2) + q % 2
                            cols = slice(nq_ * QD + c * 128, nq_ * QD + (c + 1) * 128)
                            return _halves(tmp[pl.ds(pl.multiple_of(kq * 8 + zero, 8), 8), cols]).astype(f32)

                        def store(i, w):
                            dst.at[i][wrows(d2 * 128 + g * PR, PR), c * 128:(c + 1) * 128] = w
                        two_level(block, _rhs_terms, store, wait_for)

        def expand_x(xn, part, nparts):
            n = QS // nparts
            for sb in range(n // PR):
                m0 = part * n + sb * PR
                for c in range(QD // 128):
                    def block(p, q):
                        mq, kq = 2 * (p // 2) + q // 2, 2 * (p % 2) + q % 2
                        cols = slice(kq * QD + c * 128, kq * QD + (c + 1) * 128)
                        return _halves(xn[wrows(mq * QS + m0, PR), cols]).astype(f32)

                    def store(i, w):
                        xc2.at[i][wrows(m0, PR), c * 128:(c + 1) * 128] = w

                    def wait_for(v):
                        xn[pl.ds(pl.multiple_of(S // 2 + zero, 8), 8), 0:128] = _words(v)
                    two_level(block, _lhs_terms, store, wait_for)

        def project(lhs, wc, hm, finish, shadow):
            keep, fetch = kept(pproj, hm)
            for cb in range(NB // 2):
                def product(i):
                    m = _dot(lhs(i, zeros[cb]), _halves(wc[i + zero, :, cb * 128:(cb + 1) * 128]))
                    if (cb, i) == (0, ORDER[0]):
                        shadow(m)
                    return m
                _seven_products(product, keep, fetch, lambda b, v: finish(b, cb, v))

        def project_x(xc, wc, dst, off, t, hm, scale=None, shadow=lambda m: None):
            def finish(b, cb, v):
                dst[(b % 2) * (NB // 2) + cb, pl.ds(hint(off + (b // 2) * HS + t * hm, 8), hm), :] = (
                    v if scale is None else v * scale)
            project(lambda i, z: _halves(xc[i, wrows(t * hm + (0 if isinstance(t, int) else z), hm), :]), wc, hm, finish, shadow)

        def attention(step, groups):
            lane = lax.broadcasted_iota(jnp.int32, (AG, 128), 1)
            row = lax.broadcasted_iota(jnp.int32, (AG, 128), 0)
            for g in groups:
                s0 = pl.multiple_of(jnp.minimum((step * n_att + g) * AG, S), AG)
                q = [qo[c, pl.ds(s0, AG), :] for c in range(NB)]
                logits = []
                for w in range(W):
                    rows = pl.ds(s0 + (HALO - DIL * w), AG)
                    logits.append(functools.reduce(jnp.add, [q[c] * kp[c, rows, :] for c in range(NB)]))
                for d in (1, 2):
                    logits = [p + jnp.where((lane & d) == 0, pltpu.roll(p, 128 - d, 1), pltpu.roll(p, d, 1))
                              for p in logits]
                logits = [jnp.where(row + s0 >= DIL * w, p, -1e9) if g * AG < DIL * w else p
                          for w, p in enumerate(logits)]
                mx = functools.reduce(jnp.maximum, logits)
                es = [jnp.exp(p - mx) for p in logits]
                inv = 1.0 / functools.reduce(jnp.add, es)
                at = [e * inv for e in es]
                for c in range(NB):
                    o = functools.reduce(
                        jnp.add, [at[w] * vp[c, pl.ds(s0 + (HALO - DIL * w), AG), :] for w in range(W)])
                    qo[c, pl.ds(s0, AG), :] = o

        def next_weights(src, slot, t):
            transform2(graw.at[src], gc[slot], t, nf)
            transform_down(draw.at[src], dc[slot], t, nf)

        again = pl.ds(pl.multiple_of(zero, 8), HMF)

        def forty_nine_products(product, finish):
            def outer(i, q, m):
                fetch = lambda k: pout[k][q, again, :]
                if i < 5:
                    pout[i][q] = m
                if i == 1:
                    finish(2, q, fetch(3) + m)
                elif i == 4:
                    finish(1, q, fetch(2) + m)
                elif i == 5:
                    finish(3, q, fetch(2) + fetch(0) - fetch(1) + m)
                elif i == 6:
                    finish(0, q, fetch(3) + fetch(0) - fetch(4) + m)

            keep, fetch = kept(pin, HMF)
            for i in ORDER:
                _seven_products(lambda j: product(7 * i + j), keep, fetch, lambda q, v: outer(i, q, v))

        def ffn(sums, slot, t, started, early, shadow):
            m0 = t * HMF

            def gate(p, q, c):
                h = jax.nn.gelu(c[:, :128], approximate=True) * c[:, 128:]
                if (p, q) != (0, 0):
                    hkeep[p][q] = h
                if (p, q) == GATE_AT:
                    shadow(h[0:8])
                if p in (3, 0) and q in (3, 0):
                    block = lambda pp, qq: h if (pp, qq) == (p, q) else hkeep[pp][qq, again, :]
                    for i in ((1, 3, 6) if p else (0, 2, 4, 5)):
                        for j in ((1, 3, 6) if q else (0, 2, 4, 5)):
                            hc[i].at[j][...] = _words(_lhs_term(
                                j, lambda qq: _lhs_term(i, lambda pp: block(pp, qq))))

            def product(k):
                m = _dot(_halves(xc2[k, wrows(m0, HMF), :]), _halves(gc[slot][k]))
                if k == EARLY_AT:
                    early(m[0:8, 0:128])
                return m
            forty_nine_products(product, gate)

            for first in ((1, 3, 6), (0, 2, 4, 5)):
                for second in ((1, 3, 6), (0, 2, 4, 5)):
                    for i in first:
                        for j in second:
                            lhs = hc[i][j, pl.ds(pl.multiple_of(zero, 8), HMF // 2), :]
                            rows = rows_at(m0, HMF)
                            sums[i][j, rows, :] = (jnp.where(started, sums[i][j, rows, :], 0.0)
                                                   + _dot(_halves(lhs), _halves(dc[slot][7 * i + j])))

        def out_operands(dst, t, paced):
            for sb in range(HMF // PR):
                for c in range(QD // 128):
                    def block(p, q):
                        mq, kq = 2 * (p // 2) + q // 2, 2 * (p % 2) + q % 2
                        return qo[2 * kq + c, rows_at(mq * QS + t * HMF + sb * PR, PR), :]

                    def store(k, w):
                        dst.at[k][wrows(sb * PR, PR), c * 128:(c + 1) * 128] = w

                    def wait_for(v):
                        if paced:
                            qo[0, pl.ds(pl.multiple_of(S + AG + zeros[1], 8), 8), :] = v[0:8]
                    two_level(block, _lhs_terms, store, wait_for)

        def out_proj(sums, operands, t, shadow):
            m0 = t * HMF

            def window(p, q):
                return (rows_at((2 * (p // 2) + q // 2) * QS + m0, HMF), pl.ds((2 * (p % 2) + q % 2) * QD, QD))

            def finish(p, q, v):
                xraw[window(p, q)] = (xraw[window(p, q)].astype(f32) + v).astype(bf16)
                pltpu.make_async_copy(xraw.at[window(p, q)], out_hbm.at[window(p, q)], osem).start()

            def product(k):
                m = _dot(_halves(operands[k, pl.ds(pl.multiple_of(zero, 8), HMF // 2), :]), _halves(wc3[k]))
                if k == 7 * ORDER[0] + ORDER[0]:
                    shadow(m[0:8, 0:128])
                return m + sums[k // 7][k % 7, rows_at(m0, HMF), :]
            forty_nine_products(product, finish)

        def projections(xc, xn, mean, inv, tmp, wraw, wc0, wc1, wc2):
            def w_copies(p):
                src = wo_hbm if p == 3 else wqkv_hbm.at[:, p * D:(p + 1) * D]
                return [pltpu.make_async_copy(src, wraw.at[p, pl.ds(0, D), :], wsem.at[p])]

            def wq_copies(i):
                rows = [rows_at(half * HD + i * (HD // NP), HD // NP) for half in range(2)]
                return [pltpu.make_async_copy(wqkv_hbm.at[r, pl.ds(0, D)], wraw.at[0, r, :], qsem.at[i]) for r in rows]

            with scope("prologue"):
                start(x_copies(0))
                lax.fori_loop(0, NP, lambda i, _: start(wq_copies(i)), None)
                lax.fori_loop(1, n0, lambda t, _: start(x_copies(t)), None)
                start(w_copies(1))
                for c in range(NB):
                    kp[c, 0:HALO, :] = jnp.zeros((HALO, 128), f32)
                    kp[c, HALO + S:HALO + S + AG, :] = jnp.zeros((AG, 128), f32)
                    vp[c, HALO + S:HALO + S + AG, :] = jnp.zeros((AG, 128), f32)
                    qo[c, S:S + AG, :] = jnp.zeros((AG, 128), f32)
                with scope("wait_x0"):
                    wait(x_copies(0))

                def first_body(i, _):
                    wait(wq_copies(i))
                    _run(*[transform_qkv(wraw.at[0], wc0, i * TW + k, NP * TW, TB0, paced=False) for k in range(TW)],
                         layernorm(xc, xn, mean, inv, i * (HM0 // NP), HM0 // NP, PR, paced=False))
                lax.fori_loop(0, NP, first_body, None)
                start(w_copies(2))

            with scope("qphase"):
                for lo, hi in zip(QSTOPS, QSTOPS[1:] + (n0,)):
                    with scope(f"wait_x{lo}"):
                        for t in range(lo + 1, min(hi + 1, n0)):
                            wait(x_copies(t))
                    if hi == n0:
                        with scope(f"wait_wk"):
                            wait(w_copies(1))
                        start(w_copies(3))
                        start(f_copies(0, 0))
                    for t in range(lo, hi):
                        def shadow(token):
                            if t + 1 < n0:
                                pace(xraw, token)
                                _run(layernorm(xc, xn, mean, inv, (t + 1) * HM0, HM0, LB))
                        project_x(xc, wc0, qo, 0, t, HM0, DH ** -0.5, shadow)
                _run(transform_qkv(wraw.at[1], wc1, 0, 1))

            wait(w_copies(2))
            wait(w_copies(3))
            start(f_copies(1, 1))

            def k_body(t, _):
                project_x(xc, wc1, kp, HALO, t, HMQ)
                transform_out(wraw.at[3], tmp, wc3, t, nq)
                _run(transform_qkv(wraw.at[2], wc2, t, nq))
            with scope("kphase"):
                lax.fori_loop(0, nq, k_body, None)

            wait(f_copies(0, 0))

            def v_body(t, _):
                project_x(xc, wc2, vp, HALO, t, HMQ)
                expand_x(xn, t, nq)
                transform2(graw.at[0], gc0, t, nq)
                transform_down(draw.at[0], dc0, t, nq)
            with scope("vphase"):
                lax.fori_loop(0, nq, v_body, None)
            for c in range(NB):
                vp[c, 0:HALO, :] = jnp.broadcast_to(vp[c, HALO:HALO + 1, :], (HALO, 128))

        pl.run_scoped(projections,
                      pltpu.VMEM((7, HS // 2, HD), u32), pltpu.VMEM((S // 2 + 8, D), u32),
                      pltpu.VMEM((S, 128), f32), pltpu.VMEM((S, 128), f32), pltpu.VMEM((40, D), u32), pltpu.VMEM((4, D + PR, D), bf16),
                      *[pltpu.VMEM((7, HD // 2, HD), u32)] * 3)

        def second_half(*sums):
            def chunk_body(j, _):
                src = jnp.minimum(j + 1, NCH - 1) % 2

                @pl.when(j + 1 < NCH)
                def _():
                    wait(f_copies(j + 1, 1 - j % 2))

                @pl.when(j + 2 < NCH)
                def _():
                    start(f_copies(j + 2, j % 2))

                for parity in range(2):
                    @pl.when(j % 2 == parity)
                    def _():
                        def tile_body(t, _):
                            def shadow(groups, token):
                                if len(groups):
                                    qo[0, pl.ds(pl.multiple_of(S + AG + zero, 8), 8), :] = token
                                    attention(j * nf + t, groups)
                            ffn(sums, parity, t, True if parity else j > 0,
                                functools.partial(shadow, range(NE)), functools.partial(shadow, range(NE, n_att)))
                            next_weights(src, 1 - parity, t)
                        lax.fori_loop(0, nf, tile_body, None)
            with scope("ffn"):
                lax.fori_loop(0, NCH, chunk_body, None)

            with scope("ophase"):
                out_operands(gc0, 0, False)

                for t in range(nf):
                    def shadow(token):
                        if t + 1 < nf:
                            qo[0, pl.ds(pl.multiple_of(S + AG + zeros[1], 8), 8), :] = token
                            out_operands(gc[(t + 1) % 2], t + 1, True)
                    out_proj(sums, gc[t % 2], t, shadow)
            with scope("drain"):
                pltpu.make_async_copy(xraw.at[pl.ds(0, S), :], out_hbm, osem).wait()

        pl.run_scoped(second_half, *[pltpu.VMEM((7, QS, QD), f32)] * 7)

    scratch = [
        pltpu.VMEM((S + PR, D), bf16),
        pltpu.VMEM((49, QS // 2, QD), u32),
        pltpu.VMEM((49, QD // 2, QD), u32),
        pltpu.VMEM((49, QD // 2, FC // 2), u32),
        pltpu.VMEM((49, FC // 8, QD), u32),
        pltpu.VMEM((49, QD // 2, FC // 2), u32),
        pltpu.VMEM((49, FC // 8, QD), u32),
        pltpu.VMEM((2, 2, D + PR, FC), bf16),
        pltpu.VMEM((2, FC + PR, D), bf16),
        pltpu.VMEM((NB, S + AG + 8, 128), f32),
        pltpu.VMEM((NB, HALO + S + AG, 128), f32),
        pltpu.VMEM((NB, HALO + S + AG, 128), f32),
        pltpu.SemaphoreType.DMA((n0,)),
        pltpu.SemaphoreType.DMA((NP,)),
        pltpu.SemaphoreType.DMA((4,)),
        pltpu.SemaphoreType.DMA((2,)),
        pltpu.SemaphoreType.DMA(()),
        *[pltpu.VMEM((HMF, 256), f32)] * 5,
        *[pltpu.VMEM((4, HMF, 256), f32)] * 5,
        *[pltpu.VMEM((max(HM0, HMQ), 128), f32)] * 5,
        *[pltpu.VMEM((4, HMF, 128), f32)] * 4,
        *[pltpu.VMEM((7, HMF // 2, 128), u32)] * 7,
    ]
    return kernel, scratch


def make_call(flags=None, **kw):
    kernel, scratch = make_kernel(**kw)
    hbm = pl.BlockSpec(memory_space=pl.ANY)
    return pl.pallas_call(
        kernel,
        in_specs=[pl.BlockSpec(memory_space=pltpu.SMEM)] + [hbm] * 6,
        out_specs=hbm,
        out_shape=jax.ShapeDtypeStruct((S, D), bf16),
        scratch_shapes=scratch,
        compiler_params=pltpu.CompilerParams(vmem_limit_bytes=126 * 1024 * 1024, flags=flags),
    )


@jax.jit
def pallas_parallel_sum__sliding_local_dilated__glu_gated_geglu__prompt_kernel(
    A_x, A_wqkv, A_wo, B_x, B_w_gate, B_w_up, B_w_down
):
    del B_x
    out = make_call()(np.zeros((4,), np.int32), A_x.reshape(S, D), A_wqkv, A_wo, B_w_gate, B_w_up, B_w_down)
    return out.reshape(1, S, D)
```

```python
import functools
import jax
import jax.numpy as jnp
import numpy as np
from jax import lax
import jax.experimental.pallas as pl
import jax.experimental.pallas.tpu as pltpu

S, D, F = 2048, 1024, 3584
H, DH, W, DIL = 32, 32, 8, 2
HALO = 16
NB = D // 128
HS, QS = S // 2, S // 4
HD, QD = D // 2, D // 4
FC = 512
NCH = F // FC
PR = 16
LOG2E = 1.4426950408889634
ORDER = (2, 3, 0, 1, 4, 5, 6)
f32, bf16, u32 = jnp.float32, jnp.bfloat16, jnp.uint32


def _dot(a, b):
    return jnp.dot(a, b, preferred_element_type=f32)


def _words(v):
    return pltpu.bitcast(v.astype(bf16), u32)


def _halves(w):
    return pltpu.bitcast(w, bf16)


def _lhs_terms(a11, a12, a21, a22):
    return [a11 + a22, a21 + a22, a11, a22, a11 + a12, a21 - a11, a12 - a22]


def _lhs_term(i, a):
    return (lambda: a(0) + a(3), lambda: a(2) + a(3), lambda: a(0), lambda: a(3),
            lambda: a(0) + a(1), lambda: a(2) - a(0), lambda: a(1) - a(3))[i]()


def _rhs_terms(b11, b12, b21, b22):
    return [b11 + b22, b11, b12 - b22, b21 - b11, b22, b11 + b12, b21 + b22]


def _seven_products(product, keep, fetch, finish):
    for i in (2, 3, 0):
        keep(i, product(i))
    m = product(1)
    keep(1, m)
    finish(2, fetch(3) + m)
    m = product(4)
    keep(4, m)
    finish(1, fetch(2) + m)
    finish(3, fetch(2) + fetch(0) - fetch(1) + product(5))
    finish(0, fetch(3) + fetch(0) - fetch(4) + product(6))


def _to_head_lanes(blocks):
    slot = lax.broadcasted_iota(jnp.int32, blocks[0].shape, 1) >> 2
    blocks = [pltpu.roll(b, 4 * c, 1) if c else b for c, b in enumerate(blocks)]
    yield
    blocks = [blocks[-j % NB] for j in range(NB)]
    for bit in (1, 2, 4):
        move = (slot & bit) != 0
        blocks = [jnp.where(move, blocks[(j - bit) % NB], blocks[j]) for j in range(NB)]
    return [pltpu.roll(b, 128 - 4 * j, 1) if j else b for j, b in enumerate(blocks)]


def _run(*stages):
    stages = list(stages)
    while stages:
        stages = [g for g in stages if next(g, True) is None]


def make_kernel(HM0=128, HMQ=512, HMF=128, AG=8, LB=16, TB=32, NP=4, TB0=16, TW=4, QSTOPS=(0, 1, 3), GATE_AT=(0, 0), NCH=NCH, scopes=False, PRIO=0, NE=(6, 4), EARLY_AT=2, RC=False):
    n0, nq, nf = HS // HM0, HS // HMQ, QS // HMF
    n_att = (10, 8)
    assert nf * (n_att[0] * ((NCH + 1) // 2) + n_att[1] * (NCH // 2)) * AG == S

    def kernel(zero_ref, x_hbm, wqkv_hbm, wo_hbm, wg_hbm, wu_hbm, wd_hbm, out_hbm,
               xraw, xc2, wc3, gc0, dc0, gc1, dc1, graw, draw, qo, kp, vp,
               xsem, qsem, wsem, fsem, osem, *work):
        gc, dc = (gc0, gc1), (dc0, dc1)
        pin, pout, pproj, hkeep, hc = work[0:5], work[5:10], work[10:15], work[15:19], work[19:26]
        zeros = [zero_ref[k] for k in range(4)]
        zero = zeros[0]

        def x_copies(t):
            rows = [rows_at(half * HS + t * HM0, HM0) for half in range(2)]
            return [pltpu.make_async_copy(x_hbm.at[r, :], xraw.at[r, :], xsem.at[t]) for r in rows]

        def f_copies(j, slot):
            cols = pl.ds(pl.multiple_of(j * FC, FC), FC)
            return [pltpu.make_async_copy(wg_hbm.at[:, cols], graw.at[slot, 0, pl.ds(0, D), :], fsem.at[slot]),
                    pltpu.make_async_copy(wu_hbm.at[:, cols], graw.at[slot, 1, pl.ds(0, D), :], fsem.at[slot]),
                    pltpu.make_async_copy(wd_hbm.at[cols, :], draw.at[slot, pl.ds(0, FC), :], fsem.at[slot])]

        import contextlib
        scope = jax.named_scope if scopes else (lambda name: contextlib.nullcontext())

        def start(cps):
            for cp in cps:
                cp.start(priority=PRIO)

        def wait(cps):
            for cp in cps:
                cp.wait()

        def hint(i, n):
            return i if isinstance(i, int) else pl.multiple_of(i, n)

        def rows_at(r0, n):
            return pl.ds(r0 if isinstance(r0, int) else pl.multiple_of(r0, n), n)

        def wrows(r0, n):
            return pl.ds(r0 // 2 if isinstance(r0, int) else pl.multiple_of(r0 // 2, 8), n // 2)

        def pace(raw, value):
            spare = raw.shape[0] - PR
            raw[pl.ds(pl.multiple_of(spare + zeros[1], 8), 8), 0:128] = value[0:8].astype(bf16)

        def widen(ref, *idx):
            return _halves(pltpu.bitcast(ref[idx], u32)).astype(f32)

        def kept(bufs, n):
            def keep(i, v):
                bufs[i][0:n, :] = v
            return keep, lambda i: bufs[i][pl.ds(pl.multiple_of(zero, 8), n), :]

        def layernorm(xc, xn, mean, inv, first, count, n, paced=True):
            def block(r0, c, z):
                return widen(xraw, rows_at(r0 + zeros[z], n), slice(c * 128, (c + 1) * 128))

            def row_mean(vals):
                total = functools.reduce(jnp.add, vals)
                if paced:
                    pace(xraw, total)
                return jnp.broadcast_to(jnp.sum(total, axis=-1, keepdims=True) * (1.0 / D), (n, 128))

            def stat(ref, r0):
                return ref[rows_at(r0 + zero, n), :]

            pieces = [first + k for k in range(0, count, n)]
            starts = [half * HS + m0 for m0 in pieces for half in range(2)]
            for r0 in starts:
                mean[rows_at(r0, n), :] = row_mean([block(r0, c, 0) for c in range(NB)])
            yield
            for r0 in starts:
                mu = stat(mean, r0)
                inv[rows_at(r0, n), :] = lax.rsqrt(
                    row_mean([jnp.square(block(r0, c, 2) - mu) for c in range(NB)]) + 1e-5)
            yield
            for m0 in pieces:
                mu = [stat(mean, half * HS + m0) for half in range(2)]
                scale = [stat(inv, half * HS + m0) for half in range(2)]
                for c in range(NB // 2):
                    vals = []
                    for b in range(4):
                        r0, cb = (b // 2) * HS + m0, (b % 2) * (NB // 2) + c
                        vals.append((block(r0, cb, 3) - mu[b // 2]) * scale[b // 2])
                        xn[wrows(r0, n), cb * 128:(cb + 1) * 128] = _words(vals[b])
                    terms = _lhs_terms(*vals)
                    for i in range(7):
                        xc.at[i][wrows(m0, n), c * 128:(c + 1) * 128] = _words(terms[i])
                    if paced:
                        pace(xraw, terms[6])

        def transform_qkv(raw, dst, part, nparts, TB=TB, paced=True):
            n = HD // nparts
            for sb in range(n // TB):
                r0 = part * n + sb * TB
                words = yield from _to_head_lanes([
                    jnp.concatenate([pltpu.bitcast(raw[rows_at(half * HD + r0, TB), c * 128:(c + 1) * 128], u32)
                                     for half in range(2)], axis=0) for c in range(NB)])
                yield
                top = [_halves(w[:TB // 2]).astype(f32) for w in words]
                bot = [_halves(w[TB // 2:]).astype(f32) for w in words]
                for c in range(NB // 2):
                    terms = _rhs_terms(top[c], top[c + NB // 2], bot[c], bot[c + NB // 2])
                    for i in range(7):
                        dst.at[i][wrows(r0, TB), c * 128:(c + 1) * 128] = _words(terms[i])
                if paced:
                    pace(raw, terms[6])

        def two_level(block, terms_of, store, wait_for):
            for i in range(7):
                inner = terms_of(*[terms_of(*[block(p, q) for p in range(4)])[i] for q in range(4)])
                for j in range(7):
                    store(7 * i + j, _words(inner[j]))
                wait_for(inner[6])

        def transform2(raw, dst, part, nparts):
            n = QD // nparts
            for sb in range(n // PR):
                r0 = part * n + sb * PR
                for z in range(2):
                    def block(p, q):
                        kq, nq_ = 2 * (p // 2) + q // 2, 2 * (p % 2) + q % 2
                        return widen(raw, z, rows_at(kq * QD + r0, PR), slice(nq_ * 128, (nq_ + 1) * 128))

                    def store(i, w):
                        dst.at[i][wrows(r0, PR), z * 128:(z + 1) * 128] = w
                    two_level(block, _rhs_terms, store, functools.partial(pace, raw.at[z]))

        def transform_down(raw, dst, part, nparts):
            n = FC // 4 // nparts
            for sb in range(n // PR):
                r0 = part * n + sb * PR
                for c in range(QD // 128):
                    def block(p, q):
                        kq, nq_ = 2 * (p // 2) + q // 2, 2 * (p % 2) + q % 2
                        cols = slice(nq_ * QD + c * 128, nq_ * QD + (c + 1) * 128)
                        return widen(raw, rows_at(kq * (FC // 4) + r0, PR), cols)

                    def store(i, w):
                        dst.at[i][wrows(r0, PR), c * 128:(c + 1) * 128] = w
                    two_level(block, _rhs_terms, store, functools.partial(pace, raw))

        def transform_out(raw, tmp, dst, part, nparts):
            n = 8 // nparts
            low = lax.broadcasted_iota(jnp.int32, (8, 128), 0) < 4

            def wait_for(v):
                tmp[pl.ds(pl.multiple_of(32 + zeros[1], 8), 8), 0:128] = _words(v)
            for sb in range(n):
                g = part * n + sb
                for d2 in range(2):
                    for kq in range(4):
                        r = (g & 1) * 512 + (g >> 1) * 32 + kq * 8
                        for c in range(NB):
                            cols = slice(c * 128, (c + 1) * 128)
                            rows = []
                            for h3 in range(2):
                                u = raw[rows_at(r + h3 * 256, 8), cols].astype(f32)
                                v = raw[rows_at(r + h3 * 256 + 128, 8), cols].astype(f32)
                                rows.append(jnp.where(low, pltpu.roll(u, 4, 0), v) if d2
                                            else jnp.where(low, u, pltpu.roll(v, 4, 0)))
                            tmp[kq * 8:(kq + 1) * 8, cols] = _words(jnp.concatenate(rows, axis=0))
                            if c % 4 == 3:
                                pace(raw, rows[1])
                    for c in range(QD // 128):
                        def block(p, q):
                            kq, nq_ = 2 * (p // 2) + q // 2, 2 * (p % 2) + q % 2
                            cols = slice(nq_ * QD + c * 128, nq_ * QD + (c + 1) * 128)
                            return _halves(tmp[pl.ds(pl.multiple_of(kq * 8 + zero, 8), 8), cols]).astype(f32)

                        def store(i, w):
                            dst.at[i][wrows(d2 * 128 + g * PR, PR), c * 128:(c + 1) * 128] = w
                        two_level(block, _rhs_terms, store, wait_for)

        def expand_x(xn, part, nparts):
            n = QS // nparts
            for sb in range(n // PR):
                m0 = part * n + sb * PR
                for c in range(QD // 128):
                    def block(p, q):
                        mq, kq = 2 * (p // 2) + q // 2, 2 * (p % 2) + q % 2
                        cols = slice(kq * QD + c * 128, kq * QD + (c + 1) * 128)
                        return _halves(xn[wrows(mq * QS + m0, PR), cols]).astype(f32)

                    def store(i, w):
                        xc2.at[i][wrows(m0, PR), c * 128:(c + 1) * 128] = w

                    def wait_for(v):
                        xn[pl.ds(pl.multiple_of(S // 2 + zero, 8), 8), 0:128] = _words(v)
                    two_level(block, _lhs_terms, store, wait_for)

        def project(lhs, wc, hm, finish, shadow):
            keep, fetch = kept(pproj, hm)
            for cb in range(NB // 2):
                def product(i):
                    m = _dot(lhs(i, zeros[cb]), _halves(wc[i + zero, :, cb * 128:(cb + 1) * 128]))
                    if (cb, i) == (0, ORDER[0]):
                        shadow(m)
                    return m
                _seven_products(product, keep, fetch, lambda b, v: finish(b, cb, v))

        def project_x(xc, wc, dst, off, t, hm, scale=None, shadow=lambda m: None):
            def finish(b, cb, v):
                dst[(b % 2) * (NB // 2) + cb, pl.ds(hint(off + (b // 2) * HS + t * hm, 8), hm), :] = (
                    v if scale is None else v * scale)
            project(lambda i, z: _halves(xc[i, wrows(t * hm + (0 if isinstance(t, int) else z), hm), :]), wc, hm, finish, shadow)

        def attention(first, groups):
            lane = lax.broadcasted_iota(jnp.int32, (AG, 128), 1)
            row = lax.broadcasted_iota(jnp.int32, (AG, 128), 0)
            for g in groups:
                s0 = pl.multiple_of((first + g) * AG + zeros[2 + g % 2], AG)
                q = [qo[c, pl.ds(s0, AG), :] for c in range(NB)]
                logits = []
                for w in range(W):
                    rows = pl.ds(s0 + (HALO - DIL * w), AG)
                    logits.append(functools.reduce(jnp.add, [q[c] * kp[c, rows, :] for c in range(NB)]))
                for d in (1, 2):
                    logits = [p + jnp.where((lane & d) == 0, pltpu.roll(p, 128 - d, 1), pltpu.roll(p, d, 1))
                              for p in logits]
                logits = [jnp.where(row + s0 >= DIL * w, p, -1e9 * LOG2E) if g * AG < DIL * w else p
                          for w, p in enumerate(logits)]
                mx = functools.reduce(jnp.maximum, logits)
                es = [jnp.exp2(p - mx) for p in logits]
                inv = pl.reciprocal(functools.reduce(jnp.add, es), approx=False) if RC else 1.0 / functools.reduce(jnp.add, es)
                at = [e * inv for e in es]
                for c in range(NB):
                    o = functools.reduce(
                        jnp.add, [at[w] * vp[c, pl.ds(s0 + (HALO - DIL * w), AG), :] for w in range(W)])
                    qo[c, pl.ds(s0, AG), :] = o

        def next_weights(src, slot, t):
            transform2(graw.at[src], gc[slot], t, nf)
            transform_down(draw.at[src], dc[slot], t, nf)

        again = pl.ds(pl.multiple_of(zero, 8), HMF)

        def forty_nine_products(product, finish):
            def outer(i, q, m):
                fetch = lambda k: pout[k][q, again, :]
                if i < 5:
                    pout[i][q] = m
                if i == 1:
                    finish(2, q, fetch(3) + m)
                elif i == 4:
                    finish(1, q, fetch(2) + m)
                elif i == 5:
                    finish(3, q, fetch(2) + fetch(0) - fetch(1) + m)
                elif i == 6:
                    finish(0, q, fetch(3) + fetch(0) - fetch(4) + m)

            keep, fetch = kept(pin, HMF)
            for i in ORDER:
                _seven_products(lambda j: product(7 * i + j), keep, fetch, lambda q, v: outer(i, q, v))

        def ffn(sums, slot, t, started, early, shadow):
            m0 = t * HMF

            def gate(p, q, c):
                h = jax.nn.gelu(c[:, :128], approximate=True) * c[:, 128:]
                if (p, q) != (0, 0):
                    hkeep[p][q] = h
                if (p, q) == GATE_AT:
                    shadow(h[0:8])
                if p in (3, 0) and q in (3, 0):
                    block = lambda pp, qq: h if (pp, qq) == (p, q) else hkeep[pp][qq, again, :]
                    for i in ((1, 3, 6) if p else (0, 2, 4, 5)):
                        for j in ((1, 3, 6) if q else (0, 2, 4, 5)):
                            hc[i].at[j][...] = _words(_lhs_term(
                                j, lambda qq: _lhs_term(i, lambda pp: block(pp, qq))))

            def product(k):
                m = _dot(_halves(xc2[k, wrows(m0, HMF), :]), _halves(gc[slot][k]))
                if k == EARLY_AT:
                    early(m[0:8, 0:128])
                return m
            forty_nine_products(product, gate)

            for first in ((1, 3, 6), (0, 2, 4, 5)):
                for second in ((1, 3, 6), (0, 2, 4, 5)):
                    for i in first:
                        for j in second:
                            lhs = hc[i][j, pl.ds(pl.multiple_of(zero, 8), HMF // 2), :]
                            rows = rows_at(m0, HMF)
                            sums[i][j, rows, :] = (jnp.where(started, sums[i][j, rows, :], 0.0)
                                                   + _dot(_halves(lhs), _halves(dc[slot][7 * i + j])))

        def out_operands(dst, t, paced):
            for sb in range(HMF // PR):
                for c in range(QD // 128):
                    def block(p, q):
                        mq, kq = 2 * (p // 2) + q // 2, 2 * (p % 2) + q % 2
                        return qo[2 * kq + c, rows_at(mq * QS + t * HMF + sb * PR, PR), :]

                    def store(k, w):
                        dst.at[k][wrows(sb * PR, PR), c * 128:(c + 1) * 128] = w

                    def wait_for(v):
                        if paced:
                            qo[0, pl.ds(pl.multiple_of(S + zeros[1], 8), 8), :] = v[0:8]
                    two_level(block, _lhs_terms, store, wait_for)

        def out_proj(sums, operands, t, shadow):
            m0 = t * HMF

            def window(p, q):
                return (rows_at((2 * (p // 2) + q // 2) * QS + m0, HMF), pl.ds((2 * (p % 2) + q % 2) * QD, QD))

            def finish(p, q, v):
                xraw[window(p, q)] = (xraw[window(p, q)].astype(f32) + v).astype(bf16)
                pltpu.make_async_copy(xraw.at[window(p, q)], out_hbm.at[window(p, q)], osem).start()

            def product(k):
                m = _dot(_halves(operands[k, pl.ds(pl.multiple_of(zero, 8), HMF // 2), :]), _halves(wc3[k]))
                if k == 7 * ORDER[0] + ORDER[0]:
                    shadow(m[0:8, 0:128])
                return m + sums[k // 7][k % 7, rows_at(m0, HMF), :]
            forty_nine_products(product, finish)

        def projections(xc, xn, mean, inv, tmp, wraw, wc0, wc1, wc2):
            def w_copies(p):
                src = wo_hbm if p == 3 else wqkv_hbm.at[:, p * D:(p + 1) * D]
                return [pltpu.make_async_copy(src, wraw.at[p, pl.ds(0, D), :], wsem.at[p])]

            def wq_copies(i):
                rows = [rows_at(half * HD + i * (HD // NP), HD // NP) for half in range(2)]
                return [pltpu.make_async_copy(wqkv_hbm.at[r, pl.ds(0, D)], wraw.at[0, r, :], qsem.at[i]) for r in rows]

            with scope("prologue"):
                start(x_copies(0))
                lax.fori_loop(0, NP, lambda i, _: start(wq_copies(i)), None)
                lax.fori_loop(1, n0, lambda t, _: start(x_copies(t)), None)
                start(w_copies(1))
                for c in range(NB):
                    kp[c, 0:HALO, :] = jnp.zeros((HALO, 128), f32)
                with scope("wait_x0"):
                    wait(x_copies(0))

                def first_body(i, _):
                    wait(wq_copies(i))
                    _run(*[transform_qkv(wraw.at[0], wc0, i * TW + k, NP * TW, TB0, paced=False) for k in range(TW)],
                         layernorm(xc, xn, mean, inv, i * (HM0 // NP), HM0 // NP, PR, paced=False))
                lax.fori_loop(0, NP, first_body, None)
                start(w_copies(2))

            with scope("qphase"):
                for lo, hi in zip(QSTOPS, QSTOPS[1:] + (n0,)):
                    with scope(f"wait_x{lo}"):
                        for t in range(lo + 1, min(hi + 1, n0)):
                            wait(x_copies(t))
                    if hi == n0:
                        with scope(f"wait_wk"):
                            wait(w_copies(1))
                        start(w_copies(3))
                        start(f_copies(0, 0))
                    for t in range(lo, hi):
                        def shadow(token):
                            if t + 1 < n0:
                                pace(xraw, token)
                                _run(layernorm(xc, xn, mean, inv, (t + 1) * HM0, HM0, LB))
                        project_x(xc, wc0, qo, 0, t, HM0, DH ** -0.5 * LOG2E, shadow)
                _run(transform_qkv(wraw.at[1], wc1, 0, 1))

            wait(w_copies(2))
            wait(w_copies(3))
            start(f_copies(1, 1))

            def k_body(t, _):
                project_x(xc, wc1, kp, HALO, t, HMQ)
                transform_out(wraw.at[3], tmp, wc3, t, nq)
                _run(transform_qkv(wraw.at[2], wc2, t, nq))
            with scope("kphase"):
                lax.fori_loop(0, nq, k_body, None)

            wait(f_copies(0, 0))

            def v_body(t, _):
                project_x(xc, wc2, vp, HALO, t, HMQ)
                expand_x(xn, t, nq)
                transform2(graw.at[0], gc0, t, nq)
                transform_down(draw.at[0], dc0, t, nq)
            with scope("vphase"):
                lax.fori_loop(0, nq, v_body, None)
            for c in range(NB):
                vp[c, 0:HALO, :] = jnp.broadcast_to(vp[c, HALO:HALO + 1, :], (HALO, 128))

        pl.run_scoped(projections,
                      pltpu.VMEM((7, HS // 2, HD), u32), pltpu.VMEM((S // 2 + 8, D), u32),
                      pltpu.VMEM((S, 128), f32), pltpu.VMEM((S, 128), f32), pltpu.VMEM((40, D), u32), pltpu.VMEM((4, D + PR, D), bf16),
                      *[pltpu.VMEM((7, HD // 2, HD), u32)] * 3)

        def second_half(*sums):
            def chunk_body(j, _):
                src = jnp.minimum(j + 1, NCH - 1) % 2

                @pl.when(j + 1 < NCH)
                def _():
                    wait(f_copies(j + 1, 1 - j % 2))

                @pl.when(j + 2 < NCH)
                def _():
                    start(f_copies(j + 2, j % 2))

                for parity in range(2):
                    @pl.when(j % 2 == parity)
                    def _():
                        def tile_body(t, _):
                            first = nf * (n_att[0] * ((j + 1) // 2) + n_att[1] * (j // 2)) + t * n_att[parity]
                            def shadow(groups, token):
                                if len(groups):
                                    qo[0, pl.ds(pl.multiple_of(S + zero, 8), 8), :] = token
                                    attention(first, groups)
                            ffn(sums, parity, t, True if parity else j > 0,
                                functools.partial(shadow, range(NE[parity])),
                                functools.partial(shadow, range(NE[parity], n_att[parity])))
                            next_weights(src, 1 - parity, t)
                        lax.fori_loop(0, nf, tile_body, None)
            with scope("ffn"):
                lax.fori_loop(0, NCH, chunk_body, None)

            with scope("ophase"):
                out_operands(gc0, 0, False)

                for t in range(nf):
                    def shadow(token):
                        if t + 1 < nf:
                            qo[0, pl.ds(pl.multiple_of(S + zeros[1], 8), 8), :] = token
                            out_operands(gc[(t + 1) % 2], t + 1, True)
                    out_proj(sums, gc[t % 2], t, shadow)
            with scope("drain"):
                pltpu.make_async_copy(xraw.at[pl.ds(0, S), :], out_hbm, osem).wait()

        pl.run_scoped(second_half, *[pltpu.VMEM((7, QS, QD), f32)] * 7)

    scratch = [
        pltpu.VMEM((S + PR, D), bf16),
        pltpu.VMEM((49, QS // 2, QD), u32),
        pltpu.VMEM((49, QD // 2, QD), u32),
        pltpu.VMEM((49, QD // 2, FC // 2), u32),
        pltpu.VMEM((49, FC // 8, QD), u32),
        pltpu.VMEM((49, QD // 2, FC // 2), u32),
        pltpu.VMEM((49, FC // 8, QD), u32),
        pltpu.VMEM((2, 2, D + PR, FC), bf16),
        pltpu.VMEM((2, FC + PR, D), bf16),
        pltpu.VMEM((NB, S + 8, 128), f32),
        pltpu.VMEM((NB, HALO + S + 8, 128), f32),
        pltpu.VMEM((NB, HALO + S + 8, 128), f32),
        pltpu.SemaphoreType.DMA((n0,)),
        pltpu.SemaphoreType.DMA((NP,)),
        pltpu.SemaphoreType.DMA((4,)),
        pltpu.SemaphoreType.DMA((2,)),
        pltpu.SemaphoreType.DMA(()),
        *[pltpu.VMEM((HMF, 256), f32)] * 5,
        *[pltpu.VMEM((4, HMF, 256), f32)] * 5,
        *[pltpu.VMEM((max(HM0, HMQ), 128), f32)] * 5,
        *[pltpu.VMEM((4, HMF, 128), f32)] * 4,
        *[pltpu.VMEM((7, HMF // 2, 128), u32)] * 7,
    ]
    return kernel, scratch


def make_call(flags=None, **kw):
    kernel, scratch = make_kernel(**kw)
    hbm = pl.BlockSpec(memory_space=pl.ANY)
    return pl.pallas_call(
        kernel,
        in_specs=[pl.BlockSpec(memory_space=pltpu.SMEM)] + [hbm] * 6,
        out_specs=hbm,
        out_shape=jax.ShapeDtypeStruct((S, D), bf16),
        scratch_shapes=scratch,
        compiler_params=pltpu.CompilerParams(vmem_limit_bytes=126 * 1024 * 1024, flags=flags),
    )


@jax.jit
def pallas_parallel_sum__sliding_local_dilated__glu_gated_geglu__prompt_kernel(
    A_x, A_wqkv, A_wo, B_x, B_w_gate, B_w_up, B_w_down
):
    del B_x
    out = make_call()(np.zeros((4,), np.int32), A_x.reshape(S, D), A_wqkv, A_wo, B_w_gate, B_w_up, B_w_down)
    return out.reshape(1, S, D)
```

```python
import functools
import jax
import jax.numpy as jnp
import numpy as np
from jax import lax
import jax.experimental.pallas as pl
import jax.experimental.pallas.tpu as pltpu

S, D, F = 2048, 1024, 3584
H, DH, W, DIL = 32, 32, 8, 2
HALO = 16
NB = D // 128
HS, QS = S // 2, S // 4
HD, QD = D // 2, D // 4
FC = 512
NCH = F // FC
PR = 16
LOG2E = 1.4426950408889634
ORDER = (2, 3, 0, 1, 4, 5, 6)
f32, bf16, u32 = jnp.float32, jnp.bfloat16, jnp.uint32


def _dot(a, b):
    return jnp.dot(a, b, preferred_element_type=f32)


def _words(v):
    return pltpu.bitcast(v.astype(bf16), u32)


def _halves(w):
    return pltpu.bitcast(w, bf16)


def _lhs_terms(a11, a12, a21, a22):
    return [a11 + a22, a21 + a22, a11, a22, a11 + a12, a21 - a11, a12 - a22]


def _lhs_term(i, a):
    return (lambda: a(0) + a(3), lambda: a(2) + a(3), lambda: a(0), lambda: a(3),
            lambda: a(0) + a(1), lambda: a(2) - a(0), lambda: a(1) - a(3))[i]()


def _rhs_terms(b11, b12, b21, b22):
    return [b11 + b22, b11, b12 - b22, b21 - b11, b22, b11 + b12, b21 + b22]


def _seven_products(product, keep, fetch, finish):
    for i in (2, 3, 0):
        keep(i, product(i))
    m = product(1)
    keep(1, m)
    finish(2, fetch(3) + m)
    m = product(4)
    keep(4, m)
    finish(1, fetch(2) + m)
    finish(3, fetch(2) + fetch(0) - fetch(1) + product(5))
    finish(0, fetch(3) + fetch(0) - fetch(4) + product(6))


def _to_head_lanes(blocks):
    slot = lax.broadcasted_iota(jnp.int32, blocks[0].shape, 1) >> 2
    blocks = [pltpu.roll(b, 4 * c, 1) if c else b for c, b in enumerate(blocks)]
    yield
    blocks = [blocks[-j % NB] for j in range(NB)]
    for bit in (1, 2, 4):
        move = (slot & bit) != 0
        blocks = [jnp.where(move, blocks[(j - bit) % NB], blocks[j]) for j in range(NB)]
    return [pltpu.roll(b, 128 - 4 * j, 1) if j else b for j, b in enumerate(blocks)]


def _run(*stages):
    stages = list(stages)
    while stages:
        stages = [g for g in stages if next(g, True) is None]


def make_kernel(HM0=128, HMQ=512, HMF=128, AG=8, LB=16, TB=32, NP=4, TB0=16, TW=4, QSTOPS=(0, 1, 3), GATE_AT=(0, 0), NCH=NCH, scopes=False, PRIO=0, NE=(9, 7), EARLY_AT=3, NA=(10, 8)):
    n0, nq, nf = HS // HM0, HS // HMQ, QS // HMF
    n_att = NA
    assert nf * (n_att[0] * ((NCH + 1) // 2) + n_att[1] * (NCH // 2)) * AG == S

    def kernel(zero_ref, x_hbm, wqkv_hbm, wo_hbm, wg_hbm, wu_hbm, wd_hbm, out_hbm,
               xraw, xc2, wc3, gc0, dc0, gc1, dc1, graw, draw, qo, kp, vp,
               xsem, qsem, wsem, fsem, osem, *work):
        gc, dc = (gc0, gc1), (dc0, dc1)
        pin, pout, pproj, hkeep, hc = work[0:5], work[5:10], work[10:15], work[15:19], work[19:26]
        zeros = [zero_ref[k] for k in range(4)]
        zero = zeros[0]

        def x_copies(t):
            rows = [rows_at(half * HS + t * HM0, HM0) for half in range(2)]
            return [pltpu.make_async_copy(x_hbm.at[r, :], xraw.at[r, :], xsem.at[t]) for r in rows]

        def f_copies(j, slot):
            cols = pl.ds(pl.multiple_of(j * FC, FC), FC)
            return [pltpu.make_async_copy(wg_hbm.at[:, cols], graw.at[slot, 0, pl.ds(0, D), :], fsem.at[slot]),
                    pltpu.make_async_copy(wu_hbm.at[:, cols], graw.at[slot, 1, pl.ds(0, D), :], fsem.at[slot]),
                    pltpu.make_async_copy(wd_hbm.at[cols, :], draw.at[slot, pl.ds(0, FC), :], fsem.at[slot])]

        import contextlib
        scope = jax.named_scope if scopes else (lambda name: contextlib.nullcontext())

        def start(cps):
            for cp in cps:
                cp.start(priority=PRIO)

        def wait(cps):
            for cp in cps:
                cp.wait()

        def hint(i, n):
            return i if isinstance(i, int) else pl.multiple_of(i, n)

        def rows_at(r0, n):
            return pl.ds(r0 if isinstance(r0, int) else pl.multiple_of(r0, n), n)

        def wrows(r0, n):
            return pl.ds(r0 // 2 if isinstance(r0, int) else pl.multiple_of(r0 // 2, 8), n // 2)

        def pace(raw, value):
            spare = raw.shape[0] - PR
            raw[pl.ds(pl.multiple_of(spare + zeros[1], 8), 8), 0:128] = value[0:8].astype(bf16)

        def widen(ref, *idx):
            return _halves(pltpu.bitcast(ref[idx], u32)).astype(f32)

        def kept(bufs, n):
            def keep(i, v):
                bufs[i][0:n, :] = v
            return keep, lambda i: bufs[i][pl.ds(pl.multiple_of(zero, 8), n), :]

        def layernorm(xc, xn, mean, inv, first, count, n, paced=True):
            def block(r0, c, z):
                return widen(xraw, rows_at(r0 + zeros[z], n), slice(c * 128, (c + 1) * 128))

            def row_mean(vals):
                total = functools.reduce(jnp.add, vals)
                if paced:
                    pace(xraw, total)
                return jnp.broadcast_to(jnp.sum(total, axis=-1, keepdims=True) * (1.0 / D), (n, 128))

            def stat(ref, r0):
                return ref[rows_at(r0 + zero, n), :]

            pieces = [first + k for k in range(0, count, n)]
            starts = [half * HS + m0 for m0 in pieces for half in range(2)]
            for r0 in starts:
                mean[rows_at(r0, n), :] = row_mean([block(r0, c, 0) for c in range(NB)])
            yield
            for r0 in starts:
                mu = stat(mean, r0)
                inv[rows_at(r0, n), :] = lax.rsqrt(
                    row_mean([jnp.square(block(r0, c, 2) - mu) for c in range(NB)]) + 1e-5)
            yield
            for m0 in pieces:
                mu = [stat(mean, half * HS + m0) for half in range(2)]
                scale = [stat(inv, half * HS + m0) for half in range(2)]
                for c in range(NB // 2):
                    vals = []
                    for b in range(4):
                        r0, cb = (b // 2) * HS + m0, (b % 2) * (NB // 2) + c
                        vals.append((block(r0, cb, 3) - mu[b // 2]) * scale[b // 2])
                        xn[wrows(r0, n), cb * 128:(cb + 1) * 128] = _words(vals[b])
                    terms = _lhs_terms(*vals)
                    for i in range(7):
                        xc.at[i][wrows(m0, n), c * 128:(c + 1) * 128] = _words(terms[i])
                    if paced:
                        pace(xraw, terms[6])

        def transform_qkv(raw, dst, part, nparts, TB=TB, paced=True):
            n = HD // nparts
            for sb in range(n // TB):
                r0 = part * n + sb * TB
                words = yield from _to_head_lanes([
                    jnp.concatenate([pltpu.bitcast(raw[rows_at(half * HD + r0, TB), c * 128:(c + 1) * 128], u32)
                                     for half in range(2)], axis=0) for c in range(NB)])
                yield
                top = [_halves(w[:TB // 2]).astype(f32) for w in words]
                bot = [_halves(w[TB // 2:]).astype(f32) for w in words]
                for c in range(NB // 2):
                    terms = _rhs_terms(top[c], top[c + NB // 2], bot[c], bot[c + NB // 2])
                    for i in range(7):
                        dst.at[i][wrows(r0, TB), c * 128:(c + 1) * 128] = _words(terms[i])
                if paced:
                    pace(raw, terms[6])

        def two_level(block, terms_of, store, wait_for):
            for i in range(7):
                inner = terms_of(*[terms_of(*[block(p, q) for p in range(4)])[i] for q in range(4)])
                for j in range(7):
                    store(7 * i + j, _words(inner[j]))
                wait_for(inner[6])

        def transform2(raw, dst, part, nparts):
            n = QD // nparts
            for sb in range(n // PR):
                r0 = part * n + sb * PR
                for z in range(2):
                    def block(p, q):
                        kq, nq_ = 2 * (p // 2) + q // 2, 2 * (p % 2) + q % 2
                        return widen(raw, z, rows_at(kq * QD + r0, PR), slice(nq_ * 128, (nq_ + 1) * 128))

                    def store(i, w):
                        dst.at[i][wrows(r0, PR), z * 128:(z + 1) * 128] = w
                    two_level(block, _rhs_terms, store, functools.partial(pace, raw.at[z]))

        def transform_down(raw, dst, part, nparts):
            n = FC // 4 // nparts
            for sb in range(n // PR):
                r0 = part * n + sb * PR
                for c in range(QD // 128):
                    def block(p, q):
                        kq, nq_ = 2 * (p // 2) + q // 2, 2 * (p % 2) + q % 2
                        cols = slice(nq_ * QD + c * 128, nq_ * QD + (c + 1) * 128)
                        return widen(raw, rows_at(kq * (FC // 4) + r0, PR), cols)

                    def store(i, w):
                        dst.at[i][wrows(r0, PR), c * 128:(c + 1) * 128] = w
                    two_level(block, _rhs_terms, store, functools.partial(pace, raw))

        def transform_out(raw, tmp, dst, part, nparts):
            n = 8 // nparts
            low = lax.broadcasted_iota(jnp.int32, (8, 128), 0) < 4

            def wait_for(v):
                tmp[pl.ds(pl.multiple_of(32 + zeros[1], 8), 8), 0:128] = _words(v)
            for sb in range(n):
                g = part * n + sb
                for d2 in range(2):
                    for kq in range(4):
                        r = (g & 1) * 512 + (g >> 1) * 32 + kq * 8
                        for c in range(NB):
                            cols = slice(c * 128, (c + 1) * 128)
                            rows = []
                            for h3 in range(2):
                                u = raw[rows_at(r + h3 * 256, 8), cols].astype(f32)
                                v = raw[rows_at(r + h3 * 256 + 128, 8), cols].astype(f32)
                                rows.append(jnp.where(low, pltpu.roll(u, 4, 0), v) if d2
                                            else jnp.where(low, u, pltpu.roll(v, 4, 0)))
                            tmp[kq * 8:(kq + 1) * 8, cols] = _words(jnp.concatenate(rows, axis=0))
                            if c % 4 == 3:
                                pace(raw, rows[1])
                    for c in range(QD // 128):
                        def block(p, q):
                            kq, nq_ = 2 * (p // 2) + q // 2, 2 * (p % 2) + q % 2
                            cols = slice(nq_ * QD + c * 128, nq_ * QD + (c + 1) * 128)
                            return _halves(tmp[pl.ds(pl.multiple_of(kq * 8 + zero, 8), 8), cols]).astype(f32)

                        def store(i, w):
                            dst.at[i][wrows(d2 * 128 + g * PR, PR), c * 128:(c + 1) * 128] = w
                        two_level(block, _rhs_terms, store, wait_for)

        def expand_x(xn, part, nparts):
            n = QS // nparts
            for sb in range(n // PR):
                m0 = part * n + sb * PR
                for c in range(QD // 128):
                    def block(p, q):
                        mq, kq = 2 * (p // 2) + q // 2, 2 * (p % 2) + q % 2
                        cols = slice(kq * QD + c * 128, kq * QD + (c + 1) * 128)
                        return _halves(xn[wrows(mq * QS + m0, PR), cols]).astype(f32)

                    def store(i, w):
                        xc2.at[i][wrows(m0, PR), c * 128:(c + 1) * 128] = w

                    def wait_for(v):
                        xn[pl.ds(pl.multiple_of(S // 2 + zero, 8), 8), 0:128] = _words(v)
                    two_level(block, _lhs_terms, store, wait_for)

        def project(lhs, wc, hm, finish, shadow):
            keep, fetch = kept(pproj, hm)
            for cb in range(NB // 2):
                def product(i):
                    m = _dot(lhs(i, zeros[cb]), _halves(wc[i + zero, :, cb * 128:(cb + 1) * 128]))
                    if (cb, i) == (0, ORDER[0]):
                        shadow(m)
                    return m
                _seven_products(product, keep, fetch, lambda b, v: finish(b, cb, v))

        def project_x(xc, wc, dst, off, t, hm, scale=None, shadow=lambda m: None):
            def finish(b, cb, v):
                dst[(b % 2) * (NB // 2) + cb, pl.ds(hint(off + (b // 2) * HS + t * hm, 8), hm), :] = (
                    v if scale is None else v * scale)
            project(lambda i, z: _halves(xc[i, wrows(t * hm + (0 if isinstance(t, int) else z), hm), :]), wc, hm, finish, shadow)

        def attention(first, groups):
            lane = lax.broadcasted_iota(jnp.int32, (AG, 128), 1)
            row = lax.broadcasted_iota(jnp.int32, (AG, 128), 0)
            for g in groups:
                s0 = pl.multiple_of((first + g) * AG + zeros[2 + g % 2], AG)
                q = [qo[c, pl.ds(s0, AG), :] for c in range(NB)]
                logits = []
                for w in range(W):
                    rows = pl.ds(s0 + (HALO - DIL * w), AG)
                    logits.append(functools.reduce(jnp.add, [q[c] * kp[c, rows, :] for c in range(NB)]))
                for d in (1, 2):
                    logits = [p + jnp.where((lane & d) == 0, pltpu.roll(p, 128 - d, 1), pltpu.roll(p, d, 1))
                              for p in logits]
                logits = [jnp.where(row + s0 >= DIL * w, p, -1e9 * LOG2E) if g * AG < DIL * w else p
                          for w, p in enumerate(logits)]
                mx = functools.reduce(jnp.maximum, logits)
                es = [jnp.exp2(p - mx) for p in logits]
                inv = 1.0 / functools.reduce(jnp.add, es)
                at = [e * inv for e in es]
                for c in range(NB):
                    o = functools.reduce(
                        jnp.add, [at[w] * vp[c, pl.ds(s0 + (HALO - DIL * w), AG), :] for w in range(W)])
                    qo[c, pl.ds(s0, AG), :] = o

        def next_weights(src, slot, t):
            transform2(graw.at[src], gc[slot], t, nf)
            transform_down(draw.at[src], dc[slot], t, nf)

        again = pl.ds(pl.multiple_of(zero, 8), HMF)

        def forty_nine_products(product, finish):
            def outer(i, q, m):
                fetch = lambda k: pout[k][q, again, :]
                if i < 5:
                    pout[i][q] = m
                if i == 1:
                    finish(2, q, fetch(3) + m)
                elif i == 4:
                    finish(1, q, fetch(2) + m)
                elif i == 5:
                    finish(3, q, fetch(2) + fetch(0) - fetch(1) + m)
                elif i == 6:
                    finish(0, q, fetch(3) + fetch(0) - fetch(4) + m)

            keep, fetch = kept(pin, HMF)
            for i in ORDER:
                _seven_products(lambda j: product(7 * i + j), keep, fetch, lambda q, v: outer(i, q, v))

        def ffn(sums, slot, t, started, early, shadow):
            m0 = t * HMF

            def gate(p, q, c):
                h = jax.nn.gelu(c[:, :128], approximate=True) * c[:, 128:]
                if (p, q) != (0, 0):
                    hkeep[p][q] = h
                if (p, q) == GATE_AT:
                    shadow(h[0:8])
                if p in (3, 0) and q in (3, 0):
                    block = lambda pp, qq: h if (pp, qq) == (p, q) else hkeep[pp][qq, again, :]
                    for i in ((1, 3, 6) if p else (0, 2, 4, 5)):
                        for j in ((1, 3, 6) if q else (0, 2, 4, 5)):
                            hc[i].at[j][...] = _words(_lhs_term(
                                j, lambda qq: _lhs_term(i, lambda pp: block(pp, qq))))

            def product(k):
                m = _dot(_halves(xc2[k, wrows(m0, HMF), :]), _halves(gc[slot][k]))
                if k == EARLY_AT:
                    early(m[0:8, 0:128])
                return m
            forty_nine_products(product, gate)

            for first in ((1, 3, 6), (0, 2, 4, 5)):
                for second in ((1, 3, 6), (0, 2, 4, 5)):
                    for i in first:
                        for j in second:
                            lhs = hc[i][j, pl.ds(pl.multiple_of(zero, 8), HMF // 2), :]
                            rows = rows_at(m0, HMF)
                            sums[i][j, rows, :] = (jnp.where(started, sums[i][j, rows, :], 0.0)
                                                   + _dot(_halves(lhs), _halves(dc[slot][7 * i + j])))

        def out_operands(dst, t, paced):
            for sb in range(HMF // PR):
                for c in range(QD // 128):
                    def block(p, q):
                        mq, kq = 2 * (p // 2) + q // 2, 2 * (p % 2) + q % 2
                        return qo[2 * kq + c, rows_at(mq * QS + t * HMF + sb * PR, PR), :]

                    def store(k, w):
                        dst.at[k][wrows(sb * PR, PR), c * 128:(c + 1) * 128] = w

                    def wait_for(v):
                        if paced:
                            qo[0, pl.ds(pl.multiple_of(S + zeros[1], 8), 8), :] = v[0:8]
                    two_level(block, _lhs_terms, store, wait_for)

        def out_proj(sums, operands, t, shadow):
            m0 = t * HMF

            def window(p, q):
                return (rows_at((2 * (p // 2) + q // 2) * QS + m0, HMF), pl.ds((2 * (p % 2) + q % 2) * QD, QD))

            def finish(p, q, v):
                xraw[window(p, q)] = (xraw[window(p, q)].astype(f32) + v).astype(bf16)
                pltpu.make_async_copy(xraw.at[window(p, q)], out_hbm.at[window(p, q)], osem).start()

            def product(k):
                m = _dot(_halves(operands[k, pl.ds(pl.multiple_of(zero, 8), HMF // 2), :]), _halves(wc3[k]))
                if k == 7 * ORDER[0] + ORDER[0]:
                    shadow(m[0:8, 0:128])
                return m + sums[k // 7][k % 7, rows_at(m0, HMF), :]
            forty_nine_products(product, finish)

        def projections(xc, xn, mean, inv, tmp, wraw, wc0, wc1, wc2):
            def w_copies(p):
                src = wo_hbm if p == 3 else wqkv_hbm.at[:, p * D:(p + 1) * D]
                return [pltpu.make_async_copy(src, wraw.at[p, pl.ds(0, D), :], wsem.at[p])]

            def wq_copies(i):
                rows = [rows_at(half * HD + i * (HD // NP), HD // NP) for half in range(2)]
                return [pltpu.make_async_copy(wqkv_hbm.at[r, pl.ds(0, D)], wraw.at[0, r, :], qsem.at[i]) for r in rows]

            with scope("prologue"):
                start(x_copies(0))
                lax.fori_loop(0, NP, lambda i, _: start(wq_copies(i)), None)
                lax.fori_loop(1, n0, lambda t, _: start(x_copies(t)), None)
                start(w_copies(1))
                for c in range(NB):
                    kp[c, 0:HALO, :] = jnp.zeros((HALO, 128), f32)
                with scope("wait_x0"):
                    wait(x_copies(0))

                _run(layernorm(xc, xn, mean, inv, 0, HM0, PR, paced=False))

                def first_body(i, _):
                    wait(wq_copies(i))
                    _run(*[transform_qkv(wraw.at[0], wc0, i * TW + k, NP * TW, TB0, paced=False) for k in range(TW)])
                lax.fori_loop(0, NP, first_body, None)
                start(w_copies(2))

            with scope("qphase"):
                for lo, hi in zip(QSTOPS, QSTOPS[1:] + (n0,)):
                    with scope(f"wait_x{lo}"):
                        for t in range(lo + 1, min(hi + 1, n0)):
                            wait(x_copies(t))
                    if hi == n0:
                        with scope(f"wait_wk"):
                            wait(w_copies(1))
                        start(w_copies(3))
                        start(f_copies(0, 0))
                    for t in range(lo, hi):
                        def shadow(token):
                            if t + 1 < n0:
                                pace(xraw, token)
                                _run(layernorm(xc, xn, mean, inv, (t + 1) * HM0, HM0, LB))
                        project_x(xc, wc0, qo, 0, t, HM0, DH ** -0.5 * LOG2E, shadow)
                _run(transform_qkv(wraw.at[1], wc1, 0, 1))

            wait(w_copies(2))
            wait(w_copies(3))
            start(f_copies(1, 1))

            def k_body(t, _):
                project_x(xc, wc1, kp, HALO, t, HMQ)
                transform_out(wraw.at[3], tmp, wc3, t, nq)
                _run(transform_qkv(wraw.at[2], wc2, t, nq))
            with scope("kphase"):
                lax.fori_loop(0, nq, k_body, None)

            wait(f_copies(0, 0))

            def v_body(t, _):
                project_x(xc, wc2, vp, HALO, t, HMQ)
                expand_x(xn, t, nq)
                transform2(graw.at[0], gc0, t, nq)
                transform_down(draw.at[0], dc0, t, nq)
            with scope("vphase"):
                lax.fori_loop(0, nq, v_body, None)
            for c in range(NB):
                vp[c, 0:HALO, :] = jnp.broadcast_to(vp[c, HALO:HALO + 1, :], (HALO, 128))

        pl.run_scoped(projections,
                      pltpu.VMEM((7, HS // 2, HD), u32), pltpu.VMEM((S // 2 + 8, D), u32),
                      pltpu.VMEM((S, 128), f32), pltpu.VMEM((S, 128), f32), pltpu.VMEM((40, D), u32), pltpu.VMEM((4, D + PR, D), bf16),
                      *[pltpu.VMEM((7, HD // 2, HD), u32)] * 3)

        def second_half(*sums):
            def chunk_body(j, _):
                src = jnp.minimum(j + 1, NCH - 1) % 2

                @pl.when(j + 1 < NCH)
                def _():
                    wait(f_copies(j + 1, 1 - j % 2))

                @pl.when(j + 2 < NCH)
                def _():
                    start(f_copies(j + 2, j % 2))

                for parity in range(2):
                    @pl.when(j % 2 == parity)
                    def _():
                        def tile_body(t, _):
                            first = nf * (n_att[0] * ((j + 1) // 2) + n_att[1] * (j // 2)) + t * n_att[parity]
                            def shadow(groups, token):
                                if len(groups):
                                    qo[0, pl.ds(pl.multiple_of(S + zero, 8), 8), :] = token
                                    attention(first, groups)
                            ffn(sums, parity, t, True if parity else j > 0,
                                functools.partial(shadow, range(NE[parity])),
                                functools.partial(shadow, range(NE[parity], n_att[parity])))
                            next_weights(src, 1 - parity, t)
                        lax.fori_loop(0, nf, tile_body, None)
            with scope("ffn"):
                lax.fori_loop(0, NCH, chunk_body, None)

            with scope("ophase"):
                out_operands(gc0, 0, False)

                for t in range(nf):
                    def shadow(token):
                        if t + 1 < nf:
                            qo[0, pl.ds(pl.multiple_of(S + zeros[1], 8), 8), :] = token
                            out_operands(gc[(t + 1) % 2], t + 1, True)
                    out_proj(sums, gc[t % 2], t, shadow)
            with scope("drain"):
                pltpu.make_async_copy(xraw.at[pl.ds(0, S), :], out_hbm, osem).wait()

        pl.run_scoped(second_half, *[pltpu.VMEM((7, QS, QD), f32)] * 7)

    scratch = [
        pltpu.VMEM((S + PR, D), bf16),
        pltpu.VMEM((49, QS // 2, QD), u32),
        pltpu.VMEM((49, QD // 2, QD), u32),
        pltpu.VMEM((49, QD // 2, FC // 2), u32),
        pltpu.VMEM((49, FC // 8, QD), u32),
        pltpu.VMEM((49, QD // 2, FC // 2), u32),
        pltpu.VMEM((49, FC // 8, QD), u32),
        pltpu.VMEM((2, 2, D + PR, FC), bf16),
        pltpu.VMEM((2, FC + PR, D), bf16),
        pltpu.VMEM((NB, S + 8, 128), f32),
        pltpu.VMEM((NB, HALO + S + 8, 128), f32),
        pltpu.VMEM((NB, HALO + S + 8, 128), f32),
        pltpu.SemaphoreType.DMA((n0,)),
        pltpu.SemaphoreType.DMA((NP,)),
        pltpu.SemaphoreType.DMA((4,)),
        pltpu.SemaphoreType.DMA((2,)),
        pltpu.SemaphoreType.DMA(()),
        *[pltpu.VMEM((HMF, 256), f32)] * 5,
        *[pltpu.VMEM((4, HMF, 256), f32)] * 5,
        *[pltpu.VMEM((max(HM0, HMQ), 128), f32)] * 5,
        *[pltpu.VMEM((4, HMF, 128), f32)] * 4,
        *[pltpu.VMEM((7, HMF // 2, 128), u32)] * 7,
    ]
    return kernel, scratch


def make_call(flags=None, **kw):
    kernel, scratch = make_kernel(**kw)
    hbm = pl.BlockSpec(memory_space=pl.ANY)
    return pl.pallas_call(
        kernel,
        in_specs=[pl.BlockSpec(memory_space=pltpu.SMEM)] + [hbm] * 6,
        out_specs=hbm,
        out_shape=jax.ShapeDtypeStruct((S, D), bf16),
        scratch_shapes=scratch,
        compiler_params=pltpu.CompilerParams(vmem_limit_bytes=126 * 1024 * 1024, flags=flags),
    )


@jax.jit
def pallas_parallel_sum__sliding_local_dilated__glu_gated_geglu__prompt_kernel(
    A_x, A_wqkv, A_wo, B_x, B_w_gate, B_w_up, B_w_down
):
    del B_x
    out = make_call()(np.zeros((4,), np.int32), A_x.reshape(S, D), A_wqkv, A_wo, B_w_gate, B_w_up, B_w_down)
    return out.reshape(1, S, D)
```

```python
import functools
import jax
import jax.numpy as jnp
import numpy as np
from jax import lax
import jax.experimental.pallas as pl
import jax.experimental.pallas.tpu as pltpu

S, D, F = 2048, 1024, 3584
H, DH, W, DIL = 32, 32, 8, 2
HALO = 16
NB = D // 128
HS, QS = S // 2, S // 4
HD, QD = D // 2, D // 4
FC = 512
NCH = F // FC
PR = 16
LOG2E = 1.4426950408889634
ORDER = (2, 3, 0, 1, 4, 5, 6)
f32, bf16, u32 = jnp.float32, jnp.bfloat16, jnp.uint32


def _dot(a, b):
    return jnp.dot(a, b, preferred_element_type=f32)


def _words(v):
    return pltpu.bitcast(v.astype(bf16), u32)


def _halves(w):
    return pltpu.bitcast(w, bf16)


def _lhs_terms(a11, a12, a21, a22):
    return [a11 + a22, a21 + a22, a11, a22, a11 + a12, a21 - a11, a12 - a22]


def _lhs_term(i, a):
    return (lambda: a(0) + a(3), lambda: a(2) + a(3), lambda: a(0), lambda: a(3),
            lambda: a(0) + a(1), lambda: a(2) - a(0), lambda: a(1) - a(3))[i]()


def _rhs_terms(b11, b12, b21, b22):
    return [b11 + b22, b11, b12 - b22, b21 - b11, b22, b11 + b12, b21 + b22]


def _seven_products(product, keep, fetch, finish):
    for i in (2, 3, 0):
        keep(i, product(i))
    m = product(1)
    keep(1, m)
    finish(2, fetch(3) + m)
    m = product(4)
    keep(4, m)
    finish(1, fetch(2) + m)
    finish(3, fetch(2) + fetch(0) - fetch(1) + product(5))
    finish(0, fetch(3) + fetch(0) - fetch(4) + product(6))


def _to_head_lanes(blocks):
    slot = lax.broadcasted_iota(jnp.int32, blocks[0].shape, 1) >> 2
    blocks = [pltpu.roll(b, 4 * c, 1) if c else b for c, b in enumerate(blocks)]
    yield
    blocks = [blocks[-j % NB] for j in range(NB)]
    for bit in (1, 2, 4):
        move = (slot & bit) != 0
        blocks = [jnp.where(move, blocks[(j - bit) % NB], blocks[j]) for j in range(NB)]
    return [pltpu.roll(b, 128 - 4 * j, 1) if j else b for j, b in enumerate(blocks)]


def _run(*stages):
    stages = list(stages)
    while stages:
        stages = [g for g in stages if next(g, True) is None]


def make_kernel(HM0=128, HMQ=512, HMF=128, AG=8, LB=16, TB=32, NP=4, TB0=16, TW=4, QSTOPS=(1, 2, 4), GATE_AT=(0, 0), NCH=NCH, scopes=False, PRIO=0, NE=(9, 7), EARLY_AT=3, NA=(10, 8), X1=False, TQ=1):
    n0, nq, nf = HS // HM0, HS // HMQ, QS // HMF
    n_att = NA
    assert nf * (n_att[0] * ((NCH + 1) // 2) + n_att[1] * (NCH // 2)) * AG == S

    def kernel(zero_ref, x_hbm, wqkv_hbm, wo_hbm, wg_hbm, wu_hbm, wd_hbm, out_hbm,
               xraw, xc2, wc3, gc0, dc0, gc1, dc1, graw, draw, qo, kp, vp,
               xsem, qsem, wsem, fsem, osem, *work):
        gc, dc = (gc0, gc1), (dc0, dc1)
        pin, pout, pproj, hkeep, hc = work[0:5], work[5:10], work[10:15], work[15:19], work[19:26]
        zeros = [zero_ref[k] for k in range(4)]
        zero = zeros[0]

        def x_copies(t):
            rows = [rows_at(half * HS + t * HM0, HM0) for half in range(2)]
            return [pltpu.make_async_copy(x_hbm.at[r, :], xraw.at[r, :], xsem.at[t]) for r in rows]

        def f_copies(j, slot):
            cols = pl.ds(pl.multiple_of(j * FC, FC), FC)
            return [pltpu.make_async_copy(wg_hbm.at[:, cols], graw.at[slot, 0, pl.ds(0, D), :], fsem.at[slot]),
                    pltpu.make_async_copy(wu_hbm.at[:, cols], graw.at[slot, 1, pl.ds(0, D), :], fsem.at[slot]),
                    pltpu.make_async_copy(wd_hbm.at[cols, :], draw.at[slot, pl.ds(0, FC), :], fsem.at[slot])]

        import contextlib
        scope = jax.named_scope if scopes else (lambda name: contextlib.nullcontext())

        def start(cps):
            for cp in cps:
                cp.start(priority=PRIO)

        def wait(cps):
            for cp in cps:
                cp.wait()

        def hint(i, n):
            return i if isinstance(i, int) else pl.multiple_of(i, n)

        def rows_at(r0, n):
            return pl.ds(r0 if isinstance(r0, int) else pl.multiple_of(r0, n), n)

        def wrows(r0, n):
            return pl.ds(r0 // 2 if isinstance(r0, int) else pl.multiple_of(r0 // 2, 8), n // 2)

        def pace(raw, value):
            spare = raw.shape[0] - PR
            raw[pl.ds(pl.multiple_of(spare + zeros[1], 8), 8), 0:128] = value[0:8].astype(bf16)

        def widen(ref, *idx):
            return _halves(pltpu.bitcast(ref[idx], u32)).astype(f32)

        def kept(bufs, n):
            def keep(i, v):
                bufs[i][0:n, :] = v
            return keep, lambda i: bufs[i][pl.ds(pl.multiple_of(zero, 8), n), :]

        def layernorm(xc, xn, mean, inv, first, count, n, paced=True):
            def block(r0, c, z):
                return widen(xraw, rows_at(r0 + zeros[z], n), slice(c * 128, (c + 1) * 128))

            def row_mean(vals):
                total = functools.reduce(jnp.add, vals)
                if paced:
                    pace(xraw, total)
                return jnp.broadcast_to(jnp.sum(total, axis=-1, keepdims=True) * (1.0 / D), (n, 128))

            def stat(ref, r0):
                return ref[rows_at(r0 + zero, n), :]

            pieces = [first + k for k in range(0, count, n)]
            starts = [half * HS + m0 for m0 in pieces for half in range(2)]
            for r0 in starts:
                mean[rows_at(r0, n), :] = row_mean([block(r0, c, 0) for c in range(NB)])
            yield
            for r0 in starts:
                mu = stat(mean, r0)
                inv[rows_at(r0, n), :] = lax.rsqrt(
                    row_mean([jnp.square(block(r0, c, 2) - mu) for c in range(NB)]) + 1e-5)
            yield
            for m0 in pieces:
                mu = [stat(mean, half * HS + m0) for half in range(2)]
                scale = [stat(inv, half * HS + m0) for half in range(2)]
                for c in range(NB // 2):
                    vals = []
                    for b in range(4):
                        r0, cb = (b // 2) * HS + m0, (b % 2) * (NB // 2) + c
                        vals.append((block(r0, cb, 3) - mu[b // 2]) * scale[b // 2])
                        xn[wrows(r0, n), cb * 128:(cb + 1) * 128] = _words(vals[b])
                    terms = _lhs_terms(*vals)
                    for i in range(7):
                        xc.at[i][wrows(m0, n), c * 128:(c + 1) * 128] = _words(terms[i])
                    if paced:
                        pace(xraw, terms[6])

        def transform_qkv(raw, dst, part, nparts, TB=TB, paced=True):
            n = HD // nparts
            for sb in range(n // TB):
                r0 = part * n + sb * TB
                words = yield from _to_head_lanes([
                    jnp.concatenate([pltpu.bitcast(raw[rows_at(half * HD + r0, TB), c * 128:(c + 1) * 128], u32)
                                     for half in range(2)], axis=0) for c in range(NB)])
                yield
                top = [_halves(w[:TB // 2]).astype(f32) for w in words]
                bot = [_halves(w[TB // 2:]).astype(f32) for w in words]
                for c in range(NB // 2):
                    terms = _rhs_terms(top[c], top[c + NB // 2], bot[c], bot[c + NB // 2])
                    for i in range(7):
                        dst.at[i][wrows(r0, TB), c * 128:(c + 1) * 128] = _words(terms[i])
                if paced:
                    pace(raw, terms[6])

        def two_level(block, terms_of, store, wait_for):
            for i in range(7):
                inner = terms_of(*[terms_of(*[block(p, q) for p in range(4)])[i] for q in range(4)])
                for j in range(7):
                    store(7 * i + j, _words(inner[j]))
                wait_for(inner[6])

        def transform2(raw, dst, part, nparts):
            n = QD // nparts
            for sb in range(n // PR):
                r0 = part * n + sb * PR
                for z in range(2):
                    def block(p, q):
                        kq, nq_ = 2 * (p // 2) + q // 2, 2 * (p % 2) + q % 2
                        return widen(raw, z, rows_at(kq * QD + r0, PR), slice(nq_ * 128, (nq_ + 1) * 128))

                    def store(i, w):
                        dst.at[i][wrows(r0, PR), z * 128:(z + 1) * 128] = w
                    two_level(block, _rhs_terms, store, functools.partial(pace, raw.at[z]))

        def transform_down(raw, dst, part, nparts):
            n = FC // 4 // nparts
            for sb in range(n // PR):
                r0 = part * n + sb * PR
                for c in range(QD // 128):
                    def block(p, q):
                        kq, nq_ = 2 * (p // 2) + q // 2, 2 * (p % 2) + q % 2
                        cols = slice(nq_ * QD + c * 128, nq_ * QD + (c + 1) * 128)
                        return widen(raw, rows_at(kq * (FC // 4) + r0, PR), cols)

                    def store(i, w):
                        dst.at[i][wrows(r0, PR), c * 128:(c + 1) * 128] = w
                    two_level(block, _rhs_terms, store, functools.partial(pace, raw))

        def transform_out(raw, tmp, dst, part, nparts):
            n = 8 // nparts
            low = lax.broadcasted_iota(jnp.int32, (8, 128), 0) < 4

            def wait_for(v):
                tmp[pl.ds(pl.multiple_of(32 + zeros[1], 8), 8), 0:128] = _words(v)
            for sb in range(n):
                g = part * n + sb
                for d2 in range(2):
                    for kq in range(4):
                        r = (g & 1) * 512 + (g >> 1) * 32 + kq * 8
                        for c in range(NB):
                            cols = slice(c * 128, (c + 1) * 128)
                            rows = []
                            for h3 in range(2):
                                u = raw[rows_at(r + h3 * 256, 8), cols].astype(f32)
                                v = raw[rows_at(r + h3 * 256 + 128, 8), cols].astype(f32)
                                rows.append(jnp.where(low, pltpu.roll(u, 4, 0), v) if d2
                                            else jnp.where(low, u, pltpu.roll(v, 4, 0)))
                            tmp[kq * 8:(kq + 1) * 8, cols] = _words(jnp.concatenate(rows, axis=0))
                            if c % 4 == 3:
                                pace(raw, rows[1])
                    for c in range(QD // 128):
                        def block(p, q):
                            kq, nq_ = 2 * (p // 2) + q // 2, 2 * (p % 2) + q % 2
                            cols = slice(nq_ * QD + c * 128, nq_ * QD + (c + 1) * 128)
                            return _halves(tmp[pl.ds(pl.multiple_of(kq * 8 + zero, 8), 8), cols]).astype(f32)

                        def store(i, w):
                            dst.at[i][wrows(d2 * 128 + g * PR, PR), c * 128:(c + 1) * 128] = w
                        two_level(block, _rhs_terms, store, wait_for)

        def expand_x(xn, part, nparts):
            n = QS // nparts
            for sb in range(n // PR):
                m0 = part * n + sb * PR
                for c in range(QD // 128):
                    def block(p, q):
                        mq, kq = 2 * (p // 2) + q // 2, 2 * (p % 2) + q % 2
                        cols = slice(kq * QD + c * 128, kq * QD + (c + 1) * 128)
                        return _halves(xn[wrows(mq * QS + m0, PR), cols]).astype(f32)

                    def store(i, w):
                        xc2.at[i][wrows(m0, PR), c * 128:(c + 1) * 128] = w

                    def wait_for(v):
                        xn[pl.ds(pl.multiple_of(S // 2 + zero, 8), 8), 0:128] = _words(v)
                    two_level(block, _lhs_terms, store, wait_for)

        def project(lhs, wc, hm, finish, shadow):
            keep, fetch = kept(pproj, hm)
            for cb in range(NB // 2):
                def product(i):
                    m = _dot(lhs(i, zeros[cb]), _halves(wc[i + zero, :, cb * 128:(cb + 1) * 128]))
                    if (cb, i) == (0, ORDER[0]):
                        shadow(m)
                    return m
                _seven_products(product, keep, fetch, lambda b, v: finish(b, cb, v))

        def project_x(xc, wc, dst, off, t, hm, scale=None, shadow=lambda m: None):
            def finish(b, cb, v):
                dst[(b % 2) * (NB // 2) + cb, pl.ds(hint(off + (b // 2) * HS + t * hm, 8), hm), :] = (
                    v if scale is None else v * scale)
            project(lambda i, z: _halves(xc[i, wrows(t * hm + (0 if isinstance(t, int) else z), hm), :]), wc, hm, finish, shadow)

        def attention(first, groups):
            lane = lax.broadcasted_iota(jnp.int32, (AG, 128), 1)
            row = lax.broadcasted_iota(jnp.int32, (AG, 128), 0)
            for g in groups:
                s0 = pl.multiple_of((first + g) * AG + zeros[2 + g % 2], AG)
                q = [qo[c, pl.ds(s0, AG), :] for c in range(NB)]
                logits = []
                for w in range(W):
                    rows = pl.ds(s0 + (HALO - DIL * w), AG)
                    logits.append(functools.reduce(jnp.add, [q[c] * kp[c, rows, :] for c in range(NB)]))
                for d in (1, 2):
                    logits = [p + jnp.where((lane & d) == 0, pltpu.roll(p, 128 - d, 1), pltpu.roll(p, d, 1))
                              for p in logits]
                logits = [jnp.where(row + s0 >= DIL * w, p, -1e9 * LOG2E) if g * AG < DIL * w else p
                          for w, p in enumerate(logits)]
                mx = functools.reduce(jnp.maximum, logits)
                es = [jnp.exp2(p - mx) for p in logits]
                inv = 1.0 / functools.reduce(jnp.add, es)
                at = [e * inv for e in es]
                for c in range(NB):
                    o = functools.reduce(
                        jnp.add, [at[w] * vp[c, pl.ds(s0 + (HALO - DIL * w), AG), :] for w in range(W)])
                    qo[c, pl.ds(s0, AG), :] = o

        def next_weights(src, slot, t):
            transform2(graw.at[src], gc[slot], t, nf)
            transform_down(draw.at[src], dc[slot], t, nf)

        again = pl.ds(pl.multiple_of(zero, 8), HMF)

        def forty_nine_products(product, finish):
            def outer(i, q, m):
                fetch = lambda k: pout[k][q, again, :]
                if i < 5:
                    pout[i][q] = m
                if i == 1:
                    finish(2, q, fetch(3) + m)
                elif i == 4:
                    finish(1, q, fetch(2) + m)
                elif i == 5:
                    finish(3, q, fetch(2) + fetch(0) - fetch(1) + m)
                elif i == 6:
                    finish(0, q, fetch(3) + fetch(0) - fetch(4) + m)

            keep, fetch = kept(pin, HMF)
            for i in ORDER:
                _seven_products(lambda j: product(7 * i + j), keep, fetch, lambda q, v: outer(i, q, v))

        def ffn(sums, slot, t, started, early, shadow):
            m0 = t * HMF

            def gate(p, q, c):
                h = jax.nn.gelu(c[:, :128], approximate=True) * c[:, 128:]
                if (p, q) != (0, 0):
                    hkeep[p][q] = h
                if (p, q) == GATE_AT:
                    shadow(h[0:8])
                if p in (3, 0) and q in (3, 0):
                    block = lambda pp, qq: h if (pp, qq) == (p, q) else hkeep[pp][qq, again, :]
                    for i in ((1, 3, 6) if p else (0, 2, 4, 5)):
                        for j in ((1, 3, 6) if q else (0, 2, 4, 5)):
                            hc[i].at[j][...] = _words(_lhs_term(
                                j, lambda qq: _lhs_term(i, lambda pp: block(pp, qq))))

            def product(k):
                m = _dot(_halves(xc2[k, wrows(m0, HMF), :]), _halves(gc[slot][k]))
                if k == EARLY_AT:
                    early(m[0:8, 0:128])
                return m
            forty_nine_products(product, gate)

            for first in ((1, 3, 6), (0, 2, 4, 5)):
                for second in ((1, 3, 6), (0, 2, 4, 5)):
                    for i in first:
                        for j in second:
                            lhs = hc[i][j, pl.ds(pl.multiple_of(zero, 8), HMF // 2), :]
                            rows = rows_at(m0, HMF)
                            sums[i][j, rows, :] = (jnp.where(started, sums[i][j, rows, :], 0.0)
                                                   + _dot(_halves(lhs), _halves(dc[slot][7 * i + j])))

        def out_operands(dst, t, paced):
            for sb in range(HMF // PR):
                for c in range(QD // 128):
                    def block(p, q):
                        mq, kq = 2 * (p // 2) + q // 2, 2 * (p % 2) + q % 2
                        return qo[2 * kq + c, rows_at(mq * QS + t * HMF + sb * PR, PR), :]

                    def store(k, w):
                        dst.at[k][wrows(sb * PR, PR), c * 128:(c + 1) * 128] = w

                    def wait_for(v):
                        if paced:
                            qo[0, pl.ds(pl.multiple_of(S + zeros[1], 8), 8), :] = v[0:8]
                    two_level(block, _lhs_terms, store, wait_for)

        def out_proj(sums, operands, t, shadow):
            m0 = t * HMF

            def window(p, q):
                return (rows_at((2 * (p // 2) + q // 2) * QS + m0, HMF), pl.ds((2 * (p % 2) + q % 2) * QD, QD))

            def finish(p, q, v):
                xraw[window(p, q)] = (xraw[window(p, q)].astype(f32) + v).astype(bf16)
                pltpu.make_async_copy(xraw.at[window(p, q)], out_hbm.at[window(p, q)], osem).start()

            def product(k):
                m = _dot(_halves(operands[k, pl.ds(pl.multiple_of(zero, 8), HMF // 2), :]), _halves(wc3[k]))
                if k == 7 * ORDER[0] + ORDER[0]:
                    shadow(m[0:8, 0:128])
                return m + sums[k // 7][k % 7, rows_at(m0, HMF), :]
            forty_nine_products(product, finish)

        def projections(xc, xn, mean, inv, tmp, head, wraw, wc0, wc1, wc2):
            def w_copies(p):
                src = wo_hbm if p == 3 else wqkv_hbm.at[:, p * D:(p + 1) * D]
                return [pltpu.make_async_copy(src, wraw.at[p, pl.ds(0, D), :], wsem.at[p])]

            def wq_copies(i):
                rows = [rows_at(half * HD + i * (HD // NP), HD // NP) for half in range(2)]
                return [pltpu.make_async_copy(wqkv_hbm.at[r, pl.ds(0, D)], wraw.at[0, r, :], qsem.at[i]) for r in rows]

            with scope("prologue"):
                start(x_copies(0))
                if X1:
                    lax.fori_loop(1, 2, lambda t, _: start(x_copies(t)), None)
                lax.fori_loop(0, NP, lambda i, _: start(wq_copies(i)), None)
                lax.fori_loop(2 if X1 else 1, n0, lambda t, _: start(x_copies(t)), None)
                start(w_copies(1))
                for c in range(NB):
                    kp[c, 0:HALO, :] = jnp.zeros((HALO, 128), f32)
                with scope("wait_x0"):
                    wait(x_copies(0))

                _run(layernorm(xc, xn, mean, inv, 0, HM0, PR, paced=False))

                if X1:
                    wait(x_copies(1))

                def first_body(i, _):
                    wait(wq_copies(i))
                    n = HD // NP
                    lhs = jnp.concatenate([
                        jnp.concatenate([xn[wrows(half * HS, HM0), pl.ds(pl.multiple_of(k * HD + i * n, n), n)]
                                         for k in range(2)], axis=1) for half in range(2)], axis=0)
                    for c in range(D // 256):
                        cols = slice(c * 256, (c + 1) * 256)
                        rhs = jnp.concatenate([wraw[0, rows_at(k * HD + i * n, n), cols] for k in range(2)], axis=0)
                        head[:, cols] = jnp.where(i > 0, head[:, cols], 0.0) + _dot(_halves(lhs), rhs)
                    stages = [transform_qkv(wraw.at[0], wc0, i * TW + k, NP * TW, TB0, paced=False) for k in range(TW)]
                    if X1:
                        stages.append(layernorm(xc, xn, mean, inv, HM0 + i * (HM0 // NP), HM0 // NP, PR, paced=False))
                    _run(*stages)
                lax.fori_loop(0, NP, first_body, None)
                start(w_copies(2))

            with scope("qphase"):
                if not X1:
                    wait(x_copies(1))
                    _run(layernorm(xc, xn, mean, inv, HM0, HM0, PR, paced=False))
                for lo, hi in zip(QSTOPS, QSTOPS[1:] + (n0,)):
                    with scope(f"wait_x{lo}"):
                        for t in range(lo + 1, min(hi + 1, n0)):
                            wait(x_copies(t))
                    if hi == n0:
                        with scope(f"wait_wk"):
                            wait(w_copies(1))
                        start(w_copies(3))
                        start(f_copies(0, 0))
                    if lo == QSTOPS[TQ]:
                        for sb in range(HM0 // PR):
                            def to_q(half):
                                rows = rows_at(half * HM0 + sb * PR + zeros[2 + sb % 2], PR)
                                blocks = yield from _to_head_lanes([head[rows, c * 128:(c + 1) * 128] for c in range(NB)])
                                for c in range(NB):
                                    qo[c, rows_at(half * HS + sb * PR, PR), :] = blocks[c] * (DH ** -0.5 * LOG2E)
                                head[rows, 0:128] = blocks[0]
                            _run(to_q(0), to_q(1))
                    for t in range(lo, hi):
                        def shadow(token):
                            if t + 1 < n0:
                                pace(xraw, token)
                                _run(layernorm(xc, xn, mean, inv, (t + 1) * HM0, HM0, LB))
                        project_x(xc, wc0, qo, 0, t, HM0, DH ** -0.5 * LOG2E, shadow)
                _run(transform_qkv(wraw.at[1], wc1, 0, 1))

            wait(w_copies(2))
            wait(w_copies(3))
            start(f_copies(1, 1))

            def k_body(t, _):
                project_x(xc, wc1, kp, HALO, t, HMQ)
                transform_out(wraw.at[3], tmp, wc3, t, nq)
                _run(transform_qkv(wraw.at[2], wc2, t, nq))
            with scope("kphase"):
                lax.fori_loop(0, nq, k_body, None)

            wait(f_copies(0, 0))

            def v_body(t, _):
                project_x(xc, wc2, vp, HALO, t, HMQ)
                expand_x(xn, t, nq)
                transform2(graw.at[0], gc0, t, nq)
                transform_down(draw.at[0], dc0, t, nq)
            with scope("vphase"):
                lax.fori_loop(0, nq, v_body, None)
            for c in range(NB):
                vp[c, 0:HALO, :] = jnp.broadcast_to(vp[c, HALO:HALO + 1, :], (HALO, 128))

        pl.run_scoped(projections,
                      pltpu.VMEM((7, HS // 2, HD), u32), pltpu.VMEM((S // 2 + 8, D), u32),
                      pltpu.VMEM((S, 128), f32), pltpu.VMEM((S, 128), f32), pltpu.VMEM((40, D), u32),
                      pltpu.VMEM((2 * HM0, D), f32), pltpu.VMEM((4, D + PR, D), bf16),
                      *[pltpu.VMEM((7, HD // 2, HD), u32)] * 3)

        def second_half(*sums):
            def chunk_body(j, _):
                src = jnp.minimum(j + 1, NCH - 1) % 2

                @pl.when(j + 1 < NCH)
                def _():
                    wait(f_copies(j + 1, 1 - j % 2))

                @pl.when(j + 2 < NCH)
                def _():
                    start(f_copies(j + 2, j % 2))

                for parity in range(2):
                    @pl.when(j % 2 == parity)
                    def _():
                        def tile_body(t, _):
                            first = nf * (n_att[0] * ((j + 1) // 2) + n_att[1] * (j // 2)) + t * n_att[parity]
                            def shadow(groups, token):
                                if len(groups):
                                    qo[0, pl.ds(pl.multiple_of(S + zero, 8), 8), :] = token
                                    attention(first, groups)
                            ffn(sums, parity, t, True if parity else j > 0,
                                functools.partial(shadow, range(NE[parity])),
                                functools.partial(shadow, range(NE[parity], n_att[parity])))
                            next_weights(src, 1 - parity, t)
                        lax.fori_loop(0, nf, tile_body, None)
            with scope("ffn"):
                lax.fori_loop(0, NCH, chunk_body, None)

            with scope("ophase"):
                out_operands(gc0, 0, False)

                for t in range(nf):
                    def shadow(token):
                        if t + 1 < nf:
                            qo[0, pl.ds(pl.multiple_of(S + zeros[1], 8), 8), :] = token
                            out_operands(gc[(t + 1) % 2], t + 1, True)
                    out_proj(sums, gc[t % 2], t, shadow)
            with scope("drain"):
                pltpu.make_async_copy(xraw.at[pl.ds(0, S), :], out_hbm, osem).wait()

        pl.run_scoped(second_half, *[pltpu.VMEM((7, QS, QD), f32)] * 7)

    scratch = [
        pltpu.VMEM((S + PR, D), bf16),
        pltpu.VMEM((49, QS // 2, QD), u32),
        pltpu.VMEM((49, QD // 2, QD), u32),
        pltpu.VMEM((49, QD // 2, FC // 2), u32),
        pltpu.VMEM((49, FC // 8, QD), u32),
        pltpu.VMEM((49, QD // 2, FC // 2), u32),
        pltpu.VMEM((49, FC // 8, QD), u32),
        pltpu.VMEM((2, 2, D + PR, FC), bf16),
        pltpu.VMEM((2, FC + PR, D), bf16),
        pltpu.VMEM((NB, S + 8, 128), f32),
        pltpu.VMEM((NB, HALO + S + 8, 128), f32),
        pltpu.VMEM((NB, HALO + S + 8, 128), f32),
        pltpu.SemaphoreType.DMA((n0,)),
        pltpu.SemaphoreType.DMA((NP,)),
        pltpu.SemaphoreType.DMA((4,)),
        pltpu.SemaphoreType.DMA((2,)),
        pltpu.SemaphoreType.DMA(()),
        *[pltpu.VMEM((HMF, 256), f32)] * 5,
        *[pltpu.VMEM((4, HMF, 256), f32)] * 5,
        *[pltpu.VMEM((max(HM0, HMQ), 128), f32)] * 5,
        *[pltpu.VMEM((4, HMF, 128), f32)] * 4,
        *[pltpu.VMEM((7, HMF // 2, 128), u32)] * 7,
    ]
    return kernel, scratch


def make_call(flags=None, **kw):
    kernel, scratch = make_kernel(**kw)
    hbm = pl.BlockSpec(memory_space=pl.ANY)
    return pl.pallas_call(
        kernel,
        in_specs=[pl.BlockSpec(memory_space=pltpu.SMEM)] + [hbm] * 6,
        out_specs=hbm,
        out_shape=jax.ShapeDtypeStruct((S, D), bf16),
        scratch_shapes=scratch,
        compiler_params=pltpu.CompilerParams(vmem_limit_bytes=126 * 1024 * 1024, flags=flags),
    )


@jax.jit
def pallas_parallel_sum__sliding_local_dilated__glu_gated_geglu__prompt_kernel(
    A_x, A_wqkv, A_wo, B_x, B_w_gate, B_w_up, B_w_down
):
    del B_x
    out = make_call()(np.zeros((4,), np.int32), A_x.reshape(S, D), A_wqkv, A_wo, B_w_gate, B_w_up, B_w_down)
    return out.reshape(1, S, D)
```

```python
import functools

import jax
import jax.numpy as jnp
import numpy as np
from jax import lax
import jax.experimental.pallas as pl
import jax.experimental.pallas.tpu as pltpu

S, D, F = 2048, 1024, 3584
DH, W, DIL = 32, 8, 2
HALO = 16
NB = D // 128
HS, QS = S // 2, S // 4
HD, QD = D // 2, D // 4
FC = 512
NCH = F // FC
PR = 16
AG = 8
LOG2E = 1.4426950408889634
ORDER = (2, 3, 0, 1, 4, 5, 6)
f32, bf16, u32 = jnp.float32, jnp.bfloat16, jnp.uint32


def _dot(a, b):
    return jnp.dot(a, b, preferred_element_type=f32)


def _words(v):
    return pltpu.bitcast(v.astype(bf16), u32)


def _halves(w):
    return pltpu.bitcast(w, bf16)


def _lhs_terms(a11, a12, a21, a22):
    return [a11 + a22, a21 + a22, a11, a22, a11 + a12, a21 - a11, a12 - a22]


def _lhs_term(i, a):
    return (lambda: a(0) + a(3), lambda: a(2) + a(3), lambda: a(0), lambda: a(3),
            lambda: a(0) + a(1), lambda: a(2) - a(0), lambda: a(1) - a(3))[i]()


def _rhs_terms(b11, b12, b21, b22):
    return [b11 + b22, b11, b12 - b22, b21 - b11, b22, b11 + b12, b21 + b22]


def _seven_products(product, keep, fetch, finish):
    for i in (2, 3, 0):
        keep(i, product(i))
    m = product(1)
    keep(1, m)
    finish(2, fetch(3) + m)
    m = product(4)
    keep(4, m)
    finish(1, fetch(2) + m)
    finish(3, fetch(2) + fetch(0) - fetch(1) + product(5))
    finish(0, fetch(3) + fetch(0) - fetch(4) + product(6))


def _quarter(p, q):
    return 2 * (p // 2) + q // 2, 2 * (p % 2) + q % 2


def _two_level(block, terms_of, store, wait_for):
    for i in range(7):
        inner = terms_of(*[terms_of(*[block(p, q) for p in range(4)])[i] for q in range(4)])
        for j in range(7):
            store(7 * i + j, _words(inner[j]))
        wait_for(inner[6])


def _to_head_lanes(blocks):
    slot = lax.broadcasted_iota(jnp.int32, blocks[0].shape, 1) >> 2
    blocks = [pltpu.roll(b, 4 * c, 1) if c else b for c, b in enumerate(blocks)]
    yield
    blocks = [blocks[-j % NB] for j in range(NB)]
    for bit in (1, 2, 4):
        move = (slot & bit) != 0
        blocks = [jnp.where(move, blocks[(j - bit) % NB], blocks[j]) for j in range(NB)]
    return [pltpu.roll(b, 128 - 4 * j, 1) if j else b for j, b in enumerate(blocks)]


def _run(*stages):
    stages = list(stages)
    while stages:
        stages = [g for g in stages if next(g, True) is None]


def _start(copies):
    for cp in copies:
        cp.start()


def _wait(copies):
    for cp in copies:
        cp.wait()


def _rows(r0, n):
    return pl.ds(r0 if isinstance(r0, int) else pl.multiple_of(r0, n), n)


def _word_rows(r0, n):
    return pl.ds(r0 // 2 if isinstance(r0, int) else pl.multiple_of(r0 // 2, 8), n // 2)


def _lanes(c):
    return slice(c * 128, (c + 1) * 128)


def _widen(ref, *idx):
    return _halves(pltpu.bitcast(ref[idx], u32)).astype(f32)


def _make_kernel(hm_q=128, hm_kv=512, hm_f=128, n_parts=4, q_stops=(1, 2, 4),
                 n_att=(10, 8), n_early=(9, 7), early_at=3, late_at=(0, 0)):
    n_q, n_kv, n_f = HS // hm_q, HS // hm_kv, QS // hm_f
    assert n_f * (n_att[0] * ((NCH + 1) // 2) + n_att[1] * (NCH // 2)) * AG == S

    def kernel(zero_ref, x_hbm, wqkv_hbm, wo_hbm, wg_hbm, wu_hbm, wd_hbm, out_hbm,
               xraw, xc2, woc, gc0, dc0, gc1, dc1, graw, draw, qo, kp, vp,
               xsem, qsem, wsem, fsem, osem, *work):
        gc, dc = (gc0, gc1), (dc0, dc1)
        pin, pout, pproj, hkeep, hc = work[0:5], work[5:10], work[10:15], work[15:19], work[19:26]
        zeros = [zero_ref[k] for k in range(4)]
        zero = zeros[0]

        def x_copies(t):
            rows = [_rows(half * HS + t * hm_q, hm_q) for half in range(2)]
            return [pltpu.make_async_copy(x_hbm.at[r, :], xraw.at[r, :], xsem.at[t]) for r in rows]

        def f_copies(j, slot):
            cols = pl.ds(pl.multiple_of(j * FC, FC), FC)
            return [pltpu.make_async_copy(wg_hbm.at[:, cols], graw.at[slot, 0, pl.ds(0, D), :], fsem.at[slot]),
                    pltpu.make_async_copy(wu_hbm.at[:, cols], graw.at[slot, 1, pl.ds(0, D), :], fsem.at[slot]),
                    pltpu.make_async_copy(wd_hbm.at[cols, :], draw.at[slot, pl.ds(0, FC), :], fsem.at[slot])]

        def pace(raw, value):
            spare = raw.shape[0] - PR
            raw[pl.ds(pl.multiple_of(spare + zeros[1], 8), 8), 0:128] = value[0:8].astype(bf16)

        def kept(bufs, n):
            def keep(i, v):
                bufs[i][0:n, :] = v
            return keep, lambda i: bufs[i][pl.ds(pl.multiple_of(zero, 8), n), :]

        def layernorm(xc, xn, mean, inv, first, paced=True):
            def block(r0, c, z):
                return _widen(xraw, _rows(r0 + zeros[z], PR), _lanes(c))

            def row_mean(vals):
                total = functools.reduce(jnp.add, vals)
                if paced:
                    pace(xraw, total)
                return jnp.broadcast_to(jnp.sum(total, axis=-1, keepdims=True) * (1.0 / D), (PR, 128))

            def stat(ref, r0):
                return ref[_rows(r0 + zero, PR), :]

            pieces = [first + k for k in range(0, hm_q, PR)]
            starts = [half * HS + m0 for m0 in pieces for half in range(2)]
            for r0 in starts:
                mean[_rows(r0, PR), :] = row_mean([block(r0, c, 0) for c in range(NB)])
            for r0 in starts:
                mu = stat(mean, r0)
                inv[_rows(r0, PR), :] = lax.rsqrt(
                    row_mean([jnp.square(block(r0, c, 2) - mu) for c in range(NB)]) + 1e-5)
            for m0 in pieces:
                mu = [stat(mean, half * HS + m0) for half in range(2)]
                scale = [stat(inv, half * HS + m0) for half in range(2)]
                for c in range(NB // 2):
                    vals = []
                    for b in range(4):
                        r0, cb = (b // 2) * HS + m0, (b % 2) * (NB // 2) + c
                        vals.append((block(r0, cb, 3) - mu[b // 2]) * scale[b // 2])
                        xn[_word_rows(r0, PR), _lanes(cb)] = _words(vals[b])
                    terms = _lhs_terms(*vals)
                    for i in range(7):
                        xc.at[i][_word_rows(m0, PR), _lanes(c)] = _words(terms[i])
                    if paced:
                        pace(xraw, terms[6])

        def prepare_qkv(raw, dst, part, nparts, rows=32, paced=True):
            n = HD // nparts
            for sb in range(n // rows):
                r0 = part * n + sb * rows
                words = yield from _to_head_lanes([
                    jnp.concatenate([pltpu.bitcast(raw[_rows(half * HD + r0, rows), _lanes(c)], u32)
                                     for half in range(2)], axis=0) for c in range(NB)])
                yield
                top = [_halves(w[:rows // 2]).astype(f32) for w in words]
                bot = [_halves(w[rows // 2:]).astype(f32) for w in words]
                for c in range(NB // 2):
                    terms = _rhs_terms(top[c], top[c + NB // 2], bot[c], bot[c + NB // 2])
                    for i in range(7):
                        dst.at[i][_word_rows(r0, rows), _lanes(c)] = _words(terms[i])
                if paced:
                    pace(raw, terms[6])

        def prepare_gate_up(raw, dst, part, nparts):
            n = QD // nparts
            for sb in range(n // PR):
                r0 = part * n + sb * PR
                for z in range(2):
                    def block(p, q):
                        kq, nq = _quarter(p, q)
                        return _widen(raw, z, _rows(kq * QD + r0, PR), _lanes(nq))

                    def store(i, w):
                        dst.at[i][_word_rows(r0, PR), _lanes(z)] = w
                    _two_level(block, _rhs_terms, store, functools.partial(pace, raw.at[z]))

        def prepare_down(raw, dst, part, nparts):
            n = FC // 4 // nparts
            for sb in range(n // PR):
                r0 = part * n + sb * PR
                for c in range(QD // 128):
                    def block(p, q):
                        kq, nq = _quarter(p, q)
                        return _widen(raw, _rows(kq * (FC // 4) + r0, PR), _lanes(2 * nq + c))

                    def store(i, w):
                        dst.at[i][_word_rows(r0, PR), _lanes(c)] = w
                    _two_level(block, _rhs_terms, store, functools.partial(pace, raw))

        def prepare_out(raw, tmp, dst, part, nparts):
            n = 8 // nparts
            low = lax.broadcasted_iota(jnp.int32, (8, 128), 0) < 4
            for sb in range(n):
                g = part * n + sb
                for d2 in range(2):
                    for kq in range(4):
                        r = (g & 1) * 512 + (g >> 1) * 32 + kq * 8
                        for c in range(NB):
                            rows = []
                            for h3 in range(2):
                                u = raw[_rows(r + h3 * 256, 8), _lanes(c)].astype(f32)
                                v = raw[_rows(r + h3 * 256 + 128, 8), _lanes(c)].astype(f32)
                                rows.append(jnp.where(low, pltpu.roll(u, 4, 0), v) if d2
                                            else jnp.where(low, u, pltpu.roll(v, 4, 0)))
                            tmp[kq * 8:(kq + 1) * 8, _lanes(c)] = _words(jnp.concatenate(rows, axis=0))
                            if c % 4 == 3:
                                pace(raw, rows[1])
                    for c in range(QD // 128):
                        def block(p, q):
                            kq, nq = _quarter(p, q)
                            return _halves(tmp[pl.ds(pl.multiple_of(kq * 8 + zero, 8), 8),
                                               _lanes(2 * nq + c)]).astype(f32)

                        def store(i, w):
                            dst.at[i][_word_rows(d2 * 128 + g * PR, PR), _lanes(c)] = w

                        def wait_for(v):
                            tmp[pl.ds(pl.multiple_of(32 + zeros[1], 8), 8), 0:128] = _words(v)
                        _two_level(block, _rhs_terms, store, wait_for)

        def prepare_x(xn, part, nparts):
            n = QS // nparts
            for sb in range(n // PR):
                m0 = part * n + sb * PR
                for c in range(QD // 128):
                    def block(p, q):
                        mq, kq = _quarter(p, q)
                        return _halves(xn[_word_rows(mq * QS + m0, PR), _lanes(2 * kq + c)]).astype(f32)

                    def store(i, w):
                        xc2.at[i][_word_rows(m0, PR), _lanes(c)] = w

                    def wait_for(v):
                        xn[pl.ds(pl.multiple_of(S // 2 + zero, 8), 8), 0:128] = _words(v)
                    _two_level(block, _lhs_terms, store, wait_for)

        def prepare_attended(dst, t, paced):
            for sb in range(hm_f // PR):
                for c in range(QD // 128):
                    def block(p, q):
                        mq, kq = _quarter(p, q)
                        return qo[2 * kq + c, _rows(mq * QS + t * hm_f + sb * PR, PR), :]

                    def store(k, w):
                        dst.at[k][_word_rows(sb * PR, PR), _lanes(c)] = w

                    def wait_for(v):
                        if paced:
                            qo[0, pl.ds(pl.multiple_of(S + zeros[1], 8), 8), :] = v[0:8]
                    _two_level(block, _lhs_terms, store, wait_for)

        def project(xc, wc, dst, off, t, hm, scale=None, shadow=lambda m: None):
            keep, fetch = kept(pproj, hm)
            for cb in range(NB // 2):
                def product(i):
                    lhs = _halves(xc[i, _word_rows(t * hm + (0 if isinstance(t, int) else zeros[cb]), hm), :])
                    m = _dot(lhs, _halves(wc[i + zero, :, _lanes(cb)]))
                    if (cb, i) == (0, ORDER[0]):
                        shadow(m)
                    return m

                def finish(b, v):
                    r0 = off + (b // 2) * HS + t * hm
                    r0 = r0 if isinstance(r0, int) else pl.multiple_of(r0, 8)
                    dst[(b % 2) * (NB // 2) + cb, pl.ds(r0, hm), :] = v if scale is None else v * scale
                _seven_products(product, keep, fetch, finish)

        again = pl.ds(pl.multiple_of(zero, 8), hm_f)

        def forty_nine_products(product, finish):
            def outer(i, q, m):
                fetch = lambda k: pout[k][q, again, :]
                if i < 5:
                    pout[i][q] = m
                if i == 1:
                    finish(2, q, fetch(3) + m)
                elif i == 4:
                    finish(1, q, fetch(2) + m)
                elif i == 5:
                    finish(3, q, fetch(2) + fetch(0) - fetch(1) + m)
                elif i == 6:
                    finish(0, q, fetch(3) + fetch(0) - fetch(4) + m)

            keep, fetch = kept(pin, hm_f)
            for i in ORDER:
                _seven_products(lambda j: product(7 * i + j), keep, fetch, lambda q, v: outer(i, q, v))

        def feed_forward(sums, slot, t, started, early, late):
            m0 = t * hm_f

            def gate(p, q, c):
                h = jax.nn.gelu(c[:, :128], approximate=True) * c[:, 128:]
                if (p, q) != (0, 0):
                    hkeep[p][q] = h
                if (p, q) == late_at:
                    late(h[0:8])
                if p in (3, 0) and q in (3, 0):
                    block = lambda pp, qq: h if (pp, qq) == (p, q) else hkeep[pp][qq, again, :]
                    for i in ((1, 3, 6) if p else (0, 2, 4, 5)):
                        for j in ((1, 3, 6) if q else (0, 2, 4, 5)):
                            hc[i].at[j][...] = _words(_lhs_term(
                                j, lambda qq: _lhs_term(i, lambda pp: block(pp, qq))))

            def product(k):
                m = _dot(_halves(xc2[k, _word_rows(m0, hm_f), :]), _halves(gc[slot][k]))
                if k == early_at:
                    early(m[0:8, 0:128])
                return m
            forty_nine_products(product, gate)

            for first in ((1, 3, 6), (0, 2, 4, 5)):
                for second in ((1, 3, 6), (0, 2, 4, 5)):
                    for i in first:
                        for j in second:
                            lhs = hc[i][j, pl.ds(pl.multiple_of(zero, 8), hm_f // 2), :]
                            rows = _rows(m0, hm_f)
                            sums[i][j, rows, :] = (jnp.where(started, sums[i][j, rows, :], 0.0)
                                                   + _dot(_halves(lhs), _halves(dc[slot][7 * i + j])))

        def output(sums, operands, t, shadow):
            m0 = t * hm_f

            def finish(p, q, v):
                mq, nq = _quarter(p, q)
                window = (_rows(mq * QS + m0, hm_f), pl.ds(nq * QD, QD))
                xraw[window] = (xraw[window].astype(f32) + v).astype(bf16)
                pltpu.make_async_copy(xraw.at[window], out_hbm.at[window], osem).start()

            def product(k):
                m = _dot(_halves(operands[k, pl.ds(pl.multiple_of(zero, 8), hm_f // 2), :]), _halves(woc[k]))
                if k == 8 * ORDER[0]:
                    shadow(m[0:8, 0:128])
                return m + sums[k // 7][k % 7, _rows(m0, hm_f), :]
            forty_nine_products(product, finish)

        def attention(first, groups):
            lane = lax.broadcasted_iota(jnp.int32, (AG, 128), 1)
            row = lax.broadcasted_iota(jnp.int32, (AG, 128), 0)
            for g in groups:
                s0 = pl.multiple_of((first + g) * AG + zeros[2 + g % 2], AG)
                q = [qo[c, pl.ds(s0, AG), :] for c in range(NB)]
                logits = []
                for w in range(W):
                    rows = pl.ds(s0 + (HALO - DIL * w), AG)
                    logits.append(functools.reduce(jnp.add, [q[c] * kp[c, rows, :] for c in range(NB)]))
                for d in (1, 2):
                    logits = [p + jnp.where((lane & d) == 0, pltpu.roll(p, 128 - d, 1), pltpu.roll(p, d, 1))
                              for p in logits]
                logits = [jnp.where(row + s0 >= DIL * w, p, -1e9 * LOG2E) if g * AG < DIL * w else p
                          for w, p in enumerate(logits)]
                top = functools.reduce(jnp.maximum, logits)
                es = [jnp.exp2(p - top) for p in logits]
                inv = 1.0 / functools.reduce(jnp.add, es)
                weights = [e * inv for e in es]
                for c in range(NB):
                    qo[c, pl.ds(s0, AG), :] = functools.reduce(
                        jnp.add, [weights[w] * vp[c, pl.ds(s0 + (HALO - DIL * w), AG), :] for w in range(W)])

        def first_half(xc, xn, mean, inv, tmp, head, wraw, wqc, wkc, wvc):
            q_scale = DH ** -0.5 * LOG2E

            def w_copies(p):
                src = wo_hbm if p == 3 else wqkv_hbm.at[:, p * D:(p + 1) * D]
                return [pltpu.make_async_copy(src, wraw.at[p, pl.ds(0, D), :], wsem.at[p])]

            def wq_copies(i):
                rows = [_rows(half * HD + i * (HD // n_parts), HD // n_parts) for half in range(2)]
                return [pltpu.make_async_copy(wqkv_hbm.at[r, pl.ds(0, D)], wraw.at[0, r, :], qsem.at[i])
                        for r in rows]

            _start(x_copies(0))
            lax.fori_loop(0, n_parts, lambda i, _: _start(wq_copies(i)), None)
            lax.fori_loop(1, n_q, lambda t, _: _start(x_copies(t)), None)
            _start(w_copies(1))
            for c in range(NB):
                kp[c, 0:HALO, :] = jnp.zeros((HALO, 128), f32)
            _wait(x_copies(0))
            layernorm(xc, xn, mean, inv, 0, paced=False)

            def first_body(i, _):
                _wait(wq_copies(i))
                n = HD // n_parts
                lhs = jnp.concatenate([
                    jnp.concatenate([xn[_word_rows(half * HS, hm_q), pl.ds(pl.multiple_of(k * HD + i * n, n), n)]
                                     for k in range(2)], axis=1) for half in range(2)], axis=0)
                for c in range(D // 256):
                    cols = slice(c * 256, (c + 1) * 256)
                    rhs = jnp.concatenate([wraw[0, _rows(k * HD + i * n, n), cols] for k in range(2)], axis=0)
                    head[:, cols] = jnp.where(i > 0, head[:, cols], 0.0) + _dot(_halves(lhs), rhs)
                _run(*[prepare_qkv(wraw.at[0], wqc, 4 * i + k, 4 * n_parts, PR, paced=False) for k in range(4)])
            lax.fori_loop(0, n_parts, first_body, None)
            _start(w_copies(2))

            for lo, hi in zip(q_stops, q_stops[1:] + (n_q,)):
                if lo == 1:
                    _wait(x_copies(1))
                    layernorm(xc, xn, mean, inv, hm_q, paced=False)
                for t in range(lo + 1, min(hi + 1, n_q)):
                    _wait(x_copies(t))
                if hi == n_q:
                    _wait(w_copies(1))
                    _start(w_copies(3))
                    _start(f_copies(0, 0))
                if lo == q_stops[1]:
                    for sb in range(hm_q // PR):
                        def head_to_q(half):
                            rows = _rows(half * hm_q + sb * PR + zeros[2 + sb % 2], PR)
                            blocks = yield from _to_head_lanes([head[rows, _lanes(c)] for c in range(NB)])
                            for c in range(NB):
                                qo[c, _rows(half * HS + sb * PR, PR), :] = blocks[c] * q_scale
                            head[rows, 0:128] = blocks[0]
                        _run(head_to_q(0), head_to_q(1))
                for t in range(lo, hi):
                    def next_layernorm(token):
                        if t + 1 < n_q:
                            pace(xraw, token)
                            layernorm(xc, xn, mean, inv, (t + 1) * hm_q)
                    project(xc, wqc, qo, 0, t, hm_q, q_scale, next_layernorm)
            _run(prepare_qkv(wraw.at[1], wkc, 0, 1))

            _wait(w_copies(2))
            _wait(w_copies(3))
            _start(f_copies(1, 1))

            def k_body(t, _):
                project(xc, wkc, kp, HALO, t, hm_kv)
                prepare_out(wraw.at[3], tmp, woc, t, n_kv)
                _run(prepare_qkv(wraw.at[2], wvc, t, n_kv))
            lax.fori_loop(0, n_kv, k_body, None)

            _wait(f_copies(0, 0))

            def v_body(t, _):
                project(xc, wvc, vp, HALO, t, hm_kv)
                prepare_x(xn, t, n_kv)
                prepare_gate_up(graw.at[0], gc0, t, n_kv)
                prepare_down(draw.at[0], dc0, t, n_kv)
            lax.fori_loop(0, n_kv, v_body, None)
            for c in range(NB):
                vp[c, 0:HALO, :] = jnp.broadcast_to(vp[c, HALO:HALO + 1, :], (HALO, 128))

        pl.run_scoped(
            first_half,
            pltpu.VMEM((7, HS // 2, HD), u32),
            pltpu.VMEM((S // 2 + 8, D), u32),
            pltpu.VMEM((S, 128), f32),
            pltpu.VMEM((S, 128), f32),
            pltpu.VMEM((40, D), u32),
            pltpu.VMEM((2 * hm_q, D), f32),
            pltpu.VMEM((4, D + PR, D), bf16),
            *[pltpu.VMEM((7, HD // 2, HD), u32)] * 3)

        def second_half(*sums):
            def chunk_body(j, _):
                src = jnp.minimum(j + 1, NCH - 1) % 2

                @pl.when(j + 1 < NCH)
                def _():
                    _wait(f_copies(j + 1, 1 - j % 2))

                @pl.when(j + 2 < NCH)
                def _():
                    _start(f_copies(j + 2, j % 2))

                for parity in range(2):
                    @pl.when(j % 2 == parity)
                    def _():
                        def tile_body(t, _):
                            first = n_f * (n_att[0] * ((j + 1) // 2) + n_att[1] * (j // 2)) + t * n_att[parity]

                            def shadow(groups, token):
                                qo[0, pl.ds(pl.multiple_of(S + zero, 8), 8), :] = token
                                attention(first, groups)
                            feed_forward(sums, parity, t, True if parity else j > 0,
                                         functools.partial(shadow, range(n_early[parity])),
                                         functools.partial(shadow, range(n_early[parity], n_att[parity])))
                            prepare_gate_up(graw.at[src], gc[1 - parity], t, n_f)
                            prepare_down(draw.at[src], dc[1 - parity], t, n_f)
                        lax.fori_loop(0, n_f, tile_body, None)
            lax.fori_loop(0, NCH, chunk_body, None)

            prepare_attended(gc0, 0, paced=False)
            for t in range(n_f):
                def next_operands(token):
                    if t + 1 < n_f:
                        qo[0, pl.ds(pl.multiple_of(S + zeros[1], 8), 8), :] = token
                        prepare_attended(gc[(t + 1) % 2], t + 1, paced=True)
                output(sums, gc[t % 2], t, next_operands)
            pltpu.make_async_copy(xraw.at[pl.ds(0, S), :], out_hbm, osem).wait()

        pl.run_scoped(second_half, *[pltpu.VMEM((7, QS, QD), f32)] * 7)

    scratch = [
        pltpu.VMEM((S + PR, D), bf16),
        pltpu.VMEM((49, QS // 2, QD), u32),
        pltpu.VMEM((49, QD // 2, QD), u32),
        pltpu.VMEM((49, QD // 2, FC // 2), u32),
        pltpu.VMEM((49, FC // 8, QD), u32),
        pltpu.VMEM((49, QD // 2, FC // 2), u32),
        pltpu.VMEM((49, FC // 8, QD), u32),
        pltpu.VMEM((2, 2, D + PR, FC), bf16),
        pltpu.VMEM((2, FC + PR, D), bf16),
        pltpu.VMEM((NB, S + 8, 128), f32),
        pltpu.VMEM((NB, HALO + S + 8, 128), f32),
        pltpu.VMEM((NB, HALO + S + 8, 128), f32),
        pltpu.SemaphoreType.DMA((n_q,)),
        pltpu.SemaphoreType.DMA((n_parts,)),
        pltpu.SemaphoreType.DMA((4,)),
        pltpu.SemaphoreType.DMA((2,)),
        pltpu.SemaphoreType.DMA(()),
        *[pltpu.VMEM((hm_f, 256), f32)] * 5,
        *[pltpu.VMEM((4, hm_f, 256), f32)] * 5,
        *[pltpu.VMEM((max(hm_q, hm_kv), 128), f32)] * 5,
        *[pltpu.VMEM((4, hm_f, 128), f32)] * 4,
        *[pltpu.VMEM((7, hm_f // 2, 128), u32)] * 7,
    ]
    return kernel, scratch


def make_call(**kw):
    kernel, scratch = _make_kernel(**kw)
    hbm = pl.BlockSpec(memory_space=pl.ANY)
    return pl.pallas_call(
        kernel,
        in_specs=[pl.BlockSpec(memory_space=pltpu.SMEM)] + [hbm] * 6,
        out_specs=hbm,
        out_shape=jax.ShapeDtypeStruct((S, D), bf16),
        scratch_shapes=scratch,
        compiler_params=pltpu.CompilerParams(vmem_limit_bytes=126 * 1024 * 1024),
    )


@jax.jit
def pallas_parallel_sum__sliding_local_dilated__glu_gated_geglu__prompt_kernel(
    A_x, A_wqkv, A_wo, B_x, B_w_gate, B_w_up, B_w_down
):
    del B_x
    out = make_call()(np.zeros((4,), np.int32), A_x.reshape(S, D), A_wqkv, A_wo, B_w_gate, B_w_up, B_w_down)
    return out.reshape(1, S, D)
```

```python
import functools

import jax
import jax.numpy as jnp
import numpy as np
from jax import lax
import jax.experimental.pallas as pl
import jax.experimental.pallas.tpu as pltpu

S, D, F = 2048, 1024, 3584
DH, W, DIL = 32, 8, 2
HALO = 16
NB = D // 128
HS, QS = S // 2, S // 4
HD, QD = D // 2, D // 4
FC = 512
NCH = F // FC
PR = 16
AG = 8
LOG2E = 1.4426950408889634
GELU_A = 0.7978845608028654
GELU_B = GELU_A * 0.044715
ORDER = (2, 3, 0, 1, 4, 5, 6)
f32, bf16, u32 = jnp.float32, jnp.bfloat16, jnp.uint32


def _dot(a, b):
    return jnp.dot(a, b, preferred_element_type=f32)


def _words(v):
    return pltpu.bitcast(v.astype(bf16), u32)


def _halves(w):
    return pltpu.bitcast(w, bf16)


def _lhs_terms(a11, a12, a21, a22):
    return [a11 + a22, a21 + a22, a11, a22, a11 + a12, a21 - a11, a12 - a22]


def _lhs_term(i, a):
    return (lambda: a(0) + a(3), lambda: a(2) + a(3), lambda: a(0), lambda: a(3),
            lambda: a(0) + a(1), lambda: a(2) - a(0), lambda: a(1) - a(3))[i]()


def _rhs_terms(b11, b12, b21, b22):
    return [b11 + b22, b11, b12 - b22, b21 - b11, b22, b11 + b12, b21 + b22]


def _seven_products(product, keep, fetch, finish):
    for i in (2, 3, 0):
        keep(i, product(i))
    m = product(1)
    keep(1, m)
    finish(2, fetch(3) + m)
    m = product(4)
    keep(4, m)
    finish(1, fetch(2) + m)
    finish(3, fetch(2) + fetch(0) - fetch(1) + product(5))
    finish(0, fetch(3) + fetch(0) - fetch(4) + product(6))


def _quarter(p, q):
    return 2 * (p // 2) + q // 2, 2 * (p % 2) + q % 2


def _two_level(block, terms_of, store, wait_for):
    for i in range(7):
        inner = terms_of(*[terms_of(*[block(p, q) for p in range(4)])[i] for q in range(4)])
        for j in range(7):
            store(7 * i + j, _words(inner[j]))
        wait_for(inner[6])


def _to_head_lanes(blocks):
    slot = lax.broadcasted_iota(jnp.int32, blocks[0].shape, 1) >> 2
    blocks = [pltpu.roll(b, 4 * c, 1) if c else b for c, b in enumerate(blocks)]
    yield
    blocks = [blocks[-j % NB] for j in range(NB)]
    for bit in (1, 2, 4):
        move = (slot & bit) != 0
        blocks = [jnp.where(move, blocks[(j - bit) % NB], blocks[j]) for j in range(NB)]
    return [pltpu.roll(b, 128 - 4 * j, 1) if j else b for j, b in enumerate(blocks)]


def _run(*stages):
    stages = list(stages)
    while stages:
        stages = [g for g in stages if next(g, True) is None]


def _start(copies):
    for cp in copies:
        cp.start()


def _wait(copies):
    for cp in copies:
        cp.wait()


def _rows(r0, n):
    return pl.ds(r0 if isinstance(r0, int) else pl.multiple_of(r0, n), n)


def _word_rows(r0, n):
    return pl.ds(r0 // 2 if isinstance(r0, int) else pl.multiple_of(r0 // 2, 8), n // 2)


def _lanes(c):
    return slice(c * 128, (c + 1) * 128)


def _widen(ref, *idx):
    return _halves(pltpu.bitcast(ref[idx], u32)).astype(f32)


def _make_kernel(hm_q=128, hm_kv=512, hm_f=128, n_parts=4, q_stops=(1, 2, 4),
                 n_att=(10, 8), n_early=(9, 7), early_at=3, late_at=(0, 0)):
    n_q, n_kv, n_f = HS // hm_q, HS // hm_kv, QS // hm_f
    assert n_f * (n_att[0] * ((NCH + 1) // 2) + n_att[1] * (NCH // 2)) * AG == S

    def kernel(zero_ref, x_hbm, wqkv_hbm, wo_hbm, wg_hbm, wu_hbm, wd_hbm, out_hbm,
               xraw, xc2, woc, gc0, dc0, gc1, dc1, graw, draw, qo, kp, vp,
               xsem, qsem, wsem, fsem, osem, *work):
        gc, dc = (gc0, gc1), (dc0, dc1)
        pin, pout, pproj, hkeep, hc = work[0:5], work[5:10], work[10:15], work[15:19], work[19:26]
        zeros = [zero_ref[k] for k in range(4)]
        zero = zeros[0]

        def x_copies(t):
            rows = [_rows(half * HS + t * hm_q, hm_q) for half in range(2)]
            return [pltpu.make_async_copy(x_hbm.at[r, :], xraw.at[r, :], xsem.at[t]) for r in rows]

        def f_copies(j, slot):
            cols = pl.ds(pl.multiple_of(j * FC, FC), FC)
            return [pltpu.make_async_copy(wg_hbm.at[:, cols], graw.at[slot, 0, pl.ds(0, D), :], fsem.at[slot]),
                    pltpu.make_async_copy(wu_hbm.at[:, cols], graw.at[slot, 1, pl.ds(0, D), :], fsem.at[slot]),
                    pltpu.make_async_copy(wd_hbm.at[cols, :], draw.at[slot, pl.ds(0, FC), :], fsem.at[slot])]

        def pace(raw, value):
            spare = raw.shape[0] - PR
            raw[pl.ds(pl.multiple_of(spare + zeros[1], 8), 8), 0:128] = value[0:8].astype(bf16)

        def kept(bufs, n):
            def keep(i, v):
                bufs[i][0:n, :] = v
            return keep, lambda i: bufs[i][pl.ds(pl.multiple_of(zero, 8), n), :]

        def layernorm(xc, xn, mean, inv, first, paced=True):
            def block(r0, c, z):
                return _widen(xraw, _rows(r0 + zeros[z], PR), _lanes(c))

            def row_mean(vals):
                total = functools.reduce(jnp.add, vals)
                if paced:
                    pace(xraw, total)
                return jnp.broadcast_to(jnp.sum(total, axis=-1, keepdims=True) * (1.0 / D), (PR, 128))

            def stat(ref, r0):
                return ref[_rows(r0 + zero, PR), :]

            pieces = [first + k for k in range(0, hm_q, PR)]
            starts = [half * HS + m0 for m0 in pieces for half in range(2)]
            for r0 in starts:
                mean[_rows(r0, PR), :] = row_mean([block(r0, c, 0) for c in range(NB)])
            for r0 in starts:
                mu = stat(mean, r0)
                inv[_rows(r0, PR), :] = lax.rsqrt(
                    row_mean([jnp.square(block(r0, c, 2) - mu) for c in range(NB)]) + 1e-5)
            for m0 in pieces:
                mu = [stat(mean, half * HS + m0) for half in range(2)]
                scale = [stat(inv, half * HS + m0) for half in range(2)]
                for c in range(NB // 2):
                    vals = []
                    for b in range(4):
                        r0, cb = (b // 2) * HS + m0, (b % 2) * (NB // 2) + c
                        vals.append((block(r0, cb, 3) - mu[b // 2]) * scale[b // 2])
                        xn[_word_rows(r0, PR), _lanes(cb)] = _words(vals[b])
                    terms = _lhs_terms(*vals)
                    for i in range(7):
                        xc.at[i][_word_rows(m0, PR), _lanes(c)] = _words(terms[i])
                    if paced:
                        pace(xraw, terms[6])

        def prepare_qkv(raw, dst, part, nparts, rows=32, paced=True):
            n = HD // nparts
            for sb in range(n // rows):
                r0 = part * n + sb * rows
                words = yield from _to_head_lanes([
                    jnp.concatenate([pltpu.bitcast(raw[_rows(half * HD + r0, rows), _lanes(c)], u32)
                                     for half in range(2)], axis=0) for c in range(NB)])
                yield
                top = [_halves(w[:rows // 2]).astype(f32) for w in words]
                bot = [_halves(w[rows // 2:]).astype(f32) for w in words]
                for c in range(NB // 2):
                    terms = _rhs_terms(top[c], top[c + NB // 2], bot[c], bot[c + NB // 2])
                    for i in range(7):
                        dst.at[i][_word_rows(r0, rows), _lanes(c)] = _words(terms[i])
                if paced:
                    pace(raw, terms[6])

        def prepare_gate_up(raw, dst, part, nparts):
            n = QD // nparts
            for sb in range(n // PR):
                r0 = part * n + sb * PR
                for z in range(2):
                    def block(p, q):
                        kq, nq = _quarter(p, q)
                        return _widen(raw, z, _rows(kq * QD + r0, PR), _lanes(nq))

                    def store(i, w):
                        dst.at[i][_word_rows(r0, PR), _lanes(z)] = w
                    _two_level(block, _rhs_terms, store, functools.partial(pace, raw.at[z]))

        def prepare_down(raw, dst, part, nparts):
            n = FC // 4 // nparts
            for sb in range(n // PR):
                r0 = part * n + sb * PR
                for c in range(QD // 128):
                    def block(p, q):
                        kq, nq = _quarter(p, q)
                        return _widen(raw, _rows(kq * (FC // 4) + r0, PR), _lanes(2 * nq + c))

                    def store(i, w):
                        dst.at[i][_word_rows(r0, PR), _lanes(c)] = w
                    _two_level(block, _rhs_terms, store, functools.partial(pace, raw))

        def prepare_out(raw, tmp, dst, part, nparts):
            n = 8 // nparts
            low = lax.broadcasted_iota(jnp.int32, (8, 128), 0) < 4
            for sb in range(n):
                g = part * n + sb
                for d2 in range(2):
                    for kq in range(4):
                        r = (g & 1) * 512 + (g >> 1) * 32 + kq * 8
                        for c in range(NB):
                            rows = []
                            for h3 in range(2):
                                u = raw[_rows(r + h3 * 256, 8), _lanes(c)].astype(f32)
                                v = raw[_rows(r + h3 * 256 + 128, 8), _lanes(c)].astype(f32)
                                rows.append(jnp.where(low, pltpu.roll(u, 4, 0), v) if d2
                                            else jnp.where(low, u, pltpu.roll(v, 4, 0)))
                            tmp[kq * 8:(kq + 1) * 8, _lanes(c)] = _words(jnp.concatenate(rows, axis=0))
                            if c % 4 == 3:
                                pace(raw, rows[1])
                    for c in range(QD // 128):
                        def block(p, q):
                            kq, nq = _quarter(p, q)
                            return _halves(tmp[pl.ds(pl.multiple_of(kq * 8 + zero, 8), 8),
                                               _lanes(2 * nq + c)]).astype(f32)

                        def store(i, w):
                            dst.at[i][_word_rows(d2 * 128 + g * PR, PR), _lanes(c)] = w

                        def wait_for(v):
                            tmp[pl.ds(pl.multiple_of(32 + zeros[1], 8), 8), 0:128] = _words(v)
                        _two_level(block, _rhs_terms, store, wait_for)

        def prepare_x(xn, part, nparts):
            n = QS // nparts
            for sb in range(n // PR):
                m0 = part * n + sb * PR
                for c in range(QD // 128):
                    def block(p, q):
                        mq, kq = _quarter(p, q)
                        return _halves(xn[_word_rows(mq * QS + m0, PR), _lanes(2 * kq + c)]).astype(f32)

                    def store(i, w):
                        xc2.at[i][_word_rows(m0, PR), _lanes(c)] = w

                    def wait_for(v):
                        xn[pl.ds(pl.multiple_of(S // 2 + zero, 8), 8), 0:128] = _words(v)
                    _two_level(block, _lhs_terms, store, wait_for)

        def prepare_attended(dst, t, paced):
            for sb in range(hm_f // PR):
                for c in range(QD // 128):
                    def block(p, q):
                        mq, kq = _quarter(p, q)
                        return qo[2 * kq + c, _rows(mq * QS + t * hm_f + sb * PR, PR), :]

                    def store(k, w):
                        dst.at[k][_word_rows(sb * PR, PR), _lanes(c)] = w

                    def wait_for(v):
                        if paced:
                            qo[0, pl.ds(pl.multiple_of(S + zeros[1], 8), 8), :] = v[0:8]
                    _two_level(block, _lhs_terms, store, wait_for)

        def project(xc, wc, dst, off, t, hm, scale=None, shadow=lambda m: None):
            keep, fetch = kept(pproj, hm)
            for cb in range(NB // 2):
                def product(i):
                    lhs = _halves(xc[i, _word_rows(t * hm + (0 if isinstance(t, int) else zeros[cb]), hm), :])
                    m = _dot(lhs, _halves(wc[i + zero, :, _lanes(cb)]))
                    if (cb, i) == (0, ORDER[0]):
                        shadow(m)
                    return m

                def finish(b, v):
                    r0 = off + (b // 2) * HS + t * hm
                    r0 = r0 if isinstance(r0, int) else pl.multiple_of(r0, 8)
                    dst[(b % 2) * (NB // 2) + cb, pl.ds(r0, hm), :] = v if scale is None else v * scale
                _seven_products(product, keep, fetch, finish)

        again = pl.ds(pl.multiple_of(zero, 8), hm_f)

        def forty_nine_products(product, finish):
            def outer(i, q, m):
                fetch = lambda k: pout[k][q, again, :]
                if i < 5:
                    pout[i][q] = m
                if i == 1:
                    finish(2, q, fetch(3) + m)
                elif i == 4:
                    finish(1, q, fetch(2) + m)
                elif i == 5:
                    finish(3, q, fetch(2) + fetch(0) - fetch(1) + m)
                elif i == 6:
                    finish(0, q, fetch(3) + fetch(0) - fetch(4) + m)

            keep, fetch = kept(pin, hm_f)
            for i in ORDER:
                _seven_products(lambda j: product(7 * i + j), keep, fetch, lambda q, v: outer(i, q, v))

        def feed_forward(sums, slot, t, started, early, late):
            m0 = t * hm_f

            def gate(p, q, c):
                g, u = c[:, :128], c[:, 128:]
                h = (g * u) * (0.5 + 0.5 * jnp.tanh(g * (GELU_A + GELU_B * (g * g))))
                if (p, q) != (0, 0):
                    hkeep[p][q] = h
                if (p, q) == late_at:
                    late(h[0:8])
                if p in (3, 0) and q in (3, 0):
                    block = lambda pp, qq: h if (pp, qq) == (p, q) else hkeep[pp][qq, again, :]
                    for i in ((1, 3, 6) if p else (0, 2, 4, 5)):
                        for j in ((1, 3, 6) if q else (0, 2, 4, 5)):
                            hc[i].at[j][...] = _words(_lhs_term(
                                j, lambda qq: _lhs_term(i, lambda pp: block(pp, qq))))

            def product(k):
                m = _dot(_halves(xc2[k, _word_rows(m0, hm_f), :]), _halves(gc[slot][k]))
                if k == early_at:
                    early(m[0:8, 0:128])
                return m
            forty_nine_products(product, gate)

            for first in ((1, 3, 6), (0, 2, 4, 5)):
                for second in ((1, 3, 6), (0, 2, 4, 5)):
                    for i in first:
                        for j in second:
                            lhs = hc[i][j, pl.ds(pl.multiple_of(zero, 8), hm_f // 2), :]
                            rows = _rows(m0, hm_f)
                            sums[i][j, rows, :] = (jnp.where(started, sums[i][j, rows, :], 0.0)
                                                   + _dot(_halves(lhs), _halves(dc[slot][7 * i + j])))

        def output(sums, operands, t, shadow):
            m0 = t * hm_f

            def finish(p, q, v):
                mq, nq = _quarter(p, q)
                window = (_rows(mq * QS + m0, hm_f), pl.ds(nq * QD, QD))
                xraw[window] = (xraw[window].astype(f32) + v).astype(bf16)
                pltpu.make_async_copy(xraw.at[window], out_hbm.at[window], osem).start()

            def product(k):
                m = _dot(_halves(operands[k, pl.ds(pl.multiple_of(zero, 8), hm_f // 2), :]), _halves(woc[k]))
                if k == 8 * ORDER[0]:
                    shadow(m[0:8, 0:128])
                return m + sums[k // 7][k % 7, _rows(m0, hm_f), :]
            forty_nine_products(product, finish)

        def attention(first, groups):
            lane = lax.broadcasted_iota(jnp.int32, (AG, 128), 1)
            row = lax.broadcasted_iota(jnp.int32, (AG, 128), 0)
            for g in groups:
                s0 = pl.multiple_of((first + g) * AG + zeros[2 + g % 2], AG)
                q = [qo[c, pl.ds(s0, AG), :] for c in range(NB)]
                logits = []
                for w in range(W):
                    rows = pl.ds(s0 + (HALO - DIL * w), AG)
                    logits.append(functools.reduce(jnp.add, [q[c] * kp[c, rows, :] for c in range(NB)]))
                for d in (1, 2):
                    logits = [p + jnp.where((lane & d) == 0, pltpu.roll(p, 128 - d, 1), pltpu.roll(p, d, 1))
                              for p in logits]
                logits = [jnp.where(row + s0 >= DIL * w, p, -1e9 * LOG2E) if g * AG < DIL * w else p
                          for w, p in enumerate(logits)]
                top = functools.reduce(jnp.maximum, logits)
                es = [jnp.exp2(p - top) for p in logits]
                inv = 1.0 / functools.reduce(jnp.add, es)
                weights = [e * inv for e in es]
                for c in range(NB):
                    qo[c, pl.ds(s0, AG), :] = functools.reduce(
                        jnp.add, [weights[w] * vp[c, pl.ds(s0 + (HALO - DIL * w), AG), :] for w in range(W)])

        def first_half(xc, xn, mean, inv, tmp, head, wraw, wqc, wkc, wvc):
            q_scale = DH ** -0.5 * LOG2E

            def w_copies(p):
                src = wo_hbm if p == 3 else wqkv_hbm.at[:, p * D:(p + 1) * D]
                return [pltpu.make_async_copy(src, wraw.at[p, pl.ds(0, D), :], wsem.at[p])]

            def wq_copies(i):
                rows = [_rows(half * HD + i * (HD // n_parts), HD // n_parts) for half in range(2)]
                return [pltpu.make_async_copy(wqkv_hbm.at[r, pl.ds(0, D)], wraw.at[0, r, :], qsem.at[i])
                        for r in rows]

            _start(x_copies(0))
            lax.fori_loop(0, n_parts, lambda i, _: _start(wq_copies(i)), None)
            lax.fori_loop(1, n_q, lambda t, _: _start(x_copies(t)), None)
            _start(w_copies(1))
            for c in range(NB):
                kp[c, 0:HALO, :] = jnp.zeros((HALO, 128), f32)
            _wait(x_copies(0))
            layernorm(xc, xn, mean, inv, 0, paced=False)

            def first_body(i, _):
                _wait(wq_copies(i))
                n = HD // n_parts
                lhs = jnp.concatenate([
                    jnp.concatenate([xn[_word_rows(half * HS, hm_q), pl.ds(pl.multiple_of(k * HD + i * n, n), n)]
                                     for k in range(2)], axis=1) for half in range(2)], axis=0)
                for c in range(D // 256):
                    cols = slice(c * 256, (c + 1) * 256)
                    rhs = jnp.concatenate([wraw[0, _rows(k * HD + i * n, n), cols] for k in range(2)], axis=0)
                    head[:, cols] = jnp.where(i > 0, head[:, cols], 0.0) + _dot(_halves(lhs), rhs)
                _run(*[prepare_qkv(wraw.at[0], wqc, 4 * i + k, 4 * n_parts, PR, paced=False) for k in range(4)])
            lax.fori_loop(0, n_parts, first_body, None)
            _start(w_copies(2))

            for lo, hi in zip(q_stops, q_stops[1:] + (n_q,)):
                if lo == 1:
                    _wait(x_copies(1))
                    layernorm(xc, xn, mean, inv, hm_q, paced=False)
                for t in range(lo + 1, min(hi + 1, n_q)):
                    _wait(x_copies(t))
                if hi == n_q:
                    _wait(w_copies(1))
                    _start(w_copies(3))
                    _start(f_copies(0, 0))
                if lo == q_stops[1]:
                    for sb in range(hm_q // PR):
                        def head_to_q(half):
                            rows = _rows(half * hm_q + sb * PR + zeros[2 + sb % 2], PR)
                            blocks = yield from _to_head_lanes([head[rows, _lanes(c)] for c in range(NB)])
                            for c in range(NB):
                                qo[c, _rows(half * HS + sb * PR, PR), :] = blocks[c] * q_scale
                            head[rows, 0:128] = blocks[0]
                        _run(head_to_q(0), head_to_q(1))
                for t in range(lo, hi):
                    def next_layernorm(token):
                        if t + 1 < n_q:
                            pace(xraw, token)
                            layernorm(xc, xn, mean, inv, (t + 1) * hm_q)
                    project(xc, wqc, qo, 0, t, hm_q, q_scale, next_layernorm)
            _run(prepare_qkv(wraw.at[1], wkc, 0, 1))

            _wait(w_copies(2))
            _wait(w_copies(3))
            _start(f_copies(1, 1))

            def k_body(t, _):
                project(xc, wkc, kp, HALO, t, hm_kv)
                prepare_out(wraw.at[3], tmp, woc, t, n_kv)
                _run(prepare_qkv(wraw.at[2], wvc, t, n_kv))
            lax.fori_loop(0, n_kv, k_body, None)

            _wait(f_copies(0, 0))

            def v_body(t, _):
                project(xc, wvc, vp, HALO, t, hm_kv)
                prepare_x(xn, t, n_kv)
                prepare_gate_up(graw.at[0], gc0, t, n_kv)
                prepare_down(draw.at[0], dc0, t, n_kv)
            lax.fori_loop(0, n_kv, v_body, None)
            for c in range(NB):
                vp[c, 0:HALO, :] = jnp.broadcast_to(vp[c, HALO:HALO + 1, :], (HALO, 128))

        pl.run_scoped(
            first_half,
            pltpu.VMEM((7, HS // 2, HD), u32),
            pltpu.VMEM((S // 2 + 8, D), u32),
            pltpu.VMEM((S, 128), f32),
            pltpu.VMEM((S, 128), f32),
            pltpu.VMEM((40, D), u32),
            pltpu.VMEM((2 * hm_q, D), f32),
            pltpu.VMEM((4, D + PR, D), bf16),
            *[pltpu.VMEM((7, HD // 2, HD), u32)] * 3)

        def second_half(*sums):
            def chunk_body(j, _):
                src = jnp.minimum(j + 1, NCH - 1) % 2

                @pl.when(j + 1 < NCH)
                def _():
                    _wait(f_copies(j + 1, 1 - j % 2))

                @pl.when(j + 2 < NCH)
                def _():
                    _start(f_copies(j + 2, j % 2))

                for parity in range(2):
                    @pl.when(j % 2 == parity)
                    def _():
                        def tile_body(t, _):
                            first = n_f * (n_att[0] * ((j + 1) // 2) + n_att[1] * (j // 2)) + t * n_att[parity]

                            def shadow(groups, token):
                                qo[0, pl.ds(pl.multiple_of(S + zero, 8), 8), :] = token
                                attention(first, groups)
                            feed_forward(sums, parity, t, True if parity else j > 0,
                                         functools.partial(shadow, range(n_early[parity])),
                                         functools.partial(shadow, range(n_early[parity], n_att[parity])))
                            prepare_gate_up(graw.at[src], gc[1 - parity], t, n_f)
                            prepare_down(draw.at[src], dc[1 - parity], t, n_f)
                        lax.fori_loop(0, n_f, tile_body, None)
            lax.fori_loop(0, NCH, chunk_body, None)

            prepare_attended(gc0, 0, paced=False)
            for t in range(n_f):
                def next_operands(token):
                    if t + 1 < n_f:
                        qo[0, pl.ds(pl.multiple_of(S + zeros[1], 8), 8), :] = token
                        prepare_attended(gc[(t + 1) % 2], t + 1, paced=True)
                output(sums, gc[t % 2], t, next_operands)
            pltpu.make_async_copy(xraw.at[pl.ds(0, S), :], out_hbm, osem).wait()

        pl.run_scoped(second_half, *[pltpu.VMEM((7, QS, QD), f32)] * 7)

    scratch = [
        pltpu.VMEM((S + PR, D), bf16),
        pltpu.VMEM((49, QS // 2, QD), u32),
        pltpu.VMEM((49, QD // 2, QD), u32),
        pltpu.VMEM((49, QD // 2, FC // 2), u32),
        pltpu.VMEM((49, FC // 8, QD), u32),
        pltpu.VMEM((49, QD // 2, FC // 2), u32),
        pltpu.VMEM((49, FC // 8, QD), u32),
        pltpu.VMEM((2, 2, D + PR, FC), bf16),
        pltpu.VMEM((2, FC + PR, D), bf16),
        pltpu.VMEM((NB, S + 8, 128), f32),
        pltpu.VMEM((NB, HALO + S + 8, 128), f32),
        pltpu.VMEM((NB, HALO + S + 8, 128), f32),
        pltpu.SemaphoreType.DMA((n_q,)),
        pltpu.SemaphoreType.DMA((n_parts,)),
        pltpu.SemaphoreType.DMA((4,)),
        pltpu.SemaphoreType.DMA((2,)),
        pltpu.SemaphoreType.DMA(()),
        *[pltpu.VMEM((hm_f, 256), f32)] * 5,
        *[pltpu.VMEM((4, hm_f, 256), f32)] * 5,
        *[pltpu.VMEM((max(hm_q, hm_kv), 128), f32)] * 5,
        *[pltpu.VMEM((4, hm_f, 128), f32)] * 4,
        *[pltpu.VMEM((7, hm_f // 2, 128), u32)] * 7,
    ]
    return kernel, scratch


def make_call(**kw):
    kernel, scratch = _make_kernel(**kw)
    hbm = pl.BlockSpec(memory_space=pl.ANY)
    return pl.pallas_call(
        kernel,
        in_specs=[pl.BlockSpec(memory_space=pltpu.SMEM)] + [hbm] * 6,
        out_specs=hbm,
        out_shape=jax.ShapeDtypeStruct((S, D), bf16),
        scratch_shapes=scratch,
        compiler_params=pltpu.CompilerParams(vmem_limit_bytes=126 * 1024 * 1024),
    )


@jax.jit
def pallas_parallel_sum__sliding_local_dilated__glu_gated_geglu__prompt_kernel(
    A_x, A_wqkv, A_wo, B_x, B_w_gate, B_w_up, B_w_down
):
    del B_x
    out = make_call()(np.zeros((4,), np.int32), A_x.reshape(S, D), A_wqkv, A_wo, B_w_gate, B_w_up, B_w_down)
    return out.reshape(1, S, D)
```

```python
import functools

import jax
import jax.numpy as jnp
from jax import lax
import jax.experimental.pallas as pl
import jax.experimental.pallas.tpu as pltpu

S, D, F = 2048, 1024, 3584
DH, W, DIL = 32, 8, 2
HALO = 16
NB = D // 128
HS, QS = S // 2, S // 4
HD, QD = D // 2, D // 4
FC = 512
NCH = F // FC
PR = 16
AG = 8
LOG2E = 1.4426950408889634
GELU_A = 0.7978845608028654
GELU_B = GELU_A * 0.044715
ORDER = (2, 3, 0, 1, 4, 5, 6)
f32, bf16, u32 = jnp.float32, jnp.bfloat16, jnp.uint32


def _dot(a, b):
    return jnp.dot(a, b, preferred_element_type=f32)


def _words(v):
    return pltpu.bitcast(v.astype(bf16), u32)


def _halves(w):
    return pltpu.bitcast(w, bf16)


def _lhs_terms(a11, a12, a21, a22):
    return [a11 + a22, a21 + a22, a11, a22, a11 + a12, a21 - a11, a12 - a22]


def _lhs_term(i, a):
    return (lambda: a(0) + a(3), lambda: a(2) + a(3), lambda: a(0), lambda: a(3),
            lambda: a(0) + a(1), lambda: a(2) - a(0), lambda: a(1) - a(3))[i]()


def _rhs_terms(b11, b12, b21, b22):
    return [b11 + b22, b11, b12 - b22, b21 - b11, b22, b11 + b12, b21 + b22]


def _seven_products(product, keep, fetch, finish):
    for i in (2, 3, 0):
        keep(i, product(i))
    m = product(1)
    keep(1, m)
    finish(2, fetch(3) + m)
    m = product(4)
    keep(4, m)
    finish(1, fetch(2) + m)
    finish(3, fetch(2) + fetch(0) - fetch(1) + product(5))
    finish(0, fetch(3) + fetch(0) - fetch(4) + product(6))


def _quarter(p, q):
    return 2 * (p // 2) + q // 2, 2 * (p % 2) + q % 2


def _two_level(block, terms_of, store, wait_for):
    for i in range(7):
        inner = terms_of(*[terms_of(*[block(p, q) for p in range(4)])[i] for q in range(4)])
        for j in range(7):
            store(7 * i + j, _words(inner[j]))
        wait_for(inner[6])


def _to_head_lanes(blocks):
    slot = lax.broadcasted_iota(jnp.int32, blocks[0].shape, 1) >> 2
    blocks = [pltpu.roll(b, 4 * c, 1) if c else b for c, b in enumerate(blocks)]
    yield
    blocks = [blocks[-j % NB] for j in range(NB)]
    for bit in (1, 2, 4):
        move = (slot & bit) != 0
        blocks = [jnp.where(move, blocks[(j - bit) % NB], blocks[j]) for j in range(NB)]
    return [pltpu.roll(b, 128 - 4 * j, 1) if j else b for j, b in enumerate(blocks)]


def _run(*stages):
    stages = list(stages)
    while stages:
        stages = [g for g in stages if next(g, True) is None]


def _start(copies):
    for cp in copies:
        cp.start()


def _wait(copies):
    for cp in copies:
        cp.wait()


def _rows(r0, n):
    return pl.ds(r0 if isinstance(r0, int) else pl.multiple_of(r0, n), n)


def _word_rows(r0, n):
    return pl.ds(r0 // 2 if isinstance(r0, int) else pl.multiple_of(r0 // 2, 8), n // 2)


def _lanes(c):
    return slice(c * 128, (c + 1) * 128)


def _widen(ref, *idx):
    return _halves(pltpu.bitcast(ref[idx], u32)).astype(f32)


def _make_kernel(hm_q=128, hm_kv=512, hm_f=128, n_parts=4, q_stops=(1, 2, 4),
                 n_att=(10, 8), n_early=(9, 7), early_at=3, late_at=(0, 0)):
    n_q, n_kv, n_f = HS // hm_q, HS // hm_kv, QS // hm_f
    assert n_f * (n_att[0] * ((NCH + 1) // 2) + n_att[1] * (NCH // 2)) * AG == S

    def kernel(x_hbm, wqkv_hbm, wo_hbm, wg_hbm, wu_hbm, wd_hbm, out_hbm,
               xraw, xc2, woc, gc0, dc0, gc1, dc1, graw, draw, qo, kp, vp,
               zero_ref, xsem, qsem, wsem, fsem, osem, *work):
        gc, dc = (gc0, gc1), (dc0, dc1)
        pin, pout, pproj, hkeep, hc = work[0:5], work[5:10], work[10:15], work[15:19], work[19:26]
        @pl.loop(0, 4)
        def _(k):
            zero_ref[k] = jnp.int32(0)
        zeros = [zero_ref[k] for k in range(4)]
        zero = zeros[0]

        def x_copies(t):
            rows = [_rows(half * HS + t * hm_q, hm_q) for half in range(2)]
            return [pltpu.make_async_copy(x_hbm.at[r, :], xraw.at[r, :], xsem.at[t]) for r in rows]

        def f_copies(j, slot):
            cols = pl.ds(pl.multiple_of(j * FC, FC), FC)
            return [pltpu.make_async_copy(wg_hbm.at[:, cols], graw.at[slot, 0, pl.ds(0, D), :], fsem.at[slot]),
                    pltpu.make_async_copy(wu_hbm.at[:, cols], graw.at[slot, 1, pl.ds(0, D), :], fsem.at[slot]),
                    pltpu.make_async_copy(wd_hbm.at[cols, :], draw.at[slot, pl.ds(0, FC), :], fsem.at[slot])]

        def pace(raw, value):
            spare = raw.shape[0] - PR
            raw[pl.ds(pl.multiple_of(spare + zeros[1], 8), 8), 0:128] = value[0:8].astype(bf16)

        def kept(bufs, n):
            def keep(i, v):
                bufs[i][0:n, :] = v
            return keep, lambda i: bufs[i][pl.ds(pl.multiple_of(zero, 8), n), :]

        def layernorm(xc, xn, mean, inv, first, paced=True):
            def block(r0, c, z):
                return _widen(xraw, _rows(r0 + zeros[z], PR), _lanes(c))

            def row_mean(vals):
                total = functools.reduce(jnp.add, vals)
                if paced:
                    pace(xraw, total)
                return jnp.broadcast_to(jnp.sum(total, axis=-1, keepdims=True) * (1.0 / D), (PR, 128))

            def stat(ref, r0):
                return ref[_rows(r0 + zero, PR), :]

            pieces = [first + k for k in range(0, hm_q, PR)]
            starts = [half * HS + m0 for m0 in pieces for half in range(2)]
            for r0 in starts:
                mean[_rows(r0, PR), :] = row_mean([block(r0, c, 0) for c in range(NB)])
            for r0 in starts:
                mu = stat(mean, r0)
                inv[_rows(r0, PR), :] = lax.rsqrt(
                    row_mean([jnp.square(block(r0, c, 2) - mu) for c in range(NB)]) + 1e-5)
            for m0 in pieces:
                mu = [stat(mean, half * HS + m0) for half in range(2)]
                scale = [stat(inv, half * HS + m0) for half in range(2)]
                for c in range(NB // 2):
                    vals = []
                    for b in range(4):
                        r0, cb = (b // 2) * HS + m0, (b % 2) * (NB // 2) + c
                        vals.append((block(r0, cb, 3) - mu[b // 2]) * scale[b // 2])
                        xn[_word_rows(r0, PR), _lanes(cb)] = _words(vals[b])
                    terms = _lhs_terms(*vals)
                    for i in range(7):
                        xc.at[i][_word_rows(m0, PR), _lanes(c)] = _words(terms[i])
                    if paced:
                        pace(xraw, terms[6])

        def prepare_qkv(raw, dst, part, nparts, rows=32, paced=True):
            n = HD // nparts
            for sb in range(n // rows):
                r0 = part * n + sb * rows
                words = yield from _to_head_lanes([
                    jnp.concatenate([pltpu.bitcast(raw[_rows(half * HD + r0, rows), _lanes(c)], u32)
                                     for half in range(2)], axis=0) for c in range(NB)])
                yield
                top = [_halves(w[:rows // 2]).astype(f32) for w in words]
                bot = [_halves(w[rows // 2:]).astype(f32) for w in words]
                for c in range(NB // 2):
                    terms = _rhs_terms(top[c], top[c + NB // 2], bot[c], bot[c + NB // 2])
                    for i in range(7):
                        dst.at[i][_word_rows(r0, rows), _lanes(c)] = _words(terms[i])
                if paced:
                    pace(raw, terms[6])

        def prepare_gate_up(raw, dst, part, nparts):
            n = QD // nparts
            for sb in range(n // PR):
                r0 = part * n + sb * PR
                for z in range(2):
                    def block(p, q):
                        kq, nq = _quarter(p, q)
                        return _widen(raw, z, _rows(kq * QD + r0, PR), _lanes(nq))

                    def store(i, w):
                        dst.at[i][_word_rows(r0, PR), _lanes(z)] = w
                    _two_level(block, _rhs_terms, store, functools.partial(pace, raw.at[z]))

        def prepare_down(raw, dst, part, nparts):
            n = FC // 4 // nparts
            for sb in range(n // PR):
                r0 = part * n + sb * PR
                for c in range(QD // 128):
                    def block(p, q):
                        kq, nq = _quarter(p, q)
                        return _widen(raw, _rows(kq * (FC // 4) + r0, PR), _lanes(2 * nq + c))

                    def store(i, w):
                        dst.at[i][_word_rows(r0, PR), _lanes(c)] = w
                    _two_level(block, _rhs_terms, store, functools.partial(pace, raw))

        def prepare_out(raw, tmp, dst, part, nparts):
            n = 8 // nparts
            low = lax.broadcasted_iota(jnp.int32, (8, 128), 0) < 4
            for sb in range(n):
                g = part * n + sb
                for d2 in range(2):
                    for kq in range(4):
                        r = (g & 1) * 512 + (g >> 1) * 32 + kq * 8
                        for c in range(NB):
                            rows = []
                            for h3 in range(2):
                                u = raw[_rows(r + h3 * 256, 8), _lanes(c)].astype(f32)
                                v = raw[_rows(r + h3 * 256 + 128, 8), _lanes(c)].astype(f32)
                                rows.append(jnp.where(low, pltpu.roll(u, 4, 0), v) if d2
                                            else jnp.where(low, u, pltpu.roll(v, 4, 0)))
                            tmp[kq * 8:(kq + 1) * 8, _lanes(c)] = _words(jnp.concatenate(rows, axis=0))
                            if c % 4 == 3:
                                pace(raw, rows[1])
                    for c in range(QD // 128):
                        def block(p, q):
                            kq, nq = _quarter(p, q)
                            return _halves(tmp[pl.ds(pl.multiple_of(kq * 8 + zero, 8), 8),
                                               _lanes(2 * nq + c)]).astype(f32)

                        def store(i, w):
                            dst.at[i][_word_rows(d2 * 128 + g * PR, PR), _lanes(c)] = w

                        def wait_for(v):
                            tmp[pl.ds(pl.multiple_of(32 + zeros[1], 8), 8), 0:128] = _words(v)
                        _two_level(block, _rhs_terms, store, wait_for)

        def prepare_x(xn, part, nparts):
            n = QS // nparts
            for sb in range(n // PR):
                m0 = part * n + sb * PR
                for c in range(QD // 128):
                    def block(p, q):
                        mq, kq = _quarter(p, q)
                        return _halves(xn[_word_rows(mq * QS + m0, PR), _lanes(2 * kq + c)]).astype(f32)

                    def store(i, w):
                        xc2.at[i][_word_rows(m0, PR), _lanes(c)] = w

                    def wait_for(v):
                        xn[pl.ds(pl.multiple_of(S // 2 + zero, 8), 8), 0:128] = _words(v)
                    _two_level(block, _lhs_terms, store, wait_for)

        def prepare_attended(dst, t, paced):
            for sb in range(hm_f // PR):
                for c in range(QD // 128):
                    def block(p, q):
                        mq, kq = _quarter(p, q)
                        return qo[2 * kq + c, _rows(mq * QS + t * hm_f + sb * PR, PR), :]

                    def store(k, w):
                        dst.at[k][_word_rows(sb * PR, PR), _lanes(c)] = w

                    def wait_for(v):
                        if paced:
                            qo[0, pl.ds(pl.multiple_of(S + zeros[1], 8), 8), :] = v[0:8]
                    _two_level(block, _lhs_terms, store, wait_for)

        def project(xc, wc, dst, off, t, hm, scale=None, shadow=lambda m: None):
            keep, fetch = kept(pproj, hm)
            for cb in range(NB // 2):
                def product(i):
                    lhs = _halves(xc[i, _word_rows(t * hm + (0 if isinstance(t, int) else zeros[cb]), hm), :])
                    m = _dot(lhs, _halves(wc[i + zero, :, _lanes(cb)]))
                    if (cb, i) == (0, ORDER[0]):
                        shadow(m)
                    return m

                def finish(b, v):
                    r0 = off + (b // 2) * HS + t * hm
                    r0 = r0 if isinstance(r0, int) else pl.multiple_of(r0, 8)
                    dst[(b % 2) * (NB // 2) + cb, pl.ds(r0, hm), :] = v if scale is None else v * scale
                _seven_products(product, keep, fetch, finish)

        again = pl.ds(pl.multiple_of(zero, 8), hm_f)

        def forty_nine_products(product, finish):
            def outer(i, q, m):
                fetch = lambda k: pout[k][q, again, :]
                if i < 5:
                    pout[i][q] = m
                if i == 1:
                    finish(2, q, fetch(3) + m)
                elif i == 4:
                    finish(1, q, fetch(2) + m)
                elif i == 5:
                    finish(3, q, fetch(2) + fetch(0) - fetch(1) + m)
                elif i == 6:
                    finish(0, q, fetch(3) + fetch(0) - fetch(4) + m)

            keep, fetch = kept(pin, hm_f)
            for i in ORDER:
                _seven_products(lambda j: product(7 * i + j), keep, fetch, lambda q, v: outer(i, q, v))

        def feed_forward(sums, slot, t, started, early, late):
            m0 = t * hm_f

            def gate(p, q, c):
                g, u = c[:, :128], c[:, 128:]
                h = (g * u) * (0.5 + 0.5 * jnp.tanh(g * (GELU_A + GELU_B * (g * g))))
                if (p, q) != (0, 0):
                    hkeep[p][q] = h
                if (p, q) == late_at:
                    late(h[0:8])
                if p in (3, 0) and q in (3, 0):
                    block = lambda pp, qq: h if (pp, qq) == (p, q) else hkeep[pp][qq, again, :]
                    for i in ((1, 3, 6) if p else (0, 2, 4, 5)):
                        for j in ((1, 3, 6) if q else (0, 2, 4, 5)):
                            hc[i].at[j][...] = _words(_lhs_term(
                                j, lambda qq: _lhs_term(i, lambda pp: block(pp, qq))))

            def product(k):
                m = _dot(_halves(xc2[k, _word_rows(m0, hm_f), :]), _halves(gc[slot][k]))
                if k == early_at:
                    early(m[0:8, 0:128])
                return m
            forty_nine_products(product, gate)

            for first in ((1, 3, 6), (0, 2, 4, 5)):
                for second in ((1, 3, 6), (0, 2, 4, 5)):
                    for i in first:
                        for j in second:
                            lhs = hc[i][j, pl.ds(pl.multiple_of(zero, 8), hm_f // 2), :]
                            rows = _rows(m0, hm_f)
                            sums[i][j, rows, :] = (jnp.where(started, sums[i][j, rows, :], 0.0)
                                                   + _dot(_halves(lhs), _halves(dc[slot][7 * i + j])))

        def output(sums, operands, t, shadow):
            m0 = t * hm_f

            def finish(p, q, v):
                mq, nq = _quarter(p, q)
                window = (_rows(mq * QS + m0, hm_f), pl.ds(nq * QD, QD))
                xraw[window] = (xraw[window].astype(f32) + v).astype(bf16)
                pltpu.make_async_copy(xraw.at[window], out_hbm.at[window], osem).start()

            def product(k):
                m = _dot(_halves(operands[k, pl.ds(pl.multiple_of(zero, 8), hm_f // 2), :]), _halves(woc[k]))
                if k == 8 * ORDER[0]:
                    shadow(m[0:8, 0:128])
                return m + sums[k // 7][k % 7, _rows(m0, hm_f), :]
            forty_nine_products(product, finish)

        def attention(first, groups):
            lane = lax.broadcasted_iota(jnp.int32, (AG, 128), 1)
            row = lax.broadcasted_iota(jnp.int32, (AG, 128), 0)
            for g in groups:
                s0 = pl.multiple_of((first + g) * AG + zeros[2 + g % 2], AG)
                q = [qo[c, pl.ds(s0, AG), :] for c in range(NB)]
                logits = []
                for w in range(W):
                    rows = pl.ds(s0 + (HALO - DIL * w), AG)
                    logits.append(functools.reduce(jnp.add, [q[c] * kp[c, rows, :] for c in range(NB)]))
                for d in (1, 2):
                    logits = [p + jnp.where((lane & d) == 0, pltpu.roll(p, 128 - d, 1), pltpu.roll(p, d, 1))
                              for p in logits]
                logits = [jnp.where(row + s0 >= DIL * w, p, -1e9 * LOG2E) if g * AG < DIL * w else p
                          for w, p in enumerate(logits)]
                top = functools.reduce(jnp.maximum, logits)
                es = [jnp.exp2(p - top) for p in logits]
                inv = 1.0 / functools.reduce(jnp.add, es)
                weights = [e * inv for e in es]
                for c in range(NB):
                    qo[c, pl.ds(s0, AG), :] = functools.reduce(
                        jnp.add, [weights[w] * vp[c, pl.ds(s0 + (HALO - DIL * w), AG), :] for w in range(W)])

        def first_half(xc, xn, mean, inv, tmp, head, wraw, wqc, wkc, wvc):
            q_scale = DH ** -0.5 * LOG2E

            def w_copies(p):
                src = wo_hbm if p == 3 else wqkv_hbm.at[:, p * D:(p + 1) * D]
                return [pltpu.make_async_copy(src, wraw.at[p, pl.ds(0, D), :], wsem.at[p])]

            def wq_copies(i):
                rows = [_rows(half * HD + i * (HD // n_parts), HD // n_parts) for half in range(2)]
                return [pltpu.make_async_copy(wqkv_hbm.at[r, pl.ds(0, D)], wraw.at[0, r, :], qsem.at[i])
                        for r in rows]

            _start(x_copies(0))
            lax.fori_loop(0, n_parts, lambda i, _: _start(wq_copies(i)), None)
            lax.fori_loop(1, n_q, lambda t, _: _start(x_copies(t)), None)
            _start(w_copies(1))
            for c in range(NB):
                kp[c, 0:HALO, :] = jnp.zeros((HALO, 128), f32)
            _wait(x_copies(0))
            layernorm(xc, xn, mean, inv, 0, paced=False)

            def first_body(i, _):
                _wait(wq_copies(i))
                n = HD // n_parts
                lhs = jnp.concatenate([
                    jnp.concatenate([xn[_word_rows(half * HS, hm_q), pl.ds(pl.multiple_of(k * HD + i * n, n), n)]
                                     for k in range(2)], axis=1) for half in range(2)], axis=0)
                for c in range(D // 256):
                    cols = slice(c * 256, (c + 1) * 256)
                    rhs = jnp.concatenate([wraw[0, _rows(k * HD + i * n, n), cols] for k in range(2)], axis=0)
                    head[:, cols] = jnp.where(i > 0, head[:, cols], 0.0) + _dot(_halves(lhs), rhs)
                _run(*[prepare_qkv(wraw.at[0], wqc, 4 * i + k, 4 * n_parts, PR, paced=False) for k in range(4)])
            lax.fori_loop(0, n_parts, first_body, None)
            _start(w_copies(2))

            for lo, hi in zip(q_stops, q_stops[1:] + (n_q,)):
                if lo == 1:
                    _wait(x_copies(1))
                    layernorm(xc, xn, mean, inv, hm_q, paced=False)
                for t in range(lo + 1, min(hi + 1, n_q)):
                    _wait(x_copies(t))
                if hi == n_q:
                    _wait(w_copies(1))
                    _start(w_copies(3))
                    _start(f_copies(0, 0))
                if lo == q_stops[1]:
                    for sb in range(hm_q // PR):
                        def head_to_q(half):
                            rows = _rows(half * hm_q + sb * PR + zeros[2 + sb % 2], PR)
                            blocks = yield from _to_head_lanes([head[rows, _lanes(c)] for c in range(NB)])
                            for c in range(NB):
                                qo[c, _rows(half * HS + sb * PR, PR), :] = blocks[c] * q_scale
                            head[rows, 0:128] = blocks[0]
                        _run(head_to_q(0), head_to_q(1))
                for t in range(lo, hi):
                    def next_layernorm(token):
                        if t + 1 < n_q:
                            pace(xraw, token)
                            layernorm(xc, xn, mean, inv, (t + 1) * hm_q)
                    project(xc, wqc, qo, 0, t, hm_q, q_scale, next_layernorm)
            _run(prepare_qkv(wraw.at[1], wkc, 0, 1))

            _wait(w_copies(2))
            _wait(w_copies(3))
            _start(f_copies(1, 1))

            def k_body(t, _):
                project(xc, wkc, kp, HALO, t, hm_kv)
                prepare_out(wraw.at[3], tmp, woc, t, n_kv)
                _run(prepare_qkv(wraw.at[2], wvc, t, n_kv))
            lax.fori_loop(0, n_kv, k_body, None)

            _wait(f_copies(0, 0))

            def v_body(t, _):
                project(xc, wvc, vp, HALO, t, hm_kv)
                prepare_x(xn, t, n_kv)
                prepare_gate_up(graw.at[0], gc0, t, n_kv)
                prepare_down(draw.at[0], dc0, t, n_kv)
            lax.fori_loop(0, n_kv, v_body, None)
            for c in range(NB):
                vp[c, 0:HALO, :] = jnp.broadcast_to(vp[c, HALO:HALO + 1, :], (HALO, 128))

        pl.run_scoped(
            first_half,
            pltpu.VMEM((7, HS // 2, HD), u32),
            pltpu.VMEM((S // 2 + 8, D), u32),
            pltpu.VMEM((S, 128), f32),
            pltpu.VMEM((S, 128), f32),
            pltpu.VMEM((40, D), u32),
            pltpu.VMEM((2 * hm_q, D), f32),
            pltpu.VMEM((4, D + PR, D), bf16),
            *[pltpu.VMEM((7, HD // 2, HD), u32)] * 3)

        def second_half(*sums):
            def chunk_body(j, _):
                src = jnp.minimum(j + 1, NCH - 1) % 2

                @pl.when(j + 1 < NCH)
                def _():
                    _wait(f_copies(j + 1, 1 - j % 2))

                @pl.when(j + 2 < NCH)
                def _():
                    _start(f_copies(j + 2, j % 2))

                for parity in range(2):
                    @pl.when(j % 2 == parity)
                    def _():
                        def tile_body(t, _):
                            first = n_f * (n_att[0] * ((j + 1) // 2) + n_att[1] * (j // 2)) + t * n_att[parity]

                            def shadow(groups, token):
                                qo[0, pl.ds(pl.multiple_of(S + zero, 8), 8), :] = token
                                attention(first, groups)
                            feed_forward(sums, parity, t, True if parity else j > 0,
                                         functools.partial(shadow, range(n_early[parity])),
                                         functools.partial(shadow, range(n_early[parity], n_att[parity])))
                            prepare_gate_up(graw.at[src], gc[1 - parity], t, n_f)
                            prepare_down(draw.at[src], dc[1 - parity], t, n_f)
                        lax.fori_loop(0, n_f, tile_body, None)
            lax.fori_loop(0, NCH, chunk_body, None)

            prepare_attended(gc0, 0, paced=False)
            for t in range(n_f):
                def next_operands(token):
                    if t + 1 < n_f:
                        qo[0, pl.ds(pl.multiple_of(S + zeros[1], 8), 8), :] = token
                        prepare_attended(gc[(t + 1) % 2], t + 1, paced=True)
                output(sums, gc[t % 2], t, next_operands)
            pltpu.make_async_copy(xraw.at[pl.ds(0, S), :], out_hbm, osem).wait()

        pl.run_scoped(second_half, *[pltpu.VMEM((7, QS, QD), f32)] * 7)

    scratch = [
        pltpu.VMEM((S + PR, D), bf16),
        pltpu.VMEM((49, QS // 2, QD), u32),
        pltpu.VMEM((49, QD // 2, QD), u32),
        pltpu.VMEM((49, QD // 2, FC // 2), u32),
        pltpu.VMEM((49, FC // 8, QD), u32),
        pltpu.VMEM((49, QD // 2, FC // 2), u32),
        pltpu.VMEM((49, FC // 8, QD), u32),
        pltpu.VMEM((2, 2, D + PR, FC), bf16),
        pltpu.VMEM((2, FC + PR, D), bf16),
        pltpu.VMEM((NB, S + 8, 128), f32),
        pltpu.VMEM((NB, HALO + S + 8, 128), f32),
        pltpu.VMEM((NB, HALO + S + 8, 128), f32),
        pltpu.SMEM((4,), jnp.int32),
        pltpu.SemaphoreType.DMA((n_q,)),
        pltpu.SemaphoreType.DMA((n_parts,)),
        pltpu.SemaphoreType.DMA((4,)),
        pltpu.SemaphoreType.DMA((2,)),
        pltpu.SemaphoreType.DMA(()),
        *[pltpu.VMEM((hm_f, 256), f32)] * 5,
        *[pltpu.VMEM((4, hm_f, 256), f32)] * 5,
        *[pltpu.VMEM((max(hm_q, hm_kv), 128), f32)] * 5,
        *[pltpu.VMEM((4, hm_f, 128), f32)] * 4,
        *[pltpu.VMEM((7, hm_f // 2, 128), u32)] * 7,
    ]
    return kernel, scratch


@jax.jit
def pallas_parallel_sum__sliding_local_dilated__glu_gated_geglu__prompt_kernel(
    A_x: jax.Array,
    A_wqkv: jax.Array,
    A_wo: jax.Array,
    B_x: jax.Array,
    B_w_gate: jax.Array,
    B_w_up: jax.Array,
    B_w_down: jax.Array,
):
    del B_x
    kernel, scratch = _make_kernel()
    hbm = pl.BlockSpec(memory_space=pl.ANY)
    out = pl.pallas_call(
        kernel,
        in_specs=[hbm] * 6,
        out_specs=hbm,
        out_shape=jax.ShapeDtypeStruct((S, D), bf16),
        scratch_shapes=scratch,
        compiler_params=pltpu.CompilerParams(vmem_limit_bytes=126 * 1024 * 1024),
    )(A_x.reshape(S, D), A_wqkv, A_wo, B_w_gate, B_w_up, B_w_down)
    return out.reshape(1, S, D)
```
